```python
import jax
import jax.numpy as jnp

def _softmax(x, axis=-1):
    return jax.nn.softmax(x, axis=axis)

def _gelu(x):
    return jax.nn.gelu(x, approximate=True)

def _silu(x):
    return jax.nn.silu(x)

def _sigmoid(x):
    return jax.nn.sigmoid(x)

def _layernorm(x, axis=-1, eps=1e-05):
    m = jnp.mean(x, axis=axis, keepdims=True)
    v = jnp.var(x, axis=axis, keepdims=True)
    return (x - m) / jnp.sqrt(v + eps)

def _scatter_add(tgt, idx, src, axis=0):
    return tgt.at[idx].add(src)

def _segment_sum(src, seg, n):
    return jax.ops.segment_sum(src, seg, n)

class _Rng:

    def __init__(self, key):
        self._k = key

    def _next(self):
        self._k, sub = jax.random.split(self._k)
        return sub

    def normal(self, shape):
        return jax.random.normal(self._next(), shape, dtype=jnp.bfloat16)

    def randint(self, lo, hi, shape):
        return jax.random.randint(self._next(), shape, lo, hi, dtype=jnp.int32)

    def uniform(self, shape, lo=0.0, hi=1.0):
        return jax.random.uniform(self._next(), shape, jnp.bfloat16, lo, hi)

    def permutation(self, n):
        return jax.random.permutation(self._next(), n)
kernel_name = 'interleave_layers__memory_aug_recurrent_mem_tr__glu_gated_glu__prompt'

def setup_inputs():
    _rng = _Rng(jax.random.key(int.from_bytes(__import__("os").urandom(4), "little")))
    _w = lambda a: (lambda t: t.astype(jnp.bfloat16) if jnp.issubdtype(t.dtype, jnp.floating) else t)(jnp.asarray(a))

    def _A_setup():
        B, S, Dm = (1, 2048, 1024)
        H, Dh = (32, 128)
        M, seg = (8, 32)
        seg = min(seg, S)
        S = S // seg * seg
        return {'x': _w((lambda *s: _rng.normal(s) * 0.05)(B, S, Dm)), 'mem0': _w((lambda *s: _rng.normal(s) * 0.05)(B, M, Dm)), 'Wq': _w((lambda *s: _rng.normal(s) * 0.05)(Dm, H, Dh) * Dm ** (-0.5)), 'Wk': _w((lambda *s: _rng.normal(s) * 0.05)(Dm, H, Dh) * Dm ** (-0.5)), 'Wv': _w((lambda *s: _rng.normal(s) * 0.05)(Dm, H, Dh) * Dm ** (-0.5)), 'Wo': _w((lambda *s: _rng.normal(s) * 0.05)(H, Dh, Dm) * (H * Dh) ** (-0.5)), 'seg_len': seg}
    _A_in = _A_setup()

    def _B_setup():
        B, S, D, F = (1, 2048, 1024, 3584)
        return {'x': _w((lambda *s: _rng.normal(s) * 0.05)(B, S, D)), 'w_gate': _w((lambda *s: _rng.normal(s) * 0.05)(D, F)), 'w_up': _w((lambda *s: _rng.normal(s) * 0.05)(D, F)), 'w_down': _w((lambda *s: _rng.normal(s) * 0.05)(F, D))}
    _B_in = _B_setup()
    return {'A_x': _A_in['x'], 'A_mem0': _A_in['mem0'], 'A_Wq': _A_in['Wq'], 'A_Wk': _A_in['Wk'], 'A_Wv': _A_in['Wv'], 'A_Wo': _A_in['Wo'], 'A_seg_len': _A_in['seg_len'], 'B_x': _B_in['x'], 'B_w_gate': _B_in['w_gate'], 'B_w_up': _B_in['w_up'], 'B_w_down': _B_in['w_down']}

def reference(A_x, A_mem0, A_Wq, A_Wk, A_Wv, A_Wo, A_seg_len, B_x, B_w_gate, B_w_up, B_w_down):

    def _A_ref(x, mem0, Wq, Wk, Wv, Wo, seg_len):
        B, S, Dm = x.shape
        H, Dh = (Wq.shape[1], Wq.shape[2])
        M = mem0.shape[1]
        scale = Dh ** (-0.5)
        n_seg = S // seg_len
        L = M + seg_len
        idx = jnp.arange(L)
        mask = (idx[:, None] < M) | (idx[:, None] >= idx[None, :])
        mem = mem0
        outs = []
        for s in range(n_seg):
            xs = x[:, s * seg_len:(s + 1) * seg_len, :].copy()
            h = jnp.concatenate([mem, xs], axis=1)
            q = jnp.einsum('btd,dhe->bhte', h, Wq)
            k = jnp.einsum('btd,dhe->bhte', h, Wk)
            v = jnp.einsum('btd,dhe->bhte', h, Wv)
            scores = jnp.einsum('bhqe,bhke->bhqk', q, k) * scale
            scores = jnp.where(mask[None, None], scores, -1000000000.0)
            p = _softmax(scores, axis=-1)
            o = jnp.einsum('bhqk,bhke->bhqe', p, v)
            o = jnp.einsum('bhte,hed->btd', o, Wo)
            mem = o[:, :M, :].copy()
            outs.append(o[:, M:, :])
        return jnp.concatenate(outs, axis=1)

    def _B_ref(x, w_gate, w_up, w_down):
        g = jnp.einsum('bsd,df->bsf', x, w_gate)
        u = jnp.einsum('bsd,df->bsf', x, w_up)
        h = _sigmoid(g) * u
        return jnp.einsum('bsf,fd->bsd', h, w_down)
    x = A_x
    x = x + _A_ref(_layernorm(x, axis=-1), A_mem0, A_Wq, A_Wk, A_Wv, A_Wo, A_seg_len)
    x = x + _B_ref(_layernorm(x, axis=-1), B_w_gate, B_w_up, B_w_down)
    x = x + _A_ref(_layernorm(x, axis=-1), A_mem0, A_Wq, A_Wk, A_Wv, A_Wo, A_seg_len)
    x = x + _B_ref(_layernorm(x, axis=-1), B_w_gate, B_w_up, B_w_down)
    return x
```

```python
import functools
import jax
import jax.numpy as jnp
import numpy as np
import jax.experimental.pallas as pl
import jax.experimental.pallas.tpu as pltpu

F32, BF16 = jnp.float32, jnp.bfloat16
CFG = dict(d=4, hg=8, fc=512, padk=True)


def _ln(x):
    m = jnp.mean(x, axis=-1, keepdims=True)
    c = x - m
    v = jnp.mean(c * c, axis=-1, keepdims=True)
    return c * jax.lax.rsqrt(v + 1e-5)


def _dot(a, b):
    return jnp.dot(a, b, preferred_element_type=F32)


def _dot_nt(a, b):
    return jax.lax.dot_general(a, b, (((1,), (1,)), ((), ())), preferred_element_type=F32)


def build(S, D, H, E, M, T, F, cfg):
    d, hg, fc = cfg["d"], cfg["hg"], cfg["fc"]
    nseg = S // T
    nch = nseg // d
    C = d * T
    R = 2 * (M + T)
    scale = float(E) ** -0.5

    def kern(x_hbm, mem_ref, wq, wk, wv, wo_hbm, wg_hbm, wu_hbm, wd_hbm, out_hbm,
             xs, stage, wqkv, wo, wg, wu, wd, hbuf, obuf, fbuf, xa, bn, xb, hn, yb, sems, wsem, osem):
        ws = (wq, wk, wv)

        def cp(j, m):
            return pltpu.make_async_copy(ws[m].bitcast(jnp.uint32).at[:, j, :], stage.at[j * 3 + m], sems.at[j * 3 + m])
        big = [pltpu.make_async_copy(s, t, wsem.at[i]) for i, (s, t) in enumerate(
            ((x_hbm, xs), (wo_hbm, wo), (wg_hbm, wg), (wu_hbm, wu), (wd_hbm, wd)))]
        big[0].start()
        for j in range(H // 2):
            for m in range(3):
                cp(j, m).start()
        for c in big[1:]:
            c.start()
        xb[...] = jnp.zeros_like(xb)
        hn[...] = jnp.zeros_like(hn)

        def relayout(j, c):
            for m in range(3):
                cp(j, m).wait()
                ev = stage[j * 3 + m, pl.ds(0, D // 2, stride=2), :]
                od = stage[j * 3 + m, pl.ds(1, D // 2, stride=2), :]
                lo = (ev & 0xFFFF) | (od << 16)
                hi = (ev >> 16) | (od & np.uint32(0xFFFF0000))
                wqkv[2 * j, :, m * E:(m + 1) * E] = pltpu.bitcast(lo, BF16)
                wqkv[2 * j + 1, :, m * E:(m + 1) * E] = pltpu.bitcast(hi, BF16)
            return c
        jax.lax.fori_loop(0, H // 2, relayout, 0)
        for c in big:
            c.wait()
        mem0 = mem_ref[...].astype(F32)
        hbuf[0:2 * M, :] = jnp.concatenate([mem0, mem0], axis=0).astype(BF16)
        hbuf[2 * M:2 * M + T, :] = _ln(xs[0:T, :].astype(F32)).astype(BF16)
        hbuf[2 * M + T:R, :] = jnp.zeros((T, D), BF16)

        def a_step(c, i):
            t = c * d + i
            KP = 128 if cfg["padk"] else R
            r = jax.lax.broadcasted_iota(jnp.int32, (R, KP), 0)
            k = jax.lax.broadcasted_iota(jnp.int32, (R, KP), 1)

            def info(a):
                ismem = a < 2 * M
                lay = jnp.where(ismem, a // M, (a - 2 * M) // T)
                pos = jnp.where(ismem, a % M, M + (a - 2 * M) % T)
                return lay, pos
            rl, rp = info(r)
            kl, kp = info(k)
            same = rl == kl
            valid = same & ((rp < M) | (rp >= kp))
            fill = jnp.where(same, -1e9, -jnp.inf).astype(F32)
            h = hbuf[...]

            def qkv(hd):
                y = _dot(h, wqkv[hd])
                return (y[:, :E] * scale).astype(BF16), y[:, E:2 * E].astype(BF16), y[:, 2 * E:].astype(BF16)

            def attn(hd, q, kk, v):
                if cfg["padk"]:
                    z = jnp.zeros((KP - R, E), BF16)
                    kk = jnp.concatenate([kk, z], axis=0)
                    v = jnp.concatenate([v, z], axis=0)
                s = jnp.where(valid, _dot_nt(q, kk), fill)
                p = jnp.exp(s - jnp.max(s, axis=-1, keepdims=True))
                l = jnp.sum(p, axis=-1, keepdims=True)
                o = _dot(p.astype(BF16), v) * (1.0 / l)
                obuf[:, hd * E:(hd + 1) * E] = o.astype(BF16)

            prev = None
            for hd in range(H):
                cur = qkv(hd)
                if prev is not None:
                    attn(hd - 1, *prev)
                prev = cur
            attn(H - 1, *prev)
            y = _dot(obuf[...], wo[...])
            r0 = pl.multiple_of(i * T, T)
            s1 = pl.multiple_of(jnp.minimum(t, nseg - 1) * T, T)
            x1 = xs[pl.ds(s1, T), :].astype(F32) + y[2 * M:2 * M + T]
            x3 = xb[0, pl.ds(r0, T), :] + y[2 * M + T:]
            xa[0, pl.ds(r0, T), :] = x1
            xa[1, pl.ds(r0, T), :] = x3
            bn[0, pl.ds(r0, T), :] = _ln(x1).astype(BF16)
            bn[1, pl.ds(r0, T), :] = _ln(x3).astype(BF16)
            m2 = jnp.where(t + 1 <= d, mem_ref[...].astype(F32), y[M:2 * M])
            hbuf[0:2 * M, :] = jnp.concatenate([y[0:M], m2], axis=0).astype(BF16)
            s2 = pl.multiple_of(jnp.minimum(t + 1, nseg - 1) * T, T)
            hbuf[2 * M:2 * M + T, :] = _ln(xs[pl.ds(s2, T), :].astype(F32)).astype(BF16)
            r1 = pl.multiple_of(jnp.minimum(i + 1, d - 1) * T, T)
            hbuf[2 * M + T:R, :] = hn[0, pl.ds(r1, T), :]

        def b_step(w):
            a = bn[w]
            for j in range(F // fc):
                g = _dot(a, wg[:, j * fc:(j + 1) * fc])
                u = _dot(a, wu[:, j * fc:(j + 1) * fc])
                fbuf[:, j * fc:(j + 1) * fc] = (jax.nn.sigmoid(g) * u).astype(BF16)
            y = xa[w] + _dot(fbuf[...], wd[...])
            xb[w] = y
            hn[w] = _ln(y).astype(BF16)
            yb[...] = y.astype(BF16)

        def ocp(c):
            return pltpu.make_async_copy(yb, out_hbm.at[pl.ds(pl.multiple_of(c * C, C), C), :], osem.at[0])

        def chunk(c, carry):
            def ab(i, cc):
                a_step(c, i)
                return cc
            jax.lax.fori_loop(0, d, ab, 0)

            @pl.when(c >= 2)
            def _():
                ocp(c - 2).wait()

            def bb(w, cc):
                b_step(w)
                return cc
            jax.lax.fori_loop(jnp.where(c < nch, 0, 1), jnp.where(c > 0, 2, 1), bb, 0)
            hbuf[2 * M + T:R, :] = hn[0, 0:T, :]

            @pl.when(c >= 1)
            def _():
                ocp(c - 1).start()
            return carry
        jax.lax.fori_loop(0, nch + 1, chunk, 0)
        ocp(nch - 1).wait()

    any_spec = pl.BlockSpec(memory_space=pl.ANY)
    return pl.pallas_call(
        kern,
        out_shape=jax.ShapeDtypeStruct((S, D), BF16),
        in_specs=[any_spec, pl.BlockSpec(memory_space=pltpu.VMEM)] + [any_spec] * 7,
        out_specs=any_spec,
        scratch_shapes=[
            pltpu.VMEM((S, D), BF16), pltpu.VMEM((3 * H // 2, D, E), jnp.uint32), pltpu.VMEM((H, D, 3 * E), BF16),
            pltpu.VMEM((H * E, D), BF16), pltpu.VMEM((D, F), BF16), pltpu.VMEM((D, F), BF16), pltpu.VMEM((F, D), BF16),
            pltpu.VMEM((R, D), BF16), pltpu.VMEM((R, H * E), BF16), pltpu.VMEM((C, F), BF16),
            pltpu.VMEM((2, C, D), F32), pltpu.VMEM((2, C, D), BF16), pltpu.VMEM((2, C, D), F32), pltpu.VMEM((2, C, D), BF16),
            pltpu.VMEM((C, D), BF16),
            pltpu.SemaphoreType.DMA((3 * H // 2,)), pltpu.SemaphoreType.DMA((5,)), pltpu.SemaphoreType.DMA((1,)),
        ],
        compiler_params=pltpu.CompilerParams(vmem_limit_bytes=120 * 2**20),
    )


@functools.partial(jax.jit, static_argnames=("A_seg_len",))
def pallas_interleave_layers__memory_aug_recurrent_mem_tr__glu_gated_glu__prompt_kernel(
        A_x, A_mem0, A_Wq, A_Wk, A_Wv, A_Wo, A_seg_len, B_x, B_w_gate, B_w_up, B_w_down):
    del B_x
    B, S, D = A_x.shape
    H, E = A_Wq.shape[1:]
    M = A_mem0.shape[1]
    F = B_w_gate.shape[1]
    call = build(S, D, H, E, M, int(A_seg_len), F, CFG)
    out = call(A_x.reshape(S, D), A_mem0.reshape(M, D), A_Wq, A_Wk, A_Wv, A_Wo.reshape(H * E, D),
               B_w_gate, B_w_up, B_w_down)
    return out.reshape(B, S, D)
```

```python
import functools
import jax
import jax.numpy as jnp
import numpy as np
import jax.experimental.pallas as pl
import jax.experimental.pallas.tpu as pltpu

F32, BF16, U32 = jnp.float32, jnp.bfloat16, jnp.uint32
CFG = dict(d=4, lag=2)

S11, S12, S21, S22 = 1, 2, 3, 4


def _ln(x):
    m = jnp.mean(x, axis=-1, keepdims=True)
    c = x - m
    v = jnp.mean(c * c, axis=-1, keepdims=True)
    return c * jax.lax.rsqrt(v + 1e-5)


def _dot(a, b):
    return jax.lax.dot_general(a, b, (((1,), (0,)), ((), ())), preferred_element_type=F32)


def _dot_nt(a, b):
    return jax.lax.dot_general(a, b, (((1,), (1,)), ((), ())), preferred_element_type=F32)


def _lhs7(a11, a12, a21, a22):
    return (a11 + a22, a21 + a22, a11, a22, a11 + a12, a21 - a11, a12 - a22)


def _rhs7(b11, b12, b21, b22):
    return (b11 + b22, b11, b12 - b22, b21 - b11, b22, b11 + b12, b21 + b22)


def _mm7(lhs, rhs):
    m = _dot(lhs(0), rhs(0))
    c11 = c22 = m
    m = _dot(lhs(1), rhs(1))
    c21, c22 = m, c22 - m
    m = _dot(lhs(2), rhs(2))
    c12, c22 = m, c22 + m
    m = _dot(lhs(3), rhs(3))
    c11, c21 = c11 + m, c21 + m
    m = _dot(lhs(4), rhs(4))
    c11, c12 = c11 - m, c12 + m
    c22 = c22 + _dot(lhs(5), rhs(5))
    c11 = c11 + _dot(lhs(6), rhs(6))
    return c11, c12, c21, c22


def _mm4(lhs, rhs):
    m5 = _dot(lhs(4), rhs(4))
    c12 = _dot(lhs(2), rhs(2)) + m5
    c11 = _dot(lhs(2), rhs(0)) - m5
    c11 = c11 + _dot(lhs(6), rhs(6))
    return c11, c12


def _lo(w):
    return pltpu.bitcast(w << 16, F32)


def _hi(w):
    return pltpu.bitcast(w & np.uint32(0xFFFF0000), F32)


def _pack(lo, hi):
    return pltpu.bitcast(pltpu.pack_elementwise([lo, hi], packed_dtype=BF16), U32)


def _bf(w):
    return pltpu.bitcast(w, BF16)


def _u(x):
    return pltpu.bitcast(x.astype(BF16), U32)


def build(S, D, H, E, M, T, F, cfg):
    d = cfg["d"]
    nseg = S // T
    nch = nseg // d
    C = d * T
    L = M + T
    P = H // 2
    D2, D4, F2, C2 = D // 2, D // 4, F // 2, C // 2
    scale = float(E) ** -0.5

    def kern(x_hbm, mem_ref, wq, wk, wv, wo_hbm, wg_hbm, wu_hbm, wd_hbm, out_hbm,
             xs, wqkv, wo, wg, wu, wd, hs, ha, oa, ba, fa, xa, xb, hn, yb, qsem, wsem, osem):
        def qkv_copies(j):
            return [pltpu.make_async_copy(w.bitcast(U32).at[pl.ds(hf * D4, D4), par, j, :],
                                          wqkv.at[j, m, 2 * hf + par], qsem.at[j])
                    for m, w in enumerate((wq, wk, wv)) for hf in range(2) for par in range(2)]

        def quad_copies(src, dst, sem):
            return [pltpu.make_async_copy(src(r, c), dst.at[s], sem)
                    for r, c, s in ((0, 0, S11), (0, 1, S12), (1, 0, S21), (1, 1, S22))]
        wo_cp = quad_copies(lambda r, c: wo_hbm.bitcast(U32).at[:, r, :, pl.ds(c * D2, D2)], wo, wsem.at[0])
        wg_cp = quad_copies(lambda r, c: wg_hbm.bitcast(U32).at[pl.ds(r * D4, D4), pl.ds(c * F2, F2)], wg, wsem.at[1])
        wu_cp = quad_copies(lambda r, c: wu_hbm.bitcast(U32).at[pl.ds(r * D4, D4), pl.ds(c * F2, F2)], wu, wsem.at[2])
        wd_cp = quad_copies(lambda r, c: wd_hbm.bitcast(U32).at[pl.ds(r * (F // 4), F // 4), pl.ds(c * D2, D2)], wd, wsem.at[3])
        x_cp = pltpu.make_async_copy(x_hbm, xs, wsem.at[4])
        for j in range(P):
            for cp in qkv_copies(j):
                cp.start()
        x_cp.start()
        for cp in wo_cp + wg_cp + wu_cp + wd_cp:
            cp.start()

        def prep_qkv(j, carry):
            for cp in qkv_copies(j):
                cp.wait()
            for m in range(3):
                for r in range(0, D4, 32):
                    te, to, be, bo = (wqkv[j, m, s, r:r + 32, :] for s in range(4))
                    ev = _rhs7(_lo(te), _hi(te), _lo(be), _hi(be))
                    od = _rhs7(_lo(to), _hi(to), _lo(bo), _hi(bo))
                    for s in range(7):
                        wqkv[j, m, s, r:r + 32, :] = _pack(ev[s], od[s])
            return carry

        def prep(w, idx):
            q = [w[(s,) + idx] for s in (S11, S12, S21, S22)]
            lo = _rhs7(*[_lo(v) for v in q])
            hi = _rhs7(*[_hi(v) for v in q])
            for s in (0, 2, 3, 5, 6):
                w[(s,) + idx] = _pack(lo[s], hi[s])

        def prep_rows(w, cps, step):
            for cp in cps:
                cp.wait()

            def body(r, carry):
                prep(w, (pl.ds(pl.multiple_of(r * step, step), step), slice(None)))
                return carry
            jax.lax.fori_loop(0, w.shape[1] // step, body, 0)

        jax.lax.fori_loop(0, P, prep_qkv, 0)
        x_cp.wait()
        for cp in wo_cp:
            cp.wait()

        def prep_wo(j, carry):
            prep(wo, (j, slice(None), slice(None)))
            return carry
        jax.lax.fori_loop(0, P, prep_wo, 0)

        def seg(ref, i):
            return ref[pl.ds(pl.multiple_of(i * T, T), T), :]

        def put7(ref, vals, rows, cols, which=range(7)):
            for s in which:
                ref[s, rows, cols] = vals[s]

        def put_h(top, bot, rows):
            if bot is None:
                a11, a12 = top[:, :D2], top[:, D2:]
                put7(ha, {2: a11, 4: a11 + a12, 6: a12}, rows, slice(None), (2, 4, 6))
            else:
                put7(ha, _lhs7(top[:, :D2], top[:, D2:], bot[:, :D2], bot[:, D2:]), rows, slice(None))

        def attn_masks():
            r = jax.lax.broadcasted_iota(jnp.int32, (2 * L, 128), 0)
            k = jax.lax.broadcasted_iota(jnp.int32, (2 * L, 128), 1)
            rp = jnp.where(r < L, r, r - L)
            kp = jnp.where(r < L, k, k - L)
            same = (kp >= 0) & (kp < L)
            valid = same & ((rp < M) | (rp >= kp))
            return valid, jnp.where(same, -1e9, -jnp.inf).astype(F32)

        def attn(q, k, v, valid, fill):
            z = jnp.zeros((128 - 2 * L, E), BF16)
            k = jnp.concatenate([k, z], axis=0)
            v = jnp.concatenate([v, z], axis=0)
            s = jnp.where(valid, _dot_nt(q, k), fill)
            p = jnp.exp(s - jnp.max(s, axis=-1, keepdims=True))
            return _dot(p, v) / jnp.sum(p, axis=-1, keepdims=True)

        def a_core(dual):
            valid, fill = attn_masks()
            mm = _mm7 if dual else _mm4

            def proj(j):
                res = []
                for m in range(3):
                    c = mm(lambda s: ha[s], lambda s: _bf(wqkv[j, m, s]))
                    c = ([jnp.concatenate([c[0], c[2]], axis=0), jnp.concatenate([c[1], c[3]], axis=0)] if dual
                         else [jnp.concatenate(c, axis=0)])
                    res.append([y * scale if m == 0 else y.astype(BF16) for y in c])
                return res

            def finish(j, qkv):
                o = [attn(q, k, v, valid, fill) for q, k, v in zip(*qkv)]
                cols = slice(j * E, (j + 1) * E)
                if dual:
                    put7(oa, _lhs7(o[0][:L], o[1][:L], o[0][L:], o[1][L:]), slice(None), cols)
                else:
                    a11, a12 = o[0][:L], o[0][L:]
                    put7(oa, {2: a11, 4: a11 + a12, 6: a12}, slice(None), cols, (2, 4, 6))

            pend = []
            for j in range(P):
                pend.append((j, proj(j)))
                if len(pend) > cfg["lag"]:
                    finish(*pend.pop(0))
            for p_ in pend:
                finish(*p_)
            cs = [mm(lambda s: oa[s], lambda s: _bf(wo[s, :, :, c:c + 128].reshape(P * E // 2, 128)))
                  for c in range(0, D2, 128)]
            top = jnp.concatenate([c[0] for c in cs] + [c[1] for c in cs], axis=1)
            bot = jnp.concatenate([c[2] for c in cs] + [c[3] for c in cs], axis=1) if dual else None
            return top, bot

        mrows, trows = slice(0, M), slice(M, L)

        def a_dual(c, i):
            t = c * d + i
            top, bot = a_core(True)
            rows = pl.ds(pl.multiple_of(i * T, T), T)
            xa[0, rows, :] = seg(xs, t).astype(F32) + top[M:]
            xa[1, rows, :] = xb[0, rows, :] + bot[M:]
            hs[0], hs[1] = top[:M], bot[:M]
            put_h(top[:M], bot[:M], mrows)
            put_h(_ln(seg(xs, jnp.minimum(t + 1, nseg - 1)).astype(F32)),
                  seg(hn.at[0], jnp.minimum(i + 1, d - 1)), trows)

        def a_single(w, i):
            top, _ = a_core(False)
            rows = pl.ds(pl.multiple_of(i * T, T), T)
            xa[w, rows, :] = xb[0, rows, :] + top[M:]
            hs[0] = top[:M]
            put_h(top[:M], None, mrows)
            put_h(seg(hn.at[0], jnp.minimum(i + 1, d - 1)), None, trows)

        def b_step(w):
            a = _ln(xa[w])
            put7(ba, [_u(v) for v in _lhs7(a[:C2, :D2], a[:C2, D2:], a[C2:, :D2], a[C2:, D2:])], slice(None), slice(None))
            for c in range(0, F2, 128):
                g = _mm7(lambda s: _bf(ba[s]), lambda s: _bf(wg[s, :, c:c + 128]))
                u = _mm7(lambda s: _bf(ba[s]), lambda s: _bf(wu[s, :, c:c + 128]))
                h = [jax.nn.sigmoid(gg) * uu for gg, uu in zip(g, u)]
                put7(fa, [_u(v) for v in _lhs7(*h)], slice(None), slice(c, c + 128))
            cs = [_mm7(lambda s: _bf(fa[s]), lambda s: _bf(wd[s, :, c:c + 128])) for c in range(0, D2, 128)]
            y = jnp.concatenate([jnp.concatenate([c[0] for c in cs] + [c[1] for c in cs], axis=1),
                                 jnp.concatenate([c[2] for c in cs] + [c[3] for c in cs], axis=1)], axis=0)
            y = xa[w] + y
            xb[w] = y
            hn[w] = _ln(y)
            yb[...] = y.astype(BF16)

        def ocp(c):
            return pltpu.make_async_copy(yb, out_hbm.at[pl.ds(pl.multiple_of(c * C, C), C), :], osem.at[0])

        x0 = xs[0:C, :].astype(F32)
        xb[0] = x0
        hn[0] = _ln(x0)
        hs[0] = mem_ref[...].astype(F32)

        def chunk(c, carry):
            edge = (c == 0) | (c == nch)

            @pl.when(edge)
            def _():
                w = jnp.where(c == 0, 0, 1)
                put_h(hs[w], None, mrows)
                put_h(hn[0, 0:T, :], None, trows)
                jax.lax.fori_loop(0, d, lambda i, cc: (a_single(w, i), cc)[1], 0)
                hs[1] = mem_ref[...].astype(F32)

            @pl.when(jnp.logical_not(edge))
            def _():
                put_h(hs[0], hs[1], mrows)
                put_h(_ln(seg(xs, c * d).astype(F32)), hn[0, 0:T, :], trows)
                jax.lax.fori_loop(0, d, lambda i, cc: (a_dual(c, i), cc)[1], 0)

            @pl.when(c == 0)
            def _():
                prep_rows(wg, wg_cp, 16)
                prep_rows(wu, wu_cp, 16)
                prep_rows(wd, wd_cp, 64)

            @pl.when(c >= 2)
            def _():
                ocp(c - 2).wait()

            jax.lax.fori_loop(jnp.where(c < nch, 0, 1), jnp.where(c > 0, 2, 1), lambda w, cc: (b_step(w), cc)[1], 0)

            @pl.when(c >= 1)
            def _():
                ocp(c - 1).start()
            return carry
        jax.lax.fori_loop(0, nch + 1, chunk, 0)
        ocp(nch - 1).wait()

    any_spec = pl.BlockSpec(memory_space=pl.ANY)
    V = pltpu.VMEM
    return pl.pallas_call(
        kern,
        out_shape=jax.ShapeDtypeStruct((S, D), BF16),
        in_specs=[any_spec, pl.BlockSpec(memory_space=pltpu.VMEM)] + [any_spec] * 7,
        out_specs=any_spec,
        scratch_shapes=[
            V((S, D), BF16), V((P, 3, 7, D4, E), U32), V((7, P, E // 2, D2), U32),
            V((7, D4, F2), U32), V((7, D4, F2), U32), V((7, F // 4, D2), U32),
            V((2, M, D), F32), V((7, L, D2), F32), V((7, L, P * E), F32),
            V((7, C2 // 2, D2), U32), V((7, C2 // 2, F2), U32),
            V((2, C, D), F32), V((2, C, D), F32), V((2, C, D), F32), V((C, D), BF16),
            pltpu.SemaphoreType.DMA((P,)), pltpu.SemaphoreType.DMA((5,)), pltpu.SemaphoreType.DMA((1,)),
        ],
        compiler_params=pltpu.CompilerParams(vmem_limit_bytes=126 * 2**20),
    )


@functools.partial(jax.jit, static_argnames=("A_seg_len",))
def pallas_interleave_layers__memory_aug_recurrent_mem_tr__glu_gated_glu__prompt_kernel(
        A_x, A_mem0, A_Wq, A_Wk, A_Wv, A_Wo, A_seg_len, B_x, B_w_gate, B_w_up, B_w_down):
    del B_x
    B, S, D = A_x.shape
    H, E = A_Wq.shape[1:]
    M = A_mem0.shape[1]
    F = B_w_gate.shape[1]
    call = build(S, D, H, E, M, int(A_seg_len), F, CFG)
    out = call(A_x.reshape(S, D), A_mem0.reshape(M, D), A_Wq.reshape(D // 2, 2, H, E), A_Wk.reshape(D // 2, 2, H, E),
               A_Wv.reshape(D // 2, 2, H, E), A_Wo.reshape(H // 2, 2, E, D),
               B_w_gate, B_w_up, B_w_down)
    return out.reshape(B, S, D)
```

```python
import contextlib
import functools
import jax
import jax.numpy as jnp
import numpy as np
import jax.experimental.pallas as pl
import jax.experimental.pallas.tpu as pltpu

F32, BF16, U32 = jnp.float32, jnp.bfloat16, jnp.uint32
CFG = dict(d=4, so=1, po=3, kc=[4, 4, 4, 4], keep=5, om=2, nt=1, kf=12, anc=-1, ba=1, nf=1, bj=[2, 6], bk=[3, 7], ahead=3, og=2)

S11, S12, S21, S22 = 1, 2, 3, 4


def _ln(x):
    m = jnp.mean(x, axis=-1, keepdims=True)
    c = x - m
    v = jnp.mean(c * c, axis=-1, keepdims=True)
    return c * jax.lax.rsqrt(v + 1e-5)


def _sigmoid(x):
    return 0.5 * jnp.tanh(0.5 * x) + 0.5


def _dot(a, b):
    return jax.lax.dot_general(a, b, (((1,), (0,)), ((), ())), preferred_element_type=F32)


def _dot_nt(a, b):
    return jax.lax.dot_general(a, b, (((1,), (1,)), ((), ())), preferred_element_type=F32)


def _lhs7(a11, a12, a21, a22):
    return (a11 + a22, a21 + a22, a11, a22, a11 + a12, a21 - a11, a12 - a22)


def _rhs7(b11, b12, b21, b22):
    return (b11 + b22, b11, b12 - b22, b21 - b11, b22, b11 + b12, b21 + b22)


def _mm7(lhs, rhs):
    m = _dot(lhs(0), rhs(0))
    c11 = c22 = m
    m = _dot(lhs(1), rhs(1))
    c21, c22 = m, c22 - m
    m = _dot(lhs(2), rhs(2))
    c12, c22 = m, c22 + m
    m = _dot(lhs(3), rhs(3))
    c11, c21 = c11 + m, c21 + m
    m = _dot(lhs(4), rhs(4))
    c11, c12 = c11 - m, c12 + m
    c22 = c22 + _dot(lhs(5), rhs(5))
    c11 = c11 + _dot(lhs(6), rhs(6))
    return c11, c12, c21, c22


def _mm4(lhs, rhs):
    m5 = _dot(lhs(4), rhs(4))
    c12 = _dot(lhs(2), rhs(2)) + m5
    c11 = _dot(lhs(2), rhs(0)) - m5
    c11 = c11 + _dot(lhs(6), rhs(6))
    return c11, c12


def _lo(w):
    return pltpu.bitcast(w << 16, F32)


def _hi(w):
    return pltpu.bitcast(w & np.uint32(0xFFFF0000), F32)


def _pack(lo, hi):
    return pltpu.bitcast(pltpu.pack_elementwise([lo, hi], packed_dtype=BF16), U32)


def _bf(w):
    return pltpu.bitcast(w, BF16)


def _u(x):
    return pltpu.bitcast(x.astype(BF16), U32)


def build(S, D, H, E, M, T, F, cfg):
    d = cfg["d"]
    nseg = S // T
    nch = nseg // d
    C = d * T
    L = M + T
    P = H // 2
    OG = cfg['og']
    D2, D4, F2, C2 = D // 2, D // 4, F // 2, C // 2
    T2 = T // 2
    KD, KF = D2 // 128, F2 // 128
    scale = float(E) ** -0.5
    scope = jax.named_scope if cfg.get('prof') else (lambda n: contextlib.nullcontext())

    def loop(lo, hi, fn, name):
        def body(i, carry):
            with scope(name):
                fn(i)
            return carry
        jax.lax.fori_loop(lo, hi, body, 0)

    def kern(x_hbm, mem_ref, wq, wk, wv, wo_hbm, wg_hbm, wu_hbm, wd_hbm, out_hbm,
             xs, wqkv, wo, wg, wu, wd, mem, ha, ba, fa, xa, xb, yb, qsem, osem, wsem, ysem):
        quads = ((0, 0, S11), (0, 1, S12), (1, 0, S21), (1, 1, S22))

        def qkv_copies(j):
            return [pltpu.make_async_copy(w.bitcast(U32).at[pl.ds(hf * D4, D4), par, j, :],
                                          wqkv.at[j, m, 2 * hf + par], qsem.at[j])
                    for m, w in enumerate((wq, wk, wv)) for hf in range(2) for par in range(2)]

        def wo_copies(g):
            js = pl.ds(g * OG, OG)
            return [pltpu.make_async_copy(wo_hbm.bitcast(U32).at[js, r, :, pl.ds(c * D2, D2)], wo.at[s, js], osem.at[g])
                    for r, c, s in quads]

        def b_copies(src, dst, k):
            nr, nc = dst.shape[1:]
            return [pltpu.make_async_copy(src.bitcast(U32).at[pl.ds(r * nr, nr), pl.ds(c * nc, nc)], dst.at[s], wsem.at[k])
                    for r, c, s in quads]
        b_cps = [b_copies(wg_hbm, wg, 0), b_copies(wu_hbm, wu, 1), b_copies(wd_hbm, wd, 2)]
        x_cps = [pltpu.make_async_copy(x_hbm.at[0:C], xs.at[0:C], wsem.at[3]),
                 pltpu.make_async_copy(x_hbm.at[C:S], xs.at[C:S], wsem.at[4])]

        def start(cps):
            for cp in cps:
                cp.start()

        def wait(cps):
            for cp in cps:
                cp.wait()

        def prep_qkv(j):
            for m in range(3):
                for r in range(0, D4, 32):
                    te, to, be, bo = (wqkv[j, m, s, r:r + 32, :] for s in range(4))
                    ev = _rhs7(_lo(te), _hi(te), _lo(be), _hi(be))
                    od = _rhs7(_lo(to), _hi(to), _lo(bo), _hi(bo))
                    for s in range(7):
                        wqkv[j, m, s, r:r + 32, :] = _pack(ev[s], od[s])

        def prep(w, idx):
            q = [w[(s,) + idx] for s in (S11, S12, S21, S22)]
            lo = _rhs7(*[_lo(v) for v in q])
            hi = _rhs7(*[_hi(v) for v in q])
            for s in (0, 2, 3, 5, 6):
                w[(s,) + idx] = _pack(lo[s], hi[s])

        def prep_rows(w, step):
            def body(r):
                for c in range(0, w.shape[2], 128):
                    prep(w, (pl.ds(pl.multiple_of(r * step, step), step), slice(c, c + 128)))
            loop(0, w.shape[1] // step, body, "z_prepb")

        def seg(ref, i):
            return ref[pl.ds(pl.multiple_of(i * T, T), T), :]

        def lhs(a11, a12, a21=None, a22=None):
            if a21 is None:
                return {2: a11, 4: a11 + a12, 6: a12}
            return dict(enumerate(_lhs7(a11, a12, a21, a22)))

        def put(ref, t0, rows, v):
            for k in range(v.shape[1] // 128):
                ref[t0 + k, rows, :] = v[:, k * 128:(k + 1) * 128]

        def get(ref, t0, n, nrows, after=None):
            ts = [ref[t0 + k, 0:nrows, :] for k in range(n)]
            if after is not None:
                head = jnp.where(after[1] == 0, ts[0][0:8], after[0][after[1], 0:8, :])
                ts[0] = jnp.concatenate([head, ts[0][8:]], axis=0)
            return jnp.concatenate(ts, axis=1)

        def put_h(rows, *blocks):
            for s, v in lhs(*[y for x in blocks for y in (x[:, :D2], x[:, D2:])]).items():
                put(ha, (s if len(blocks) == 2 else s // 2 - 1) * KD, rows, v)

        def attn_masks():
            r = jax.lax.broadcasted_iota(jnp.int32, (2 * L, 128), 0)
            k = jax.lax.broadcasted_iota(jnp.int32, (2 * L, 128), 1)
            rp = jnp.where(r < L, r, r - L)
            kp = jnp.where(r < L, k, k - L)
            same = (kp >= 0) & (kp < L)
            valid = same & ((rp < M) | (rp >= kp))
            return valid, jnp.where(same, -1e9, -jnp.inf).astype(F32)

        def proj(j, m, dual, after=None):
            c = (_mm7 if dual else _mm4)(lambda s: get(ha, (s if dual else s // 2 - 1) * KD, KD, L, after if s == 6 else None), lambda s: _bf(wqkv[j, m, s]))
            c = ([jnp.concatenate([c[0], c[2]], axis=0), jnp.concatenate([c[1], c[3]], axis=0)] if dual
                 else [jnp.concatenate(c, axis=0)])
            if m == 0:
                return [y * scale for y in c]
            z = jnp.zeros((128 - 2 * L, E), BF16)
            return [jnp.concatenate([y.astype(BF16), z], axis=0) for y in c]

        def probs(qs, ks, masks):
            res = []
            for q, k in zip(qs, ks):
                s = jnp.where(masks[0], _dot_nt(q, k), masks[1])
                p = jnp.exp(s - jnp.max(s, axis=-1, keepdims=True))
                l = jnp.sum(p, axis=-1, keepdims=True)
                r = pl.reciprocal(l, approx=True)
                r = r * (2.0 - l * r)
                res.append((p, r * (2.0 - l * r)))
            return res

        def mix(j, ps, vs):
            o = [_dot(p, v) * r for (p, r), v in zip(ps, vs)]
            parts = (o[0][:L], o[1][:L], o[0][L:], o[1][L:]) if len(o) == 2 else (o[0][:L], o[0][L:])
            for s, v in lhs(*parts).items():
                fa[s * P + j, 0:L, :] = v

        def out_proj(j0, n, c, dual, after=None):
            return (_mm7 if dual else _mm4)(
                lambda s: get(fa, s * P + j0, n, L, after if s == 6 else None),
                lambda s: _bf(wo[s, pl.ds(j0, n), :, c:c + 128].reshape(n * E // 2, 128)))

        def gather(cs):
            return [jnp.concatenate([c[k] for c in cs] + [c[k + 1] for c in cs], axis=1)
                    for k in range(0, len(cs[0]), 2)]

        mrows, trows = slice(0, M), slice(M, L)

        def a_step(dual, zero, extra, next_tokens, residual):
            masks = attn_masks()
            so, po, kc = cfg["so"], cfg["po"], cfg["kc"]
            pr, ps, acc = {}, {}, {}
            side = sorted([(3 * j + 1 + so, 0, j) for j in range(P)] + [(3 * j + 1 + so + po, 1, j) for j in range(P)]
                          + [(cfg["nt"] + 3 * P - 1, 2, 0)])
            done = [0]

            def run_side(now):
                while side and side[0][0] <= now:
                    _, kind, j = side.pop(0)
                    if kind == 0:
                        ps[j] = probs(pr[j, 0], pr[j, 1], masks)
                    elif kind == 1:
                        mix(j, ps[j], pr[j, 2])
                        done[0] = j + 1
                    else:
                        put_h(trows, *next_tokens())
            outs = [(j0, n, c) for j0, n in zip(np.cumsum([0] + kc[:-1]).tolist(), kc) for c in range(0, D2, 128)]

            def run_out():
                j0, n, c = outs.pop(0)
                assert j0 + n <= done[0]
                y = out_proj(j0, n, c, dual, (ha, zero) if len(outs) == cfg['anc'] else None)
                acc[c] = [u + v for u, v in zip(acc[c], y)] if j0 else list(y)
                if j0 + n == P:
                    finish_cols(c, acc[c], residual)
            keep = 4 + cfg["keep"]
            for j in range(P):
                for m in range(3):
                    if m == 0 and j in cfg["bj"][:len(extra)]:
                        extra[cfg["bj"].index(j)]()
                    pr[j, m] = proj(j, m, dual, (ba, zero) if m == 2 and j in cfg["bk"] else None)
                    run_side(3 * j + m)
                    if len(outs) > keep and outs[0][0] + outs[0][1] <= done[0] and m == cfg["om"]:
                        run_out()
            now = 3 * P - 1
            while outs:
                run_out()
                now += 1
                run_side(now)
            run_side(10 ** 6)

        def finish_cols(c, y, residual):
            for s, v in lhs(*[b[:M] for b in y]).items():
                ha[(s if len(y) == 4 else s // 2 - 1) * KD + c // 128, mrows, :] = v
            for k, b in enumerate(y):
                cols = slice(c + (k % 2) * D2, c + (k % 2) * D2 + 128)
                mem[k // 2, :, cols] = b[:M]
                residual(k // 2, cols, b[M:])

        def a_dual(c, i):
            t = c * d + i
            rows = pl.ds(pl.multiple_of(i * T, T), T)
            xrows = pl.ds(pl.multiple_of(t * T, T), T)

            def residual(layer, cols, v):
                xa[layer, rows, cols] = v + (xb[0, rows, cols] if layer else xs[xrows, cols].astype(F32))
            a_step(True, i // d, [lambda: b_head(0, (i + d - 1) % d), lambda: b_head(1, (i + d - 1) % d)], lambda: (_ln(seg(xs, jnp.minimum(t + 1, nseg - 1)).astype(F32)),
                                  _ln(seg(xb.at[0], jnp.minimum(i + 1, d - 1)))), residual)

        def single_io(w, i):
            rows = pl.ds(pl.multiple_of(i * T, T), T)

            def residual(layer, cols, v):
                xa[w, rows, cols] = v + xb[0, rows, cols]
            return (lambda: (_ln(seg(xb.at[0], jnp.minimum(i + 1, d - 1))),)), residual

        def b_head(w, i):
            a = _ln(seg(xa.at[w], i))
            rows = pl.ds(pl.multiple_of(i * T2, T2), T2)
            for s, v in enumerate(_lhs7(a[:T2, :D2], a[:T2, D2:], a[T2:, :D2], a[T2:, D2:])):
                put(ba, (w * 7 + s) * KD, rows, v)

        def a_head(c, r0, nr):
            if r0 == 0:
                put_h(mrows, mem[0], mem[1])
            x1 = xs[pl.ds(pl.multiple_of(jnp.minimum(c * d, nseg - 1) * T + r0, nr), nr), :]
            put_h(slice(M + r0, M + r0 + nr), _ln(x1.astype(F32)), _ln(xb[0, r0:r0 + nr, :]))

        def b_step(c, w):
            zero = w // 2
            for n in range(KF):
                cols = slice(n * 128, (n + 1) * 128)
                aft = (ha, zero) if n - cfg['ba'] in range(T // 16) else None
                g = _mm7(lambda s: get(ba, (w * 7 + s) * KD, KD, C2), lambda s: _bf(wg[s, :, cols]))
                u = _mm7(lambda s: get(ba, (w * 7 + s) * KD, KD, C2, aft if s == 6 else None), lambda s: _bf(wu[s, :, cols]))
                for s, v in enumerate(_lhs7(*[_sigmoid(gg) * uu for gg, uu in zip(g, u)])):
                    fa[s * KF + n] = v
                if n < T // 16:
                    a_head(c + 1, n * 16, 16)
            kf = cfg["kf"]
            mm = lambda k0, nk, n: _mm7(lambda s: get(fa, s * KF + k0, nk, C2),
                                        lambda s: _bf(wd[s, k0 * 64:(k0 + nk) * 64, n:n + 128]))
            first = [mm(0, kf, n) for n in range(0, cfg["nf"] * 128, 128)]
            for n in list(range(len(first) * 128, D2, 128)) + list(range(0, len(first) * 128, 128)):
                y = mm(0, KF, n) if n // 128 >= len(first) else [u + v for u, v in zip(first[n // 128], mm(kf, KF - kf, n))]
                for k, v in enumerate(y):
                    c_ = slice(n + (k % 2) * D2, n + (k % 2) * D2 + 128)
                    for i in range(d):
                        r_ = slice(i * T + (k // 2) * T2, i * T + (k // 2 + 1) * T2)
                        r = v[i * T2:(i + 1) * T2] + xa[w, r_, c_]
                        xb[w, r_, c_] = r
                        yb[r_, c_] = r.astype(BF16)

        def y_copy(c):
            return pltpu.make_async_copy(yb, out_hbm.at[pl.ds(pl.multiple_of(c * C, C), C), :], ysem.at[0])

        AH = cfg["ahead"]
        with scope('z_head'):
            x_cps[0].start()
            for j in range(AH):
                start(qkv_copies(j))
            x_cps[0].wait()
        x0 = xs[0:C, :].astype(F32)
        xb[0] = x0
        mem[1] = mem_ref[...].astype(F32)
        put_h(mrows, mem[1])
        put_h(trows, _ln(xb[0, 0:T, :]))
        xa[1] = jnp.zeros((C, D), F32)
        ba[...] = jnp.zeros(ba.shape, F32)

        def first_qkv(j):
            @pl.when(j + AH < P)
            def _():
                start(qkv_copies(j + AH))

            @pl.when(j + AH == P)
            def _():
                for g in range(P // OG):
                    start(wo_copies(g))
            wait(qkv_copies(j))
            prep_qkv(j)
            mix(j, probs(proj(j, 0, False), proj(j, 1, False), attn_masks()), proj(j, 2, False))
        loop(0, P, first_qkv, "z_first")
        start(b_cps[0] + b_cps[1] + b_cps[2] + x_cps[1:])

        def first_out(g):
            wait(wo_copies(g))
            for j in range(OG):
                prep(wo, (g * OG + j, slice(None), slice(None)))
            xa[1, 0:L, :] += gather([out_proj(g * OG, OG, c, False) for c in range(0, D2, 128)])[0]
        loop(0, P // OG, first_out, "z_first_o")
        nxt, res = single_io(0, 0)
        put_h(trows, *nxt())
        for c in range(0, D2, 128):
            finish_cols(c, [xa[1, 0:L, c:c + 128], xa[1, 0:L, D2 + c:D2 + c + 128]], res)

        def chunk(c):
            edge = (c == 0) | (c == nch)
            w0 = jnp.where(c < nch, 0, 1)

            @pl.when(edge)
            def _():
                @pl.when(c == nch)
                def _():
                    put_h(mrows, mem[1])
                    put_h(trows, _ln(xb[0, 0:T, :]))
                loop(1 - w0, d, lambda i: a_step(False, i // d, [lambda: b_head(w0, (i + d - 1) % d)], *single_io(w0, i)), "z_single")
                b_head(w0, d - 1)

                @pl.when(c == 0)
                def _():
                    for cps, wt, step in zip(b_cps, (wg, wu, wd), (32, 32, 128)):
                        with scope('z_waitb'):
                            wait(cps)
                        prep_rows(wt, step)
                    x_cps[1].wait()

            @pl.when(jnp.logical_not(edge))
            def _():
                loop(0, d, lambda i: a_dual(c, i), "z_dual")
                with scope("z_bhead"):
                    b_head(0, d - 1)
                    b_head(1, d - 1)

            @pl.when(c >= 2)
            def _():
                y_copy(c - 2).wait()
            loop(w0, jnp.where(c > 0, 2, 1), lambda w: b_step(c, w), "z_b")

            @pl.when(c == 0)
            def _():
                a_head(1, 0, T)

            @pl.when(c >= 1)
            def _():
                y_copy(c - 1).start()
        loop(0, nch + 1, chunk, "z_chunk")
        y_copy(nch - 1).wait()

    any_spec = pl.BlockSpec(memory_space=pl.ANY)
    V = pltpu.VMEM
    return pl.pallas_call(
        kern,
        out_shape=jax.ShapeDtypeStruct((S, D), BF16),
        in_specs=[any_spec, pl.BlockSpec(memory_space=pltpu.VMEM)] + [any_spec] * 7,
        out_specs=any_spec,
        scratch_shapes=[
            V((S, D), BF16), V((P, 3, 7, D4, E), U32), V((7, P, E // 2, D2), U32),
            V((7, D4, F2), U32), V((7, D4, F2), U32), V((7, F // 4, D2), U32),
            V((2, M, D), F32), V((7 * KD, L, 128), F32), V((14 * KD, C2, 128), F32),
            V((7 * max(KF, P), C2, 128), F32), V((2, C, D), F32), V((2, C, D), F32), V((C, D), BF16),
            pltpu.SemaphoreType.DMA((P,)), pltpu.SemaphoreType.DMA((P // OG,)),
            pltpu.SemaphoreType.DMA((5,)), pltpu.SemaphoreType.DMA((1,)),
        ],
        compiler_params=pltpu.CompilerParams(vmem_limit_bytes=126 * 2**20),
    )


@functools.partial(jax.jit, static_argnames=("A_seg_len",))
def pallas_interleave_layers__memory_aug_recurrent_mem_tr__glu_gated_glu__prompt_kernel(
        A_x, A_mem0, A_Wq, A_Wk, A_Wv, A_Wo, A_seg_len, B_x, B_w_gate, B_w_up, B_w_down):
    del B_x
    B, S, D = A_x.shape
    H, E = A_Wq.shape[1:]
    M = A_mem0.shape[1]
    F = B_w_gate.shape[1]
    call = build(S, D, H, E, M, int(A_seg_len), F, CFG)
    out = call(A_x.reshape(S, D), A_mem0.reshape(M, D), A_Wq.reshape(D // 2, 2, H, E), A_Wk.reshape(D // 2, 2, H, E),
               A_Wv.reshape(D // 2, 2, H, E), A_Wo.reshape(H // 2, 2, E, D),
               B_w_gate, B_w_up, B_w_down)
    return out.reshape(B, S, D)
```

```python
import collections
import contextlib
import functools

import jax
import jax.experimental.pallas as pl
import jax.experimental.pallas.tpu as pltpu
import jax.numpy as jnp
import numpy as np

F32, BF16, U32 = jnp.float32, jnp.bfloat16, jnp.uint32
CFG = dict(d=4, so=1, po=3, kc=[2, 2, 3, 1], keep=2, om=[1], nt=1, kf=5, nf=1, ba=1, bj=[1, 3], bk=[1, 3],
           ahead=2, cse=True)

_SCHEME = (
    '+000+000 ++000000+0000000 0000+000', '+0000000 +0+0+00000000000 +000-000',
    '0+000+00 0000++0+0+000000 0+000000', '00000+00 0-000-+000000-00 0+000-00',
    '+-000000 0000-00000000000 +-000000', '0000+-00 0-00000000000000 0000+-00',
    '+0000+00 0-00+00000000000 0-00+000', '0+-00+-0 000000000-000000 00000++0',
    '0+-00000 000000+000000000 0++00--0', '0+-00+00 000000-00-000000 0+000--0',
    '0+0-0000 0000000-00000000 0+0-0000', '00000+0- 0000000000000-00 00000+0-',
    '000+0+00 0000000-00000+00 0+00000-', '00+00000 000+00+0+0++0000 00+00000',
    '000000+0 00+000000-+0-0-0 000000+0', '+0-0+0-0 000-0000-0000000 +0-00000',
    '0000+0-0 00+000000000+000 +0-0-0+0', '+000+0-0 00-00000+0000000 +0-0-000',
    '+0-+0000 000+000000000000 +0-+0000', '0000+0-+ 000000000000+000 0000+0-+',
    '000-+0-0 000+00000000-000 +0-0000+', '000+000+ 000-0000000--+0+ 0000000+',
    '000+0000 000-000+0000+0++ 000+000-', '00++00++ 000-0000000-0000 00+-0000',
    '000000++ 000000000000-0-0 00+-00-+', '000+00++ 000+0000000++0+0 00+-000+',
)
NB = 4
NR = len(_SCHEME)
_U, _V, _W = (np.array([["-0+".index(ch) - 1 for ch in row.split()[k]] for row in _SCHEME]) for k in range(3))
for _r in range(NR):
    if _V[_r][np.flatnonzero(_V[_r])[0]] < 0:
        _V[_r], _W[_r] = -_V[_r], -_W[_r]
assert (np.einsum("ra,rb,rc->abc", _U, _V, _W).reshape(2, NB, NB, NB, 2, NB)
        == np.einsum("st,jk,il->sjkitl", np.eye(2), np.eye(NB), np.eye(NB))).all()
_ACTIVE = {2: list(range(NR)), 1: [r for r in range(NR) if _U[r, :NB].any() and _W[r, :NB].any()]}


def _combine(coef, xs):
    xs = list(xs)
    rows = [{k: int(c) for k, c in enumerate(row) if c} for row in coef]
    while True:
        count = collections.Counter((a, b, row[a] * row[b]) for row in rows for a in row for b in row if a < b)
        if not count or max(count.values()) < 2:
            break
        a, b, s = max(count, key=count.get)
        xs.append(xs[a] + xs[b] if s > 0 else xs[a] - xs[b])
        for row in rows:
            if a in row and b in row and row[a] * row[b] == s:
                row[len(xs) - 1] = row.pop(a)
                del row[b]
    out = []
    for row in rows:
        terms = sorted(row.items(), key=lambda t: -t[1])
        acc = xs[terms[0][0]] if terms[0][1] > 0 else -xs[terms[0][0]]
        for k, c in terms[1:]:
            acc = acc + xs[k] if c > 0 else acc - xs[k]
        out.append(acc)
    return out


def _left(blocks):
    act = _ACTIVE[len(blocks) // NB]
    return list(enumerate(_combine(_U[act, :len(blocks)], blocks)))


def _block_matmul(halves, lhs, rhs, outs=None):
    outs = [(1, o) for o in outs] if outs else [None] * (halves * NB)
    for slot, r in enumerate(_ACTIVE[halves]):
        m = _dot(lhs(slot), rhs(r))
        for k, c in enumerate(_W[r, :len(outs)]):
            if c and outs[k] is None:
                outs[k] = (c, m)
            elif c:
                s, acc = outs[k]
                outs[k] = (s, acc + m) if s == c else (1, acc - m) if s > 0 else (1, m - acc)
    return [acc if s > 0 else -acc for s, acc in outs]


def _ln(x):
    m = jnp.mean(x, axis=-1, keepdims=True)
    c = x - m
    v = jnp.mean(c * c, axis=-1, keepdims=True)
    return c * jax.lax.rsqrt(v + 1e-5)


def _sigmoid(x):
    return 0.5 * jnp.tanh(0.5 * x) + 0.5


def _dot(a, b):
    return jax.lax.dot_general(a, b, (((1,), (0,)), ((), ())), preferred_element_type=F32)


def _dot_nt(a, b):
    return jax.lax.dot_general(a, b, (((1,), (1,)), ((), ())), preferred_element_type=F32)


def _lo(w):
    return pltpu.bitcast(w << 16, F32)


def _hi(w):
    return pltpu.bitcast(w & np.uint32(0xFFFF0000), F32)


def _pack(lo, hi):
    return pltpu.bitcast(pltpu.pack_elementwise([lo, hi], packed_dtype=BF16), U32)


def _bf(w):
    return pltpu.bitcast(w, BF16)


def _cols(x):
    n = x.shape[1] // NB
    return [x[:, k * n:(k + 1) * n] for k in range(NB)]


def build(S, D, H, E, M, T, F, cfg):
    d = cfg["d"]
    nseg = S // T
    nch = nseg // d
    C, L, G = d * T, M + T, H // NB
    C2, T2, DB, FB = C // 2, T // 2, D // NB, F // NB
    KD, KF = DB // 128, FB // 128
    scale = float(E) ** -0.5
    scope = jax.named_scope if cfg.get("prof") else (lambda n: contextlib.nullcontext())

    def loop(lo, hi, fn, name):
        def body(i, carry):
            with scope(name):
                fn(i)
            return carry
        jax.lax.fori_loop(lo, hi, body, 0)

    def kern(x_hbm, mem_ref, wq, wk, wv, wo_hbm, wg_hbm, wu_hbm, wd_hbm, out_hbm,
             xs, wqkv, wo, wg, wu, wd, mem, ha, ba, fa, xa, xb, yb, qsem, osem, wsem, ysem):
        kn = [(k, n) for k in range(NB) for n in range(NB)]

        def qkv_copies(g):
            return [pltpu.make_async_copy(w.bitcast(U32).at[:, :, par, 2 * g + p, :],
                                          wqkv.at[g, m, pl.ds((2 * p + par) * NB, NB)], qsem.at[g])
                    for m, w in enumerate((wq, wk, wv)) for p in range(2) for par in range(2)]

        def wo_copies(g):
            return [pltpu.make_async_copy(wo_hbm.bitcast(U32).at[g, :, :, pl.ds(n * DB, DB)],
                                          wo.at[pl.ds(n * NB, NB), g], osem.at[g]) for n in range(NB)]

        def b_copies(src, dst, i):
            nc = dst.shape[2]
            return [pltpu.make_async_copy(src.bitcast(U32).at[:, :, pl.ds(n * nc, nc)],
                                          dst.at[pl.ds(n * NB, NB)], wsem.at[i]) for n in range(NB)]
        b_cps = [b_copies(wg_hbm, wg, 0), b_copies(wu_hbm, wu, 1), b_copies(wd_hbm, wd, 2)]
        x_cps = [pltpu.make_async_copy(x_hbm.at[0:C], xs.at[0:C], wsem.at[3]),
                 pltpu.make_async_copy(x_hbm.at[C:S], xs.at[C:S], wsem.at[4])]

        def start(cps):
            for cp in cps:
                cp.start()

        def wait(cps):
            for cp in cps:
                cp.wait()

        def prep_qkv(g, m, rows):
            raw = [wqkv[g, m, s, rows, :] for s in range(NB * NB)]
            ev, od = (_combine(_V, [(_hi if n % 2 else _lo)(raw[(n // 2 * 2 + par) * NB + k]) for k, n in kn])
                      for par in range(2))
            for r in range(NR):
                wqkv[g, m, r, rows, :] = _pack(ev[r], od[r])

        def prep(w, idx):
            raw = [w[(n * NB + k,) + idx] for k, n in kn]
            lo, hi = (_combine(_V, [f(v) for v in raw]) for f in (_lo, _hi))
            for r in range(NR):
                one = np.flatnonzero(_V[r])
                w[(r,) + idx] = raw[one[0]] if len(one) == 1 else _pack(lo[r], hi[r])

        def prep_rows(w, step):
            def body(i):
                for r in range(0, step, 8):
                    for c in range(0, w.shape[2], 128):
                        prep(w, (pl.ds(pl.multiple_of(i * step + r, 8), 8), slice(c, c + 128)))
            loop(0, w.shape[1] // step, body, "z_prepb")

        def seg(ref, i):
            return ref[pl.ds(pl.multiple_of(i * T, T), T), :]

        def put(ref, t0, rows, v):
            for k in range(v.shape[1] // 128):
                ref[t0 + k, rows, :] = v[:, k * 128:(k + 1) * 128]

        def get(ref, t0, n, nrows, after=None):
            ts = [ref[t0 + k, 0:nrows, :] for k in range(n)]
            if after is not None:
                head = jnp.where(after[1] == 0, ts[0][0:8], after[0][after[1], 0:8, :])
                ts[0] = jnp.concatenate([head, ts[0][8:]], axis=0)
            return jnp.concatenate(ts, axis=1)

        def put_h(rows, *xs_):
            for s, v in _left([b for x in xs_ for b in _cols(x)]):
                put(ha, s * KD, rows, v)

        def attn_masks():
            r = jax.lax.broadcasted_iota(jnp.int32, (2 * L, 128), 0)
            k = jax.lax.broadcasted_iota(jnp.int32, (2 * L, 128), 1)
            rp = jnp.where(r < L, r, r - L)
            kp = jnp.where(r < L, k, k - L)
            same = (kp >= 0) & (kp < L)
            valid = same & ((rp < M) | (rp >= kp))
            return valid, jnp.where(same, -1e9, -jnp.inf).astype(F32)

        def proj(g, m, halves, after=None):
            last = len(_ACTIVE[halves]) - 1
            c = _block_matmul(halves, lambda s: get(ha, s * KD, KD, L, after if s == last else None),
                              lambda r: _bf(wqkv[g, m, r]))
            n = len(c) // 2
            c = [jnp.concatenate([c[k], c[k + n]], axis=0) for k in range(n)]
            if m == 0:
                return [y * scale for y in c]
            z = jnp.zeros((128 - 2 * L, E), BF16)
            return [jnp.concatenate([y.astype(BF16), z], axis=0) for y in c]

        def probs(qs, ks, masks):
            res = []
            for q, k in zip(qs, ks):
                s = jnp.where(masks[0], _dot_nt(q, k), masks[1])
                p = jnp.exp(s - jnp.max(s, axis=-1, keepdims=True))
                l = jnp.sum(p, axis=-1, keepdims=True)
                r = pl.reciprocal(l, approx=True)
                r = r * (2.0 - l * r)
                res.append((p, r * (2.0 - l * r)))
            return res

        def mix(g, ps, vs):
            o = [_dot(p, v) * r for (p, r), v in zip(ps, vs)]
            for s, v in _left([y[:L] for y in o] + [y[L:] for y in o]):
                fa[s * G + g, 0:L, :] = v

        def out_proj(g0, n, c, halves, acc=None):
            return _block_matmul(halves, lambda s: get(fa, s * G + g0, n, L),
                                 lambda r: _bf(wo[r, pl.ds(g0, n), :, c * 128:(c + 1) * 128].reshape(n * E // 2, 128)),
                                 acc)

        mrows, trows = slice(0, M), slice(M, L)

        def finish_cols(c, y, residual):
            for s, v in _left([b[:M] for b in y]):
                ha[s * KD + c, mrows, :] = v
            for k, b in enumerate(y):
                cols = slice((k % NB) * DB + c * 128, (k % NB) * DB + (c + 1) * 128)
                mem[k // NB, :, cols] = b[:M]
                residual(k // NB, cols, b[M:])

        def a_step(halves, zero, extra, next_tokens, residual):
            masks = attn_masks()
            so, po, kc = cfg["so"], cfg["po"], cfg["kc"]
            pr, ps, acc, done = {}, {}, {}, [0]
            side = sorted([(3 * g + 1 + so, 0, g) for g in range(G)] + [(3 * g + 1 + so + po, 1, g) for g in range(G)]
                          + [(cfg["nt"] + 3 * G - 1, 2, 0)])

            def run_side(now):
                while side and side[0][0] <= now:
                    _, kind, g = side.pop(0)
                    if kind == 0:
                        ps[g] = probs(pr[g, 0], pr[g, 1], masks)
                    elif kind == 1:
                        mix(g, ps[g], pr[g, 2])
                        done[0] = g + 1
                    else:
                        put_h(trows, *next_tokens())
            outs = [(g0, n, c) for g0, n in zip(np.cumsum([0] + kc[:-1]).tolist(), kc) for c in range(KD)]

            def run_out():
                g0, n, c = outs.pop(0)
                assert g0 + n <= done[0]
                acc[c] = out_proj(g0, n, c, halves, acc.get(c))
                if g0 + n == G:
                    finish_cols(c, acc[c], residual)
            for g in range(G):
                for m in range(3):
                    if m == 0 and g in cfg["bj"][:len(extra)]:
                        extra[cfg["bj"].index(g)]()
                    pr[g, m] = proj(g, m, halves, (ba, zero) if m == 2 and g in cfg["bk"] else None)
                    run_side(3 * g + m)
                    if len(outs) > KD + cfg["keep"] and outs[0][0] + outs[0][1] <= done[0] and m in cfg["om"]:
                        run_out()
            now = 3 * G - 1
            while outs:
                run_out()
                now += cfg.get("os", 2)
                run_side(now)

        def a_dual(c, i):
            t = c * d + i
            rows = pl.ds(pl.multiple_of(i * T, T), T)
            xrows = pl.ds(pl.multiple_of(t * T, T), T)

            def residual(layer, cols, v):
                xa[layer, rows, cols] = v + (xb[0, rows, cols] if layer else xs[xrows, cols].astype(F32))
            a_step(2, i // d, [lambda: b_head(0, (i + d - 1) % d), lambda: b_head(1, (i + d - 1) % d)],
                   lambda: (_ln(seg(xs, jnp.minimum(t + 1, nseg - 1)).astype(F32)),
                            _ln(seg(xb.at[0], jnp.minimum(i + 1, d - 1)))), residual)

        def single_io(w, i):
            rows = pl.ds(pl.multiple_of(i * T, T), T)

            def residual(layer, cols, v):
                xa[w, rows, cols] = v + xb[0, rows, cols]
            return (lambda: (_ln(seg(xb.at[0], jnp.minimum(i + 1, d - 1))),)), residual

        def a_head(c, r0, nr):
            if r0 == 0:
                put_h(mrows, mem[0], mem[1])
            x1 = xs[pl.ds(pl.multiple_of(jnp.minimum(c * d, nseg - 1) * T + r0, nr), nr), :]
            put_h(slice(M + r0, M + r0 + nr), _ln(x1.astype(F32)), _ln(xb[0, r0:r0 + nr, :]))

        def b_head(w, i):
            a = _ln(seg(xa.at[w], i))
            rows = pl.ds(pl.multiple_of(i * T2, T2), T2)
            for s, v in _left(_cols(a[:T2]) + _cols(a[T2:])):
                put(ba, (w * NR + s) * KD, rows, v)

        def b_step(c, w):
            zero = w // 2
            for n in range(KF):
                cols = slice(n * 128, (n + 1) * 128)
                aft = (ha, zero) if n - cfg["ba"] in range(T // 16) else None
                g = _block_matmul(2, lambda s: get(ba, (w * NR + s) * KD, KD, C2), lambda r: _bf(wg[r, :, cols]))
                g = [_sigmoid(v) for v in g]
                u = _block_matmul(2, lambda s: get(ba, (w * NR + s) * KD, KD, C2, aft if s == NR - 1 else None),
                                  lambda r: _bf(wu[r, :, cols]))
                for s, v in _left([gg * uu for gg, uu in zip(g, u)]):
                    fa[s * KF + n] = v
                if n < T // 16:
                    a_head(c + 1, n * 16, 16)
            kf, nf = cfg["kf"], cfg["nf"]

            def down(k0, nk, n, acc=None):
                return _block_matmul(2, lambda s: get(fa, s * KF + k0, nk, C2),
                                     lambda r: _bf(wd[r, k0 * 64:(k0 + nk) * 64, n * 128:(n + 1) * 128]), acc)
            first = [down(0, kf, n) for n in range(nf)]
            for n in range(KD):
                y = down(kf, KF - kf, n, first[n]) if n < nf else down(0, KF, n)
                for k, v in enumerate(y):
                    cols = slice((k % NB) * DB + n * 128, (k % NB) * DB + (n + 1) * 128)
                    for i in range(d):
                        rows = slice(i * T + (k // NB) * T2, i * T + (k // NB + 1) * T2)
                        r = v[i * T2:(i + 1) * T2] + xa[w, rows, cols]
                        xb[w, rows, cols] = r
                        yb[rows, cols] = r.astype(BF16)

        def y_copy(c):
            return pltpu.make_async_copy(yb, out_hbm.at[pl.ds(pl.multiple_of(c * C, C), C), :], ysem.at[0])

        ahead = cfg["ahead"]
        with scope("z_head"):
            x_cps[0].start()
            for g in range(ahead):
                start(qkv_copies(g))
            x_cps[0].wait()
            xb[0] = xs[0:C, :].astype(F32)
            mem[1] = mem_ref[...].astype(F32)
            put_h(mrows, mem[1])
            put_h(trows, _ln(xb[0, 0:T, :]))
            xa[1] = jnp.zeros((C, D), F32)
            ba[...] = jnp.zeros(ba.shape, F32)
            ha[len(_ACTIVE[1]) * KD:] = jnp.zeros(((NR - len(_ACTIVE[1])) * KD, L, 128), F32)

        def first_qkv(g):
            @pl.when(g + ahead < G)
            def _():
                start(qkv_copies(g + ahead))

            @pl.when(g + ahead == G)
            def _():
                for g2 in range(G):
                    start(wo_copies(g2))
            wait(qkv_copies(g))

            def rows(i):
                for m in range(3):
                    for r in range(0, 16, 8):
                        prep_qkv(g, m, pl.ds(pl.multiple_of(i * 16 + r, 8), 8))
            loop(0, DB // 32, rows, "y_pq")
            mix(g, probs(proj(g, 0, 1), proj(g, 1, 1), attn_masks()), proj(g, 2, 1))
        loop(0, G, first_qkv, "z_first")
        start(b_cps[0] + b_cps[1] + b_cps[2] + x_cps[1:])

        def first_out(g):
            wait(wo_copies(g))

            def rows(i):
                for c in range(KD):
                    prep(wo, (g, pl.ds(pl.multiple_of(i * 8, 8), 8), slice(c * 128, (c + 1) * 128)))
            loop(0, E // 16, rows, "y_po")
            for c in range(KD):
                for k, v in enumerate(out_proj(g, 1, c, 1)):
                    xa[1, 0:L, k * DB + c * 128:k * DB + (c + 1) * 128] += v
        loop(0, G, first_out, "z_first_o")
        nxt, res = single_io(0, 0)
        put_h(trows, *nxt())
        for c in range(KD):
            finish_cols(c, [xa[1, 0:L, k * DB + c * 128:k * DB + (c + 1) * 128] for k in range(NB)], res)

        def chunk(c):
            edge = (c == 0) | (c == nch)
            w0 = jnp.where(c < nch, 0, 1)

            @pl.when(edge)
            def _():
                @pl.when(c == nch)
                def _():
                    put_h(mrows, mem[1])
                    put_h(trows, _ln(xb[0, 0:T, :]))
                loop(1 - w0, d, lambda i: a_step(1, i // d, [lambda: b_head(w0, (i + d - 1) % d)],
                                                 *single_io(w0, i)), "z_single")
                b_head(w0, d - 1)

                @pl.when(c == 0)
                def _():
                    for cps, wt, step in zip(b_cps, (wg, wu, wd), (8, 8, 16)):
                        with scope("z_waitb"):
                            wait(cps)
                        prep_rows(wt, step)
                    x_cps[1].wait()

            @pl.when(jnp.logical_not(edge))
            def _():
                loop(0, d, lambda i: a_dual(c, i), "z_dual")
                with scope("z_bhead"):
                    b_head(0, d - 1)
                    b_head(1, d - 1)

            @pl.when(c >= 2)
            def _():
                y_copy(c - 2).wait()
            loop(w0, jnp.where(c > 0, 2, 1), lambda w: b_step(c, w), "z_b")

            @pl.when(c == 0)
            def _():
                a_head(1, 0, T)

            @pl.when(c >= 1)
            def _():
                y_copy(c - 1).start()
        loop(0, nch + 1, chunk, "z_chunk")
        y_copy(nch - 1).wait()

    any_spec = pl.BlockSpec(memory_space=pl.ANY)
    V = pltpu.VMEM
    return pl.pallas_call(
        kern,
        out_shape=jax.ShapeDtypeStruct((S, D), BF16),
        in_specs=[any_spec, pl.BlockSpec(memory_space=pltpu.VMEM)] + [any_spec] * 7,
        out_specs=any_spec,
        scratch_shapes=[
            V((S, D), BF16), V((G, 3, NR, DB // 2, E), U32), V((NR, G, E // 2, DB), U32),
            V((NR, DB // 2, FB), U32), V((NR, DB // 2, FB), U32), V((NR, FB // 2, DB), U32),
            V((2, M, D), F32), V((NR * KD, L, 128), F32), V((2 * NR * KD, C2, 128), F32),
            V((NR * max(KF, G), C2, 128), F32), V((2, C, D), F32), V((2, C, D), F32), V((C, D), BF16),
            pltpu.SemaphoreType.DMA((G,)), pltpu.SemaphoreType.DMA((G,)),
            pltpu.SemaphoreType.DMA((5,)), pltpu.SemaphoreType.DMA((1,)),
        ],
        compiler_params=pltpu.CompilerParams(vmem_limit_bytes=126 * 2**20, flags=cfg.get("flags")),
    )


@functools.partial(jax.jit, static_argnames=("A_seg_len",))
def pallas_interleave_layers__memory_aug_recurrent_mem_tr__glu_gated_glu__prompt_kernel(
        A_x, A_mem0, A_Wq, A_Wk, A_Wv, A_Wo, A_seg_len, B_x, B_w_gate, B_w_up, B_w_down):
    del B_x
    B, S, D = A_x.shape
    H, E = A_Wq.shape[1:]
    M = A_mem0.shape[1]
    F = B_w_gate.shape[1]
    call = build(S, D, H, E, M, int(A_seg_len), F, CFG)
    qkv = [w.reshape(NB, D // (2 * NB), 2, H, E) for w in (A_Wq, A_Wk, A_Wv)]
    out = call(A_x.reshape(S, D), A_mem0.reshape(M, D), *qkv, A_Wo.reshape(H // NB, NB, E, D),
               B_w_gate.reshape(NB, D // NB, F), B_w_up.reshape(NB, D // NB, F),
               B_w_down.reshape(NB, F // NB, D))
    return out.reshape(B, S, D)
```

```python
import collections
import contextlib
import functools

import jax
import jax.experimental.pallas as pl
import jax.experimental.pallas.tpu as pltpu
import jax.numpy as jnp
import numpy as np

F32, BF16, U32 = jnp.float32, jnp.bfloat16, jnp.uint32
CFG = dict(d=4, so=1, po=2, kc=[6, 2], keep=2, om=[2], fs=1, il=False, kf=5, nf=1, p1=26, d1=60, p2=8, d2=30, p3=8, d3=8, st=False, mv=4, p4=0,
           ahead=2, cse=True)

_SCHEME = (
    '+000+000 ++000000+0000000 0000+000', '+0000000 +0+0+00000000000 +000-000',
    '0+000+00 0000++0+0+000000 0+000000', '00000+00 0-000-+000000-00 0+000-00',
    '+-000000 0000-00000000000 +-000000', '0000+-00 0-00000000000000 0000+-00',
    '+0000+00 0-00+00000000000 0-00+000', '0+-00+-0 000000000-000000 00000++0',
    '0+-00000 000000+000000000 0++00--0', '0+-00+00 000000-00-000000 0+000--0',
    '0+0-0000 0000000-00000000 0+0-0000', '00000+0- 0000000000000-00 00000+0-',
    '000+0+00 0000000-00000+00 0+00000-', '00+00000 000+00+0+0++0000 00+00000',
    '000000+0 00+000000-+0-0-0 000000+0', '+0-0+0-0 000-0000-0000000 +0-00000',
    '0000+0-0 00+000000000+000 +0-0-0+0', '+000+0-0 00-00000+0000000 +0-0-000',
    '+0-+0000 000+000000000000 +0-+0000', '0000+0-+ 000000000000+000 0000+0-+',
    '000-+0-0 000+00000000-000 +0-0000+', '000+000+ 000-0000000--+0+ 0000000+',
    '000+0000 000-000+0000+0++ 000+000-', '00++00++ 000-0000000-0000 00+-0000',
    '000000++ 000000000000-0-0 00+-00-+', '000+00++ 000+0000000++0+0 00+-000+',
)
NB = 4
NR = len(_SCHEME)
_U, _V, _W = (np.array([["-0+".index(ch) - 1 for ch in row.split()[k]] for row in _SCHEME]) for k in range(3))
for _r in range(NR):
    if _V[_r][np.flatnonzero(_V[_r])[0]] < 0:
        _V[_r], _W[_r] = -_V[_r], -_W[_r]
assert (np.einsum("ra,rb,rc->abc", _U, _V, _W).reshape(2, NB, NB, NB, 2, NB)
        == np.einsum("st,jk,il->sjkitl", np.eye(2), np.eye(NB), np.eye(NB))).all()
_ACTIVE = {2: list(range(NR)), 1: [r for r in range(NR) if _U[r, :NB].any() and _W[r, :NB].any()]}


def _combine(coef, xs):
    xs = list(xs)
    rows = [{k: int(c) for k, c in enumerate(row) if c} for row in coef]
    while True:
        count = collections.Counter((a, b, row[a] * row[b]) for row in rows for a in row for b in row if a < b)
        if not count or max(count.values()) < 2:
            break
        a, b, s = max(count, key=count.get)
        xs.append(xs[a] + xs[b] if s > 0 else xs[a] - xs[b])
        for row in rows:
            if a in row and b in row and row[a] * row[b] == s:
                row[len(xs) - 1] = row.pop(a)
                del row[b]
    out = []
    for row in rows:
        terms = sorted(row.items(), key=lambda t: -t[1])
        acc = xs[terms[0][0]] if terms[0][1] > 0 else -xs[terms[0][0]]
        for k, c in terms[1:]:
            acc = acc + xs[k] if c > 0 else acc - xs[k]
        out.append(acc)
    return out


def _left(blocks):
    act = _ACTIVE[len(blocks) // NB]
    return list(enumerate(_combine(_U[act, :len(blocks)], blocks)))


def _block_matmul(halves, lhs, rhs, outs=None):
    outs = [(1, o) for o in outs] if outs else [None] * (halves * NB)
    for slot, r in enumerate(_ACTIVE[halves]):
        m = _dot(lhs(slot), rhs(r))
        for k, c in enumerate(_W[r, :len(outs)]):
            if c and outs[k] is None:
                outs[k] = (c, m)
            elif c:
                s, acc = outs[k]
                outs[k] = (s, acc + m) if s == c else (1, acc - m) if s > 0 else (1, m - acc)
    return [acc if s > 0 else -acc for s, acc in outs]


def _ln(x):
    m = jnp.mean(x, axis=-1, keepdims=True)
    c = x - m
    v = jnp.mean(c * c, axis=-1, keepdims=True)
    return c * jax.lax.rsqrt(v + 1e-5)


def _sigmoid(x):
    return 0.5 * jnp.tanh(0.5 * x) + 0.5


def _dot(a, b):
    return jax.lax.dot_general(a, b, (((1,), (0,)), ((), ())), preferred_element_type=F32)


def _dot_nt(a, b):
    return jax.lax.dot_general(a, b, (((1,), (1,)), ((), ())), preferred_element_type=F32)


def _lo(w):
    return pltpu.bitcast(w << 16, F32)


def _hi(w):
    return pltpu.bitcast(w & np.uint32(0xFFFF0000), F32)


def _pack(lo, hi):
    return pltpu.bitcast(pltpu.pack_elementwise([lo, hi], packed_dtype=BF16), U32)


def _bf(w):
    return pltpu.bitcast(w, BF16)


def _cols(x):
    n = x.shape[1] // NB
    return [x[:, k * n:(k + 1) * n] for k in range(NB)]


def build(S, D, H, E, M, T, F, cfg):
    d = cfg["d"]
    nseg = S // T
    nch = nseg // d
    C, L, G = d * T, M + T, H // NB
    C2, T2, DB, FB = C // 2, T // 2, D // NB, F // NB
    KD, KF = DB // 128, FB // 128
    FS = cfg['fs']
    FN = -(-NR // FS)
    scale = float(E) ** -0.5
    scope = jax.named_scope if cfg.get("prof") else (lambda n: contextlib.nullcontext())

    def loop(lo, hi, fn, name):
        def body(i, carry):
            with scope(name):
                fn(i)
            return carry
        jax.lax.fori_loop(lo, hi, body, 0)

    def kern(x_hbm, mem_ref, wq, wk, wv, wo_hbm, wg_hbm, wu_hbm, wd_hbm, out_hbm,
             xs, wqkv, wo, wg, wu, wd, mem, ha, hb, ba, xa, xb, yb, qsem, osem, wsem, ysem, *fa):
        kn = [(k, n) for k in range(NB) for n in range(NB)]

        def qkv_copies(g):
            return [pltpu.make_async_copy(w.bitcast(U32).at[:, :, par, 2 * g + p, :],
                                          wqkv.at[g, m, pl.ds((2 * p + par) * NB, NB)], qsem.at[g])
                    for m, w in enumerate((wq, wk, wv)) for p in range(2) for par in range(2)]

        def wo_copies(g):
            return [pltpu.make_async_copy(wo_hbm.bitcast(U32).at[g, :, :, pl.ds(n * DB, DB)],
                                          wo.at[pl.ds(n * NB, NB), g], osem.at[g]) for n in range(NB)]

        def b_copies(src, dst, i):
            nc = dst.shape[2]
            return [pltpu.make_async_copy(src.bitcast(U32).at[:, :, pl.ds(n * nc, nc)],
                                          dst.at[pl.ds(n * NB, NB)], wsem.at[i]) for n in range(NB)]
        b_cps = [b_copies(wg_hbm, wg, 0), b_copies(wu_hbm, wu, 1), b_copies(wd_hbm, wd, 2)]
        x_cps = [pltpu.make_async_copy(x_hbm.at[0:C], xs.at[0:C], wsem.at[3]),
                 pltpu.make_async_copy(x_hbm.at[C:S], xs.at[C:S], wsem.at[4])]

        def start(cps):
            for cp in cps:
                cp.start()

        def wait(cps):
            for cp in cps:
                cp.wait()

        def prep_qkv(g, m, rows):
            raw = [wqkv[g, m, s, rows, :] for s in range(NB * NB)]
            ev, od = (_combine(_V, [(_hi if n % 2 else _lo)(raw[(n // 2 * 2 + par) * NB + k]) for k, n in kn])
                      for par in range(2))
            for r in range(NR):
                wqkv[g, m, r, rows, :] = _pack(ev[r], od[r])

        def prep(w, idx):
            raw = [w[(n * NB + k,) + idx] for k, n in kn]
            lo, hi = (_combine(_V, [f(v) for v in raw]) for f in (_lo, _hi))
            for r in range(NR):
                one = np.flatnonzero(_V[r])
                w[(r,) + idx] = raw[one[0]] if len(one) == 1 else _pack(lo[r], hi[r])

        def prep_rows(w, step):
            def body(i):
                for r in range(0, step, 8):
                    for c in range(0, w.shape[2], 128):
                        prep(w, (pl.ds(pl.multiple_of(i * step + r, 8), 8), slice(c, c + 128)))
            loop(0, w.shape[1] // step, body, "z_prepb")

        def get(tiles, nrows, after=None):
            ts = [ref[t, 0:nrows, :] for ref, t in tiles]
            if after is not None:
                head = jnp.where(after[0] == 0, ts[0][0:8], after[1])
                ts[0] = jnp.concatenate([head, ts[0][8:]], axis=0)
            return jnp.concatenate(ts, axis=1)

        def pieces(ref, t0, rows, load):
            cache = []

            def step(k):
                if not cache:
                    cache.extend(b for x in load() for b in _cols(x))
                for s, v in _left([b[:, k * 128:(k + 1) * 128] for b in cache]):
                    ref[t0 + s * KD + k, rows, :] = v
            return [(functools.partial(step, k), ref) for k in range(KD)]

        def run(steps):
            for step, _ in steps:
                step()

        class Background:
            def __init__(self, zero):
                self.zero, self.queue, self.wait, self.period = zero, [], 0, 1

            def add(self, steps, period, delay=None):
                self.queue += steps
                self.wait, self.period = period if delay is None else delay, period

            def __call__(self):
                self.wait -= 1
                if not self.queue or self.wait > 0:
                    return None
                self.wait = self.period
                step, ref = self.queue.pop(0)
                value = step()
                return self.zero, value if ref is None else ref[self.zero, 0:8, :]

        mrows = slice(0, M)

        def mem_head(*ws):
            return pieces(ha, 0, mrows, lambda: [mem[w] for w in ws])

        def tok_head(t, i, staged=False):
            def load(r):
                second = _ln(xb[0, pl.ds(pl.multiple_of(i * T + r, 16), 16), :])
                if t is None:
                    return [second]
                return [_ln(xs[pl.ds(pl.multiple_of(t * T + r, 16), 16), :].astype(F32)), second]

            def move(t0, t1, after):
                ha[t0:t1, M:L, :] = jnp.where(after[0] == 0, hb[t0:t1], jnp.tile(after[1], (T // 8, 1)))
            dst, off = (hb, 0) if staged else (ha, M)
            steps = [p for r in range(0, T, 16)
                     for p in pieces(dst, 0, slice(off + r, off + r + 16), functools.partial(load, r))]
            if not staged:
                return [], steps
            n = len(_ACTIVE[1 if t is None else 2]) * KD
            return steps, [(functools.partial(move, k, min(k + cfg["mv"], n)), ha) for k in range(0, n, cfg["mv"])]

        def attn_masks():
            r = jax.lax.broadcasted_iota(jnp.int32, (2 * L, 128), 0)
            k = jax.lax.broadcasted_iota(jnp.int32, (2 * L, 128), 1)
            rp = jnp.where(r < L, r, r - L)
            kp = k // 2
            same = (kp < L) & (k % 2 == jnp.where(r < L, 0, 1))
            valid = same & ((rp < M) | (rp >= kp))
            return valid, jnp.where(same, -1e9, -jnp.inf).astype(F32)

        def proj(g, m, halves, bg=lambda: None):
            c = _block_matmul(halves, lambda s: get([(ha, s * KD + k) for k in range(KD)], L, bg()), lambda r: _bf(wqkv[g, m, r]))
            n = len(c) // 2
            if m == 0:
                return [jnp.concatenate([c[k], c[k + n]], axis=0) * scale for k in range(n)]
            z = jnp.zeros((64 - L, E), U32)
            return [_bf(jnp.concatenate([_pack(c[k], c[k + n]), z], axis=0)) for k in range(n)]

        def probs(qs, ks, masks):
            res = []
            for q, k in zip(qs, ks):
                s = jnp.where(masks[0], _dot_nt(q, k), masks[1])
                p = jnp.exp(s - jnp.max(s, axis=-1, keepdims=True))
                l = jnp.sum(p, axis=-1, keepdims=True)
                r = pl.reciprocal(l, approx=True)
                res.append(p * (r * (2.0 - l * r)))
            return res

        def slot(g, s):
            return fa[g * FS + s % FS if cfg['il'] else g * FS + s // FN], s // FS if cfg['il'] else s % FN

        def mix(tile, ps, vs):
            o = [_dot(p, v) for p, v in zip(ps, vs)]
            for s, v in _left([y[:L] for y in o] + [y[L:] for y in o]):
                ref, t = tile(s)
                ref[t, 0:L, :] = v

        def out_proj(g0, n, c, halves, tile, acc=None, bg=lambda: None):
            return _block_matmul(halves, lambda s: get([tile(k, s) for k in range(n)], L, bg()),
                                 lambda r: _bf(wo[r, pl.ds(g0, n), :, c * 128:(c + 1) * 128].reshape(n * E // 2, 128)),
                                 acc)

        def finish_cols(c, y, residual):
            for s, v in _left([b[:M] for b in y]):
                ha[s * KD + c, mrows, :] = v
            for k, b in enumerate(y):
                cols = slice((k % NB) * DB + c * 128, (k % NB) * DB + (c + 1) * 128)
                mem[k // NB, :, cols] = b[:M]
                residual(k // NB, cols, b[M:])

        def a_step(halves, zero, extra, next_tokens, residual):
            masks = attn_masks()
            so, po, kc = cfg["so"], cfg["po"], cfg["kc"]
            pr, ps, acc, done = {}, {}, {}, [0]
            side = sorted([(3 * g + 1 + so, 0, g) for g in range(G)] + [(3 * g + 1 + so + po, 1, g) for g in range(G)])
            bg = Background(zero)
            bg.add(extra + next_tokens[0], cfg["p1"], cfg['d1'])

            def run_side(now):
                while side and side[0][0] <= now:
                    _, kind, g = side.pop(0)
                    if kind == 0:
                        ps[g] = probs(pr[g, 0], pr[g, 1], masks)
                    else:
                        mix(functools.partial(slot, g), ps[g], pr[g, 2])
                        done[0] = g + 1
            outs = [(g0, n, c) for g0, n in zip(np.cumsum([0] + kc[:-1]).tolist(), kc) for c in range(KD)]

            def run_out():
                g0, n, c = outs.pop(0)
                assert g0 + n <= done[0]
                acc[c] = out_proj(g0, n, c, halves, lambda k, s: slot(g0 + k, s), acc.get(c), bg)
                if g0 + n == G:
                    finish_cols(c, acc[c], residual)
            for g in range(G):
                for m in range(3):
                    pr[g, m] = proj(g, m, halves, bg)
                    run_side(3 * g + m)
                    if len(outs) > KD + cfg["keep"] and outs[0][0] + outs[0][1] <= done[0] and m in cfg["om"]:
                        run_out()
            late = (zero, pltpu.bitcast(pr[G - 1, 2][0][0:16], F32))
            bg.add([(functools.partial(f, late) if next_tokens[0] else f, ref) for f, ref in next_tokens[1]],
                   cfg['p2'], cfg['d2'])
            now = 3 * G - 1
            while outs:
                run_out()
                now += cfg.get("os", 2)
                run_side(now)
            run(bg.queue)

        def a_dual(c, i):
            t = c * d + i
            rows = pl.ds(pl.multiple_of(i * T, T), T)
            xrows = pl.ds(pl.multiple_of(t * T, T), T)

            def residual(layer, cols, v):
                xa[layer, rows, cols] = v + (xb[0, rows, cols] if layer else xs[xrows, cols].astype(F32))
            a_step(2, i // d, b_head(0, (i + d - 1) % d) + b_head(1, (i + d - 1) % d),
                   tok_head(jnp.minimum(t + 1, nseg - 1), jnp.minimum(i + 1, d - 1), cfg['st']), residual)

        def single_io(w, i):
            rows = pl.ds(pl.multiple_of(i * T, T), T)

            def residual(layer, cols, v):
                xa[w, rows, cols] = v + xb[0, rows, cols]
            return tok_head(None, jnp.minimum(i + 1, d - 1)), residual

        def a_head(c):
            return sum(tok_head(jnp.minimum(c * d, nseg - 1), 0), mem_head(0, 1))

        def b_head(w, i):
            def load(r):
                return [_ln(xa[w, pl.ds(pl.multiple_of(i * T + h + r, 8), 8), :]) for h in (0, T2)]
            return [p for r in range(0, T2, 8)
                    for p in pieces(ba, w * NR * KD, pl.ds(pl.multiple_of(i * T2 + r, 8), 8), functools.partial(load, r))]

        def b_step(c, w):
            bg = Background(w // 2)
            bg.add(a_head(c + 1), cfg["p3"], cfg["d3"])
            pend = None
            for n in range(KF):
                cols = slice(n * 128, (n + 1) * 128)
                g = _block_matmul(2, lambda s: get([(ba, (w * NR + s) * KD + k) for k in range(KD)], C2, bg()), lambda r: _bf(wg[r, :, cols]))
                g = [_sigmoid(v) for v in g]
                u = _block_matmul(2, lambda s: get([(ba, (w * NR + s) * KD + k) for k in range(KD)], C2, bg()), lambda r: _bf(wu[r, :, cols]))
                h = [gg * uu for gg, uu in zip(g, u)]

                def store(r, n=n, h=h):
                    for s, v in _left([b[r:r + 8] for b in h]):
                        ref, t = slot(n, s)
                        ref[t, r:r + 8, :] = v
                steps = [(functools.partial(store, r), fa[n]) for r in range(0, C2, 8)]
                if cfg["p4"] and n < KF - 1:
                    bg.add(steps, cfg["p4"])
                else:
                    run(bg.queue + steps)
            kf, nf = cfg["kf"], cfg["nf"]

            def down(k0, nk, n, acc=None):
                return _block_matmul(2, lambda s: get([slot(k0 + k, s) for k in range(nk)], C2),
                                     lambda r: _bf(wd[r, k0 * 64:(k0 + nk) * 64, n * 128:(n + 1) * 128]), acc)
            first = [down(0, kf, n) for n in range(nf)]
            for n in range(KD):
                y = down(kf, KF - kf, n, first[n]) if n < nf else down(0, KF, n)
                for k, v in enumerate(y):
                    cols = slice((k % NB) * DB + n * 128, (k % NB) * DB + (n + 1) * 128)
                    for i in range(d):
                        rows = slice(i * T + (k // NB) * T2, i * T + (k // NB + 1) * T2)
                        r = v[i * T2:(i + 1) * T2] + xa[w, rows, cols]
                        xb[w, rows, cols] = r
                        yb[rows, cols] = r.astype(BF16)

        def y_copy(c):
            return pltpu.make_async_copy(yb, out_hbm.at[pl.ds(pl.multiple_of(c * C, C), C), :], ysem.at[0])

        ahead, n1 = cfg["ahead"], len(_ACTIVE[1])
        with scope("z_head"):
            x_cps[0].start()
            for g in range(ahead):
                start(qkv_copies(g))
            x_cps[0].wait()
            xb[0] = xs[0:C, :].astype(F32)
            mem[1] = mem_ref[...].astype(F32)
            run(sum(tok_head(None, 0), mem_head(1)))
            xa[1] = jnp.zeros((C, D), F32)
            ba[...] = jnp.zeros(ba.shape, F32)
            ha[len(_ACTIVE[1]) * KD:] = jnp.zeros(((NR - len(_ACTIVE[1])) * KD, L, 128), F32)

        def first_qkv(g):
            @pl.when(g + ahead < G)
            def _():
                start(qkv_copies(g + ahead))

            @pl.when(g + ahead == G)
            def _():
                for g2 in range(G):
                    start(wo_copies(g2))
            wait(qkv_copies(g))

            def rows(i):
                for m in range(3):
                    for r in range(0, 16, 8):
                        prep_qkv(g, m, pl.ds(pl.multiple_of(i * 16 + r, 8), 8))
            loop(0, DB // 32, rows, "y_pq")
            mix(lambda s: (ba, g * n1 + s), probs(proj(g, 0, 1), proj(g, 1, 1), attn_masks()), proj(g, 2, 1))
        loop(0, G, first_qkv, "z_first")
        start(b_cps[0] + b_cps[1] + b_cps[2] + x_cps[1:])

        def first_out(g):
            wait(wo_copies(g))

            def rows(i):
                for c in range(KD):
                    prep(wo, (g, pl.ds(pl.multiple_of(i * 8, 8), 8), slice(c * 128, (c + 1) * 128)))
            loop(0, E // 16, rows, "y_po")
            for c in range(KD):
                for k, v in enumerate(out_proj(g, 1, c, 1, lambda k, s: (ba, g * n1 + s))):
                    xa[1, 0:L, k * DB + c * 128:k * DB + (c + 1) * 128] += v
        loop(0, G, first_out, "z_first_o")
        nxt, res = single_io(0, 0)
        run(sum(nxt, []))
        for c in range(KD):
            finish_cols(c, [xa[1, 0:L, k * DB + c * 128:k * DB + (c + 1) * 128] for k in range(NB)], res)

        def chunk(c):
            edge = (c == 0) | (c == nch)
            w0 = jnp.where(c < nch, 0, 1)

            @pl.when(edge)
            def _():
                @pl.when(c == nch)
                def _():
                    run(sum(tok_head(None, 0), mem_head(1)))
                loop(1 - w0, d, lambda i: a_step(1, i // d, b_head(w0, (i + d - 1) % d),
                                                 *single_io(w0, i)), "z_single")
                run(b_head(w0, d - 1))

                @pl.when(c == 0)
                def _():
                    for cps, wt, step in zip(b_cps, (wg, wu, wd), (8, 8, 16)):
                        with scope("z_waitb"):
                            wait(cps)
                        prep_rows(wt, step)
                    x_cps[1].wait()

            @pl.when(jnp.logical_not(edge))
            def _():
                loop(0, d, lambda i: a_dual(c, i), "z_dual")
                with scope("z_bhead"):
                    run(b_head(0, d - 1) + b_head(1, d - 1))

            @pl.when(c >= 2)
            def _():
                y_copy(c - 2).wait()
            loop(w0, jnp.where(c > 0, 2, 1), lambda w: b_step(c, w), "z_b")

            @pl.when(c == 0)
            def _():
                run(a_head(1))

            @pl.when(c >= 1)
            def _():
                y_copy(c - 1).start()
        loop(0, nch + 1, chunk, "z_chunk")
        y_copy(nch - 1).wait()

    any_spec = pl.BlockSpec(memory_space=pl.ANY)
    V = pltpu.VMEM
    return pl.pallas_call(
        kern,
        out_shape=jax.ShapeDtypeStruct((S, D), BF16),
        in_specs=[any_spec, pl.BlockSpec(memory_space=pltpu.VMEM)] + [any_spec] * 7,
        out_specs=any_spec,
        scratch_shapes=[
            V((S, D), BF16), V((G, 3, NR, DB // 2, E), U32), V((NR, G, E // 2, DB), U32),
            V((NR, DB // 2, FB), U32), V((NR, DB // 2, FB), U32), V((NR, FB // 2, DB), U32),
            V((2, M, D), F32), V((NR * KD, L, 128), F32), V((NR * KD, T, 128), F32), V((max(2 * NR * KD, G * len(_ACTIVE[1])), C2, 128), F32),
            V((2, C, D), F32), V((2, C, D), F32), V((C, D), BF16),
            pltpu.SemaphoreType.DMA((G,)), pltpu.SemaphoreType.DMA((G,)),
            pltpu.SemaphoreType.DMA((5,)), pltpu.SemaphoreType.DMA((1,)),
        ] + [V((FN, C2, 128), F32)] * (max(KF, G) * FS),
        compiler_params=pltpu.CompilerParams(vmem_limit_bytes=126 * 2**20, flags=cfg.get("flags")),
    )


@functools.partial(jax.jit, static_argnames=("A_seg_len",))
def pallas_interleave_layers__memory_aug_recurrent_mem_tr__glu_gated_glu__prompt_kernel(
        A_x, A_mem0, A_Wq, A_Wk, A_Wv, A_Wo, A_seg_len, B_x, B_w_gate, B_w_up, B_w_down):
    del B_x
    B, S, D = A_x.shape
    H, E = A_Wq.shape[1:]
    M = A_mem0.shape[1]
    F = B_w_gate.shape[1]
    call = build(S, D, H, E, M, int(A_seg_len), F, CFG)
    qkv = [w.reshape(NB, D // (2 * NB), 2, H, E) for w in (A_Wq, A_Wk, A_Wv)]
    out = call(A_x.reshape(S, D), A_mem0.reshape(M, D), *qkv, A_Wo.reshape(H // NB, NB, E, D),
               B_w_gate.reshape(NB, D // NB, F), B_w_up.reshape(NB, D // NB, F),
               B_w_down.reshape(NB, F // NB, D))
    return out.reshape(B, S, D)
```

```python
import collections
import contextlib
import functools

import jax
import jax.experimental.pallas as pl
import jax.experimental.pallas.tpu as pltpu
import jax.numpy as jnp
import numpy as np

F32, BF16, U32 = jnp.float32, jnp.bfloat16, jnp.uint32
CFG = dict(d=4, so=1, po=2, kc=[6, 2], kf=5, bg_mlp=(52, 30), bg_tok=(8, 30), bg_head=(8, 8), ahead=2)

_SCHEME = (
    '+000+000 ++000000+0000000 0000+000', '+0000000 +0+0+00000000000 +000-000',
    '0+000+00 0000++0+0+000000 0+000000', '00000+00 0-000-+000000-00 0+000-00',
    '+-000000 0000-00000000000 +-000000', '0000+-00 0-00000000000000 0000+-00',
    '+0000+00 0-00+00000000000 0-00+000', '0+-00+-0 000000000-000000 00000++0',
    '0+-00000 000000+000000000 0++00--0', '0+-00+00 000000-00-000000 0+000--0',
    '0+0-0000 0000000-00000000 0+0-0000', '00000+0- 0000000000000-00 00000+0-',
    '000+0+00 0000000-00000+00 0+00000-', '00+00000 000+00+0+0++0000 00+00000',
    '000000+0 00+000000-+0-0-0 000000+0', '+0-0+0-0 000-0000-0000000 +0-00000',
    '0000+0-0 00+000000000+000 +0-0-0+0', '+000+0-0 00-00000+0000000 +0-0-000',
    '+0-+0000 000+000000000000 +0-+0000', '0000+0-+ 000000000000+000 0000+0-+',
    '000-+0-0 000+00000000-000 +0-0000+', '000+000+ 000-0000000--+0+ 0000000+',
    '000+0000 000-000+0000+0++ 000+000-', '00++00++ 000-0000000-0000 00+-0000',
    '000000++ 000000000000-0-0 00+-00-+', '000+00++ 000+0000000++0+0 00+-000+',
)
NB = 4
NR = len(_SCHEME)
_U, _V, _W = (np.array([["-0+".index(ch) - 1 for ch in row.split()[k]] for row in _SCHEME]) for k in range(3))
for _r in range(NR):
    if _V[_r][np.flatnonzero(_V[_r])[0]] < 0:
        _V[_r], _W[_r] = -_V[_r], -_W[_r]
assert (np.einsum("ra,rb,rc->abc", _U, _V, _W).reshape(2, NB, NB, NB, 2, NB)
        == np.einsum("st,jk,il->sjkitl", np.eye(2), np.eye(NB), np.eye(NB))).all()
_ACTIVE = {2: list(range(NR)), 1: [r for r in range(NR) if _U[r, :NB].any() and _W[r, :NB].any()]}


_ORDER_OUT = list(range(NR - 1, -1, -1))
_ORDER_MLP = [4, 5, 6, 7, 8, 9, 10, 11, 12, 2, 3, 15, 16, 17, 18, 19, 20, 0, 1, 23, 24, 25, 13, 14, 21, 22]


def _combine(coef, xs):
    xs = list(xs)
    rows = [{k: int(c) for k, c in enumerate(row) if c} for row in coef]
    while True:
        count = collections.Counter((a, b, row[a] * row[b]) for row in rows for a in row for b in row if a < b)
        if not count or max(count.values()) < 2:
            break
        a, b, s = max(count, key=count.get)
        xs.append(xs[a] + xs[b] if s > 0 else xs[a] - xs[b])
        for row in rows:
            if a in row and b in row and row[a] * row[b] == s:
                row[len(xs) - 1] = row.pop(a)
                del row[b]
    out = []
    for row in rows:
        terms = sorted(row.items(), key=lambda t: -t[1])
        acc = xs[terms[0][0]] if terms[0][1] > 0 else -xs[terms[0][0]]
        for k, c in terms[1:]:
            acc = acc + xs[k] if c > 0 else acc - xs[k]
        out.append(acc)
    return out


def _left(blocks):
    act = _ACTIVE[len(blocks) // NB]
    return list(enumerate(_combine(_U[act, :len(blocks)], blocks)))


def _block_matmul(halves, lhs, rhs, outs=None, order=None):
    outs = [(1, o) for o in outs] if outs else [None] * (halves * NB)
    todo = list(enumerate(_ACTIVE[halves]))
    for slot, r in sorted(todo, key=lambda t: order.index(t[1])) if order else todo:
        m = _dot(lhs(slot), rhs(r))
        for k, c in enumerate(_W[r, :len(outs)]):
            if c and outs[k] is None:
                outs[k] = (c, m)
            elif c:
                s, acc = outs[k]
                outs[k] = (s, acc + m) if s == c else (1, acc - m) if s > 0 else (1, m - acc)
    return [acc if s > 0 else -acc for s, acc in outs]


def _ln(x):
    m = jnp.mean(x, axis=-1, keepdims=True)
    c = x - m
    v = jnp.mean(c * c, axis=-1, keepdims=True)
    return c * jax.lax.rsqrt(v + 1e-5)


def _sigmoid(x):
    return 0.5 * jnp.tanh(0.5 * x) + 0.5


def _dot(a, b):
    return jax.lax.dot_general(a, b, (((1,), (0,)), ((), ())), preferred_element_type=F32)


def _dot_nt(a, b):
    return jax.lax.dot_general(a, b, (((1,), (1,)), ((), ())), preferred_element_type=F32)


def _lo(w):
    return pltpu.bitcast(w << 16, F32)


def _hi(w):
    return pltpu.bitcast(w & np.uint32(0xFFFF0000), F32)


def _pack(lo, hi):
    return pltpu.bitcast(pltpu.pack_elementwise([lo, hi], packed_dtype=BF16), U32)


def _bf(w):
    return pltpu.bitcast(w, BF16)


def _cols(x):
    n = x.shape[1] // NB
    return [x[:, k * n:(k + 1) * n] for k in range(NB)]


def build(S, D, H, E, M, T, F, cfg):
    d = cfg["d"]
    nseg = S // T
    nch = nseg // d
    C, L, G = d * T, M + T, H // NB
    C2, T2, DB, FB = C // 2, T // 2, D // NB, F // NB
    KD, KF = DB // 128, FB // 128
    scale = float(E) ** -0.5
    scope = jax.named_scope if cfg.get("prof") else (lambda n: contextlib.nullcontext())

    def loop(lo, hi, fn, name):
        def body(i, carry):
            with scope(name):
                fn(i)
            return carry
        jax.lax.fori_loop(lo, hi, body, 0)

    def kern(x_hbm, mem_ref, wq, wk, wv, wo_hbm, wg_hbm, wu_hbm, wd_hbm, out_hbm,
             xs, wqkv, wo, wg, wu, wd, mem, ha, ba, xa, xb, yb, qsem, osem, wsem, ysem, *fa):
        kn = [(k, n) for k in range(NB) for n in range(NB)]

        def qkv_copies(g):
            return [pltpu.make_async_copy(w.bitcast(U32).at[:, :, par, 2 * g + p, :],
                                          wqkv.at[g, m, pl.ds((2 * p + par) * NB, NB)], qsem.at[g])
                    for m, w in enumerate((wq, wk, wv)) for p in range(2) for par in range(2)]

        def wo_copies(g):
            return [pltpu.make_async_copy(wo_hbm.bitcast(U32).at[g, :, :, pl.ds(n * DB, DB)],
                                          wo.at[pl.ds(n * NB, NB), g], osem.at[g]) for n in range(NB)]

        def b_copies(src, dst, i):
            nc = dst.shape[2]
            return [pltpu.make_async_copy(src.bitcast(U32).at[:, :, pl.ds(n * nc, nc)],
                                          dst.at[pl.ds(n * NB, NB)], wsem.at[i]) for n in range(NB)]
        b_cps = [b_copies(wg_hbm, wg, 0), b_copies(wu_hbm, wu, 1), b_copies(wd_hbm, wd, 2)]
        x_cps = [pltpu.make_async_copy(x_hbm.at[0:2 * C], xs.at[0:2 * C], wsem.at[3]),
                 pltpu.make_async_copy(x_hbm.at[2 * C:S], xs.at[2 * C:S], wsem.at[4])]

        def start(cps):
            for cp in cps:
                cp.start()

        def wait(cps):
            for cp in cps:
                cp.wait()

        def prep_qkv(g, m, rows):
            raw = [wqkv[g, m, s, rows, :] for s in range(NB * NB)]
            ev, od = (_combine(_V, [(_hi if n % 2 else _lo)(raw[(n // 2 * 2 + par) * NB + k]) for k, n in kn])
                      for par in range(2))
            for r in range(NR):
                wqkv[g, m, r, rows, :] = _pack(ev[r], od[r])

        def prep(w, idx):
            raw = [w[(n * NB + k,) + idx] for k, n in kn]
            lo, hi = (_combine(_V, [f(v) for v in raw]) for f in (_lo, _hi))
            for r in range(NR):
                one = np.flatnonzero(_V[r])
                w[(r,) + idx] = raw[one[0]] if len(one) == 1 else _pack(lo[r], hi[r])

        def prep_rows(w, step):
            def body(i):
                for r in range(0, step, 8):
                    for c in range(0, w.shape[2], 128):
                        prep(w, (pl.ds(pl.multiple_of(i * step + r, 8), 8), slice(c, c + 128)))
            loop(0, w.shape[1] // step, body, "z_prepb")

        def get(tiles, nrows, after=None):
            ts = [ref[t, 0:nrows, :] for ref, t in tiles]
            if after is not None:
                head = jnp.where(after[0] == 0, ts[0][0:8], after[1])
                ts[0] = jnp.concatenate([head, ts[0][8:]], axis=0)
            return jnp.concatenate(ts, axis=1)

        def pieces(ref, t0, rows, load):
            cache = []

            def step(k):
                if not cache:
                    cache.extend(b for x in load() for b in _cols(x))
                for s, v in _left([b[:, k * 128:(k + 1) * 128] for b in cache]):
                    ref[t0 + s * KD + k, rows, :] = v
            return [(functools.partial(step, k), ref) for k in range(KD)]

        def run(steps):
            for step, _ in steps:
                step()

        class Background:
            def __init__(self, zero):
                self.zero, self.queue, self.wait, self.period = zero, [], 0, 1

            def add(self, steps, period, delay):
                self.queue += steps
                self.period, self.wait = period, delay

            def __call__(self):
                self.wait -= 1
                if not self.queue or self.wait > 0:
                    return None
                self.wait = self.period
                step, ref = self.queue.pop(0)
                step()
                return self.zero, ref[self.zero, 0:8, :]

        mrows = slice(0, M)

        def mem_head(*ws):
            return pieces(ha, 0, mrows, lambda: [mem[w] for w in ws])

        def tok_head(t, i):
            def load(r):
                second = _ln(xb[0, pl.ds(pl.multiple_of(i * T + r, 16), 16), :])
                if t is None:
                    return [second]
                return [_ln(xs[pl.ds(pl.multiple_of(t * T + r, 16), 16), :].astype(F32)), second]
            return [p for r in range(0, T, 16)
                    for p in pieces(ha, 0, slice(M + r, M + r + 16), functools.partial(load, r))]

        def attn_masks():
            r = jax.lax.broadcasted_iota(jnp.int32, (2 * L, 128), 0)
            k = jax.lax.broadcasted_iota(jnp.int32, (2 * L, 128), 1)
            rp = jnp.where(r < L, r, r - L)
            kp = k // 2
            same = (kp < L) & (k % 2 == jnp.where(r < L, 0, 1))
            valid = same & ((rp < M) | (rp >= kp))
            return valid, jnp.where(same, -1e9, -jnp.inf).astype(F32)

        def proj(g, m, halves, bg=lambda: None):
            c = _block_matmul(halves, lambda s: get([(ha, s * KD + k) for k in range(KD)], L, bg()), lambda r: _bf(wqkv[g, m, r]))
            n = len(c) // 2
            if m == 0:
                return [jnp.concatenate([c[k], c[k + n]], axis=0) * scale for k in range(n)]
            z = jnp.zeros((64 - L, E), U32)
            return [_bf(jnp.concatenate([_pack(c[k], c[k + n]), z], axis=0)) for k in range(n)]

        def probs(qs, ks, masks):
            res = []
            for q, k in zip(qs, ks):
                s = jnp.where(masks[0], _dot_nt(q, k), masks[1])
                p = jnp.exp(s - jnp.max(s, axis=-1, keepdims=True))
                l = jnp.sum(p, axis=-1, keepdims=True)
                r = pl.reciprocal(l, approx=True)
                res.append(p * (r * (2.0 - l * r)))
            return res

        def mix(tile, ps, vs):
            o = [_dot(p, v) for p, v in zip(ps, vs)]
            for s, v in _left([y[:L] for y in o] + [y[L:] for y in o]):
                ref, t = tile(s)
                ref[t, 0:L, :] = v

        def out_proj(g0, n, c, halves, tile, acc=None, bg=lambda: None):
            return _block_matmul(halves, lambda s: get([tile(k, s) for k in range(n)], L, bg()),
                                 lambda r: _bf(wo[r, pl.ds(g0, n), :, c * 128:(c + 1) * 128].reshape(n * E // 2, 128)),
                                 acc, _ORDER_OUT)

        def finish_cols(c, y, residual):
            for s, v in _left([b[:M] for b in y]):
                ha[s * KD + c, mrows, :] = v
            for k, b in enumerate(y):
                cols = slice((k % NB) * DB + c * 128, (k % NB) * DB + (c + 1) * 128)
                mem[k // NB, :, cols] = b[:M]
                residual(k // NB, cols, b[M:])

        def a_step(halves, zero, mlp_input, next_tokens, residual):
            masks = attn_masks()
            so, po, kc = cfg["so"], cfg["po"], cfg["kc"]
            pr, ps, acc = {}, {}, {}
            side = sorted([(3 * g + 1 + so, 1, g) for g in range(G)] + [(3 * g + 1 + so + po, 0, g) for g in range(G)])

            def run_side(now):
                while side and side[0][0] <= now:
                    _, scores, g = side.pop(0)
                    if scores:
                        ps[g] = probs(pr[g, 0], pr[g, 1], masks)
                    else:
                        mix(lambda s: (fa[g], s), ps[g], pr[g, 2])
            bg = Background(zero)
            bg.add(mlp_input, *cfg["bg_mlp"])
            for g in range(G):
                for m in range(3):
                    pr[g, m] = proj(g, m, halves, bg)
                    run_side(3 * g + m)
            bg.add(next_tokens, *cfg["bg_tok"])
            now = 3 * G - 1
            for g0, n in zip(np.cumsum([0] + kc[:-1]).tolist(), kc):
                for c in range(KD):
                    assert all(g >= g0 + n for _, _, g in side)
                    acc[c] = out_proj(g0, n, c, halves, lambda k, s: (fa[g0 + k], s), acc.get(c), bg)
                    if g0 + n == G:
                        finish_cols(c, acc[c], residual)
                    now += 2
                    run_side(now)
            run(bg.queue)

        def a_dual(c, i):
            t = c * d + i
            rows = pl.ds(pl.multiple_of(i * T, T), T)
            xrows = pl.ds(pl.multiple_of(t * T, T), T)

            def residual(layer, cols, v):
                xa[layer, rows, cols] = v + (xb[0, rows, cols] if layer else xs[xrows, cols].astype(F32))
            a_step(2, i // d, b_head(0, (i + d - 1) % d) + b_head(1, (i + d - 1) % d),
                   tok_head(jnp.minimum(t + 1, nseg - 1), jnp.minimum(i + 1, d - 1)), residual)

        def single_io(w, i):
            rows = pl.ds(pl.multiple_of(i * T, T), T)

            def residual(layer, cols, v):
                xa[w, rows, cols] = v + xb[0, rows, cols]
            return tok_head(None, jnp.minimum(i + 1, d - 1)), residual

        def a_head(c):
            return mem_head(0, 1) + tok_head(jnp.minimum(c * d, nseg - 1), 0)

        def b_head(w, i):
            def load(r):
                return [_ln(xa[w, pl.ds(pl.multiple_of(i * T + h + r, 8), 8), :]) for h in (0, T2)]
            return [p for r in range(0, T2, 8)
                    for p in pieces(ba, w * NR * KD, pl.ds(pl.multiple_of(i * T2 + r, 8), 8), functools.partial(load, r))]

        def b_step(c, w):
            bg = Background(w // 2)
            bg.add(a_head(c + 1), *cfg["bg_head"])
            for n in range(KF):
                cols = slice(n * 128, (n + 1) * 128)
                g = _block_matmul(2, lambda s: get([(ba, (w * NR + s) * KD + k) for k in range(KD)], C2, bg()), lambda r: _bf(wg[r, :, cols]),
                                  order=_ORDER_MLP)
                g = [_sigmoid(v) for v in g]
                u = _block_matmul(2, lambda s: get([(ba, (w * NR + s) * KD + k) for k in range(KD)], C2, bg()), lambda r: _bf(wu[r, :, cols]),
                                  order=_ORDER_MLP)
                h = [gg * uu for gg, uu in zip(g, u)]
                run(bg.queue)
                bg.queue.clear()
                for r in range(0, C2, 8):
                    for s, v in _left([b[r:r + 8] for b in h]):
                        fa[n][s, r:r + 8, :] = v
            kf = cfg["kf"]

            def down(k0, nk, n, acc=None):
                return _block_matmul(2, lambda s: get([(fa[k0 + k], s) for k in range(nk)], C2),
                                     lambda r: _bf(wd[r, k0 * 64:(k0 + nk) * 64, n * 128:(n + 1) * 128]), acc)
            first = down(0, kf, 0)
            for n in range(KD):
                y = down(0, KF, n) if n else down(kf, KF - kf, 0, first)
                for k, v in enumerate(y):
                    cols = slice((k % NB) * DB + n * 128, (k % NB) * DB + (n + 1) * 128)
                    for i in range(d):
                        rows = slice(i * T + (k // NB) * T2, i * T + (k // NB + 1) * T2)
                        r = v[i * T2:(i + 1) * T2] + xa[w, rows, cols]
                        xb[w, rows, cols] = r
                        yb[rows, cols] = r.astype(BF16)

        def y_copy(c):
            return pltpu.make_async_copy(yb, out_hbm.at[pl.ds(pl.multiple_of(c * C, C), C), :], ysem.at[0])

        ahead, n1 = cfg["ahead"], len(_ACTIVE[1])
        with scope("z_head"):
            x_cps[0].start()
            for g in range(ahead):
                start(qkv_copies(g))
            x_cps[0].wait()
            xb[0] = xs[0:C, :].astype(F32)
            mem[1] = mem_ref[...].astype(F32)
            run(mem_head(1) + tok_head(None, 0))
            xa[1] = jnp.zeros((C, D), F32)
            ba[...] = jnp.zeros(ba.shape, F32)
            ha[len(_ACTIVE[1]) * KD:] = jnp.zeros(((NR - len(_ACTIVE[1])) * KD, L, 128), F32)

        def first_qkv(g):
            @pl.when(g + ahead < G)
            def _():
                start(qkv_copies(g + ahead))

            @pl.when(g + ahead == G)
            def _():
                for g2 in range(G):
                    start(wo_copies(g2))
            wait(qkv_copies(g))

            def rows(i):
                for m in range(3):
                    for r in range(0, 16, 8):
                        prep_qkv(g, m, pl.ds(pl.multiple_of(i * 16 + r, 8), 8))
            loop(0, DB // 32, rows, "y_pq")
            mix(lambda s: (ba, g * n1 + s), probs(proj(g, 0, 1), proj(g, 1, 1), attn_masks()), proj(g, 2, 1))
        loop(0, G, first_qkv, "z_first")
        start(b_cps[0] + b_cps[1] + b_cps[2])

        def first_out(g):
            wait(wo_copies(g))

            def rows(i):
                for c in range(KD):
                    prep(wo, (g, pl.ds(pl.multiple_of(i * 8, 8), 8), slice(c * 128, (c + 1) * 128)))
            loop(0, E // 16, rows, "y_po")
            for c in range(KD):
                for k, v in enumerate(out_proj(g, 1, c, 1, lambda k, s: (ba, g * n1 + s))):
                    xa[1, 0:L, k * DB + c * 128:k * DB + (c + 1) * 128] += v
        loop(0, G, first_out, "z_first_o")
        nxt, res = single_io(0, 0)
        run(nxt)
        for c in range(KD):
            finish_cols(c, [xa[1, 0:L, k * DB + c * 128:k * DB + (c + 1) * 128] for k in range(NB)], res)

        def chunk(c):
            edge = (c == 0) | (c == nch)
            w0 = jnp.where(c < nch, 0, 1)

            @pl.when(edge)
            def _():
                @pl.when(c == nch)
                def _():
                    run(mem_head(1) + tok_head(None, 0))
                loop(1 - w0, d, lambda i: a_step(1, i // d, b_head(w0, (i + d - 1) % d),
                                                 *single_io(w0, i)), "z_single")
                run(b_head(w0, d - 1))

                @pl.when(c == 0)
                def _():
                    for cps, wt, step in zip(b_cps, (wg, wu, wd), (8, 8, 16)):
                        with scope("z_waitb"):
                            wait(cps)
                        prep_rows(wt, step)
                    x_cps[1].start()

            @pl.when(jnp.logical_not(edge))
            def _():
                loop(0, d, lambda i: a_dual(c, i), "z_dual")
                with scope("z_bhead"):
                    run(b_head(0, d - 1) + b_head(1, d - 1))

            @pl.when(c >= 2)
            def _():
                y_copy(c - 2).wait()
            loop(w0, jnp.where(c > 0, 2, 1), lambda w: b_step(c, w), "z_b")

            @pl.when(c == 0)
            def _():
                run(a_head(1))
                x_cps[1].wait()

            @pl.when(c >= 1)
            def _():
                y_copy(c - 1).start()
        loop(0, nch + 1, chunk, "z_chunk")
        y_copy(nch - 1).wait()

    any_spec = pl.BlockSpec(memory_space=pl.ANY)
    V = pltpu.VMEM
    return pl.pallas_call(
        kern,
        out_shape=jax.ShapeDtypeStruct((S, D), BF16),
        in_specs=[any_spec, pl.BlockSpec(memory_space=pltpu.VMEM)] + [any_spec] * 7,
        out_specs=any_spec,
        scratch_shapes=[
            V((S, D), BF16), V((G, 3, NR, DB // 2, E), U32), V((NR, G, E // 2, DB), U32),
            V((NR, DB // 2, FB), U32), V((NR, DB // 2, FB), U32), V((NR, FB // 2, DB), U32),
            V((2, M, D), F32), V((NR * KD, L, 128), F32), V((max(2 * NR * KD, G * len(_ACTIVE[1])), C2, 128), F32),
            V((2, C, D), F32), V((2, C, D), F32), V((C, D), BF16),
            pltpu.SemaphoreType.DMA((G,)), pltpu.SemaphoreType.DMA((G,)),
            pltpu.SemaphoreType.DMA((5,)), pltpu.SemaphoreType.DMA((1,)),
        ] + [V((NR, C2, 128), F32)] * max(KF, G),
        compiler_params=pltpu.CompilerParams(vmem_limit_bytes=126 * 2**20),
    )


@functools.partial(jax.jit, static_argnames=("A_seg_len",))
def pallas_interleave_layers__memory_aug_recurrent_mem_tr__glu_gated_glu__prompt_kernel(
        A_x, A_mem0, A_Wq, A_Wk, A_Wv, A_Wo, A_seg_len, B_x, B_w_gate, B_w_up, B_w_down):
    del B_x
    B, S, D = A_x.shape
    H, E = A_Wq.shape[1:]
    M = A_mem0.shape[1]
    F = B_w_gate.shape[1]
    call = build(S, D, H, E, M, int(A_seg_len), F, CFG)
    qkv = [w.reshape(NB, D // (2 * NB), 2, H, E) for w in (A_Wq, A_Wk, A_Wv)]
    out = call(A_x.reshape(S, D), A_mem0.reshape(M, D), *qkv, A_Wo.reshape(H // NB, NB, E, D),
               B_w_gate.reshape(NB, D // NB, F), B_w_up.reshape(NB, D // NB, F),
               B_w_down.reshape(NB, F // NB, D))
    return out.reshape(B, S, D)
```

```python
import collections
import contextlib
import functools

import jax
import jax.experimental.pallas as pl
import jax.experimental.pallas.tpu as pltpu
import jax.numpy as jnp
import numpy as np

F32, BF16, U32 = jnp.float32, jnp.bfloat16, jnp.uint32
CFG = dict(d=4, so=60, po=150, kc=[3, 1], bg_mlp=(60, 320), bg_tok=(10, 10), bg_head=(30, 220), rb=1, rev=-1)


class _Scheme:
    def __init__(self, nb, rows):
        self.nb, self.n = nb, len(rows)
        self.u, self.v, self.w = (np.zeros((self.n, size), np.int64) for size in (2 * nb, nb * nb, 2 * nb))
        for r, row in enumerate(rows):
            for coef, text in zip((self.u, self.v, self.w), row.split()):
                for k in range(0, len(text), 3):
                    coef[r, int(text[k + 1:k + 3])] = 1 if text[k] == "+" else -1
            if self.v[r][np.flatnonzero(self.v[r])[0]] < 0:
                self.v[r], self.w[r] = -self.v[r], -self.w[r]
        assert (np.einsum("ra,rb,rc->abc", self.u, self.v, self.w).reshape(2, nb, nb, nb, 2, nb)
                == np.einsum("st,jk,il->sjkitl", np.eye(2), np.eye(nb), np.eye(nb))).all()
        self.active = {2: list(range(self.n)),
                       1: [r for r in range(self.n) if self.u[r, :nb].any() and self.w[r, :nb].any()]}


_S4 = _Scheme(4, (
    '+00+04 +00+01+08 +04', '+00 +00+02+04 +00-04', '+01+05 +04+05+07+09 +01', '+05 -01-05+06-13 +01-05',
    '+00-01 -04 +00-01', '+04-05 -01 +04-05', '+00+05 -01+04 -01+04', '+01-02+05-06 -09 +05+06',
    '+01-02 +06 +01+02-05-06', '+01-02+05 -06-09 +01-05-06', '+01-03 -07 +01-03', '+05-07 -13 +05-07',
    '+03+05 -07+13 +01-07', '+02 +03+06+08+10+11 +02', '+06 +02-09+10-12-14 +06', '+00-02+04-06 -03-08 +00-02',
    '+04-06 +02+12 +00-02-04+06', '+00+04-06 -02+08 +00-02-04', '+00-02+03 +03 +00-02+03', '+04-06+07 +12 +04-06+07',
    '-03+04-06 +03-12 +00-02+07', '+03+07 -03-11-12+13+15 +07', '+03 -03+07+12+14+15 +03-07',
    '+02+03+06+07 -03-11 +02-03', '+06+07 -12-14 +02-03-06+07', '+03+06+07 +03+11+12+14 +02-03+07',
))
_S8 = _Scheme(8, (
    '+00+08 +00-01-04+06-07+16-33-40+48 +08', '+00 +00-02+05-06-08+12+32-48-56 +00-08', '+00+01 +08-12 +00+01',
    '+08+09 +01+33 +08+09', '+00-09 +01-08+12+33 +01+08', '+00-02+08-10 -16 +00+02', '+08-10 -02 +00+02-08-10',
    '+00+08-10 +02+16 +00+02-08', '+00+03-04+08+11-12 -03 +00-03+04', '+08+11-12 -24 +00-03+04-08+11-12',
    '+03+08+11-12 +03+24 +00-03+04+11', '+00-04 +03+12-32 +00+04', '+08-12 +04-24-33 +08+12', '+00+12 +04+32 +04+08',
    '+00+05+08+13 +40 +00-05', '+08+13 +05 +00-05-08+13', '+00+08+13 -05-40 +00-05-08',
    '-00+06-07-08+14-15 +48 +00+06+07', '-08+14-15 +06 +00+06+07-08-14-15', '-00-08+14-15 -06-48 +00+06+07-08',
    '+00+07 +48+56 +00+07', '+08+15 -06+07 +08+15', '+00-15 -06+07-48-56 +07+08',
    '+01+09 -08+09-11+12-14+15-17-33-41+57 +01', '+09 +01-09-10-12-13+15-25+33-49-57 +01-09',
    '+01+02+09+10 +17 +09-10', '+01+02 -10 +01-02-09+10', '+01+02+09 +10+17 +01-09+10', '+01-03 +11 +01+03',
    '+09-11 -25 +09+11', '+03+09 +11+25 +01+11', '+00-01-04+08-09-12 +33 +08-09+12',
    '+00-01-04 -12 +00-01+04-08+09-12', '+00-01-04-09 -12-33 +01+08-09+12', '+01+05+09+13 +41 +09-13',
    '+01+05 -13 +01-05-09+13', '+01+05+09 +13+41 +01-09+13', '+01-06 +14-15 +01+06', '+09-14 -49-57 +09+14',
    '+06+09 +14-15+49+57 +01+14', '+01+06-07+09+14-15 -57 +09+14+15', '+01+06-07 +15 +01+06+07-09-14-15',
    '+01+06-07+09 +15+57 -01+09+14+15', '+02 -10-16+18+19+22+30+34+58 +02', '+10 +02+17+18+20+23+26+50+51 +10',
    '+02-03+10-11 -19-30-42 +02-03', '+10-11 -21+26+51 +02-03-10+11', '-03+10-11 +19-26 +02-03+11',
    '+02-04+10-12 -20 +10-12', '+02-04 -34 +02-04-10+12', '+02-04-12 +20-34 +04+10-12',
    '+02-03+05+10-11+13 +42 +10-11-13', '+02-03+05 -21 +02-03-05-10+11+13', '+02-03+05+10-11 +21+42 +02-03-10+11+13',
    '+02-06+10-14 -22-30 +02-06', '+10-14 +50+51 +02-06-10+14', '-06+10-14 +22+30-50-51 +02-06+14',
    '+02-07+10-15 -23 +10-15', '+02-07 -58 +02-07-10+15', '+02-07-15 +23-58 +07+10-15',
    '+03+11 -03+19-24-25+27+28-31-42-43 +11', '+03 +03+11+21+24+26+27+29+35-59 +03-11', '+03-04 -03-35 +03-04',
    '+11-12 +24-28 +11-12', '+03+12 +03+24-28+35 -04+11', '+03+05+11+13 +42+43 +03-05', '+11+13 +21+29 +03-05-11+13',
    '+03+11+13 -21-29-42-43 +03-05-11', '+02-03-06 +30 +02-03-06', '+10-11-14 +51 +10-11-14',
    '+06+10-11 +30-51 +02-03-14', '+03+07 +59 +03+07', '+11+15 +31 +11+15', '+03-15 +31-59 +07+11',
    '+04+12 +03+20-32+35+36-38-44 +04', '+12 -04+24-28-34-36-37-52 +04-12', '+04+05+12+13 -39+44 +12-13',
    '+04+05 -37+60 +04-05-12+13', '+04+05+12 +37+44 +04-12+13', '+04-06 +38 +04+06', '+12-14 -52 +12+14',
    '+06+12 +38+52 +04+14', '+04+05-07 -60 +04-05+07', '+12+13-15 +39 +12-13+15', '+04+05+15 +39+60 +07+12-13',
    '+05 -13-21-37+40+42+43+45-46+60+61 +05', '+13 -05-21-29-39+41+42+44+45+47+53 +13', '+05-06+13-14 +46 +05+06',
    '+13-14 +53 +05+06-13-14', '-06+13-14 -46-53 +05+06-14', '+05-07+13-15 +39-47 +13-15',
    '+05-07 -60-61 +05-07-13+15', '+05-07-15 -39+47-60-61 +07+13-15', '+06+14 +22+30+46-49-51-52+54-55-57 +14',
    '+06 +14-15-30+38+50+51-53+54+62 +06-14', '+06-07 -15-48-62 +06+07', '+14-15 +06+55+57 +14+15',
    '+06+15 +55+62 +07+14', '+07+15 +23-39+47-48-56-59-60-62+63 +07', '+15 -06+07+31-39-55-58-60-61-63 +07-15',
))
_ORDER_MLP = [4, 5, 6, 7, 8, 9, 10, 11, 12, 2, 3, 15, 16, 17, 18, 19, 20, 0, 1, 23, 24, 25, 13, 14, 21, 22]


def _combine(coef, xs):
    xs = list(xs)
    rows = [{k: int(c) for k, c in enumerate(row) if c} for row in coef]
    while True:
        count = collections.Counter((a, b, row[a] * row[b]) for row in rows for a in row for b in row if a < b)
        if not count or max(count.values()) < 2:
            break
        a, b, s = max(count, key=count.get)
        xs.append(xs[a] + xs[b] if s > 0 else xs[a] - xs[b])
        for row in rows:
            if a in row and b in row and row[a] * row[b] == s:
                row[len(xs) - 1] = row.pop(a)
                del row[b]
    out = []
    for row in rows:
        terms = sorted(row.items(), key=lambda t: -t[1])
        acc = xs[terms[0][0]] if terms[0][1] > 0 else -xs[terms[0][0]]
        for k, c in terms[1:]:
            acc = acc + xs[k] if c > 0 else acc - xs[k]
        out.append(acc)
    return out


def _left(sc, blocks):
    return list(enumerate(_combine(sc.u[sc.active[len(blocks) // sc.nb], :len(blocks)], blocks)))


def _block_matmul(sc, halves, lhs, rhs, outs=None, order=None):
    outs = [(1, o) for o in outs] if outs else [None] * (halves * sc.nb)
    todo = list(enumerate(sc.active[halves]))
    for slot, r in sorted(todo, key=lambda t: order.index(t[1])) if order else todo:
        m = _dot(lhs(slot), rhs(r))
        for k, c in enumerate(sc.w[r, :len(outs)]):
            if c and outs[k] is None:
                outs[k] = (c, m)
            elif c:
                s, acc = outs[k]
                outs[k] = (s, acc + m) if s == c else (1, acc - m) if s > 0 else (1, m - acc)
    return [acc if s > 0 else -acc for s, acc in outs]


def _ln(x):
    m = jnp.mean(x, axis=-1, keepdims=True)
    c = x - m
    v = jnp.mean(c * c, axis=-1, keepdims=True)
    return c * jax.lax.rsqrt(v + 1e-5)


def _sigmoid(x):
    return 0.5 * jnp.tanh(0.5 * x) + 0.5


def _dot(a, b):
    return jax.lax.dot_general(a, b, (((1,), (0,)), ((), ())), preferred_element_type=F32)


def _dot_nt(a, b):
    return jax.lax.dot_general(a, b, (((1,), (1,)), ((), ())), preferred_element_type=F32)


def _lo(w):
    return pltpu.bitcast(w << 16, F32)


def _hi(w):
    return pltpu.bitcast(w & np.uint32(0xFFFF0000), F32)


def _pack(lo, hi):
    return pltpu.bitcast(pltpu.pack_elementwise([lo, hi], packed_dtype=BF16), U32)


def _bf(w):
    return pltpu.bitcast(w, BF16)


def _cols(x, nb):
    n = x.shape[1] // nb
    return [x[:, k * n:(k + 1) * n] for k in range(nb)]


def build(S, D, H, E, M, T, F, cfg):
    d = cfg["d"]
    nseg = S // T
    nch = nseg // d
    sa, sb = _S8, _S4
    NA, NB = sa.nb, sb.nb
    NI = F // D
    assert D == NA * 128 and F == NI * D + NB * 128 and E == 128 and 2 * (M + T) <= 128
    C, L, G, DA = d * T, M + T, H // NA, D // NA
    KA, n1 = DA // 128, len(sa.active[1])
    C2, T2, DB = C // 2, T // 2, D // NB
    scale = float(E) ** -0.5
    scope = jax.named_scope if cfg.get("prof") else (lambda n: contextlib.nullcontext())

    def loop(lo, hi, fn, name):
        def body(i, carry):
            with scope(name):
                fn(i)
            return carry
        jax.lax.fori_loop(lo, hi, body, 0)

    def kern(x_hbm, mem_ref, wq, wk, wv, wo_hbm, wg_hbm, wu_hbm, wd_hbm, out_hbm,
             xs, wqkv, wo, wg, wu, wd, wg4, wu4, wd4, ha, ba, bn, xa, xb, yb, qsem, osem, wsem, ysem):
        def qkv_copies(g, m):
            return [pltpu.make_async_copy((wq, wk, wv)[m].bitcast(U32).at[:, :, par, NA // 2 * g + p, :],
                                          wqkv.at[g, m, pl.ds((2 * p + par) * NA, NA)], qsem.at[g, m])
                    for p in range(NA // 2) for par in range(2)]

        def wo_copies(g):
            return [pltpu.make_async_copy(wo_hbm.bitcast(U32).at[g, :, :, pl.ds(n * DA, DA)],
                                          wo.at[pl.ds(n * NA, NA), g], osem.at[g]) for n in range(NA)]

        def in_copies(src, dst, dst4, sem):
            src = src.bitcast(U32)
            return ([pltpu.make_async_copy(src.at[:, :, :, pl.ds((i * NA + n) * 128, 128)],
                                           dst.at[i, pl.ds(n * NA // 2, NA // 2)], sem)
                     for i in range(NI) for n in range(NA)]
                    + [pltpu.make_async_copy(src.at[:, :, :, pl.ds((NI * NA + n) * 128, 128)],
                                             dst4.at[pl.ds(n * NB, NB)], sem) for n in range(NB)])
        wd_src = wd_hbm.bitcast(U32)
        b_cps = [in_copies(wg_hbm, wg, wg4, wsem.at[0]), in_copies(wu_hbm, wu, wu4, wsem.at[1]),
                 [pltpu.make_async_copy(wd_src.at[pl.ds(i * NA, NA), :, pl.ds(n * 128, 128)],
                                        wd.at[i, pl.ds(n * NA, NA)], wsem.at[2]) for i in range(NI) for n in range(NA)]
                 + [pltpu.make_async_copy(wd_src.at[pl.ds(NI * NA, NB), :, pl.ds(n * DB, DB)],
                                          wd4.at[pl.ds(n * NB, NB)], wsem.at[2]) for n in range(NB)]]
        x_cps = [pltpu.make_async_copy(x_hbm.at[0:2 * C], xs.at[0:2 * C], wsem.at[3]),
                 pltpu.make_async_copy(x_hbm.at[2 * C:S], xs.at[2 * C:S], wsem.at[4])]

        def start(cps):
            for cp in cps:
                cp.start()

        def wait(cps):
            for cp in cps:
                cp.wait()

        def prep_qkv(g, m, rows):
            raw = [wqkv[g, m, s, rows, :] for s in range(NA * NA)]
            ev, od = (_combine(sa.v, [(_hi if n % 2 else _lo)(raw[(n // 2 * 2 + par) * NA + k])
                                      for k in range(NA) for n in range(NA)]) for par in range(2))
            for r in range(sa.n):
                wqkv[g, m, r, rows, :] = _pack(ev[r], od[r])

        def prep(sc, w, at):
            raw = [w[at(n * sc.nb + k)] for k in range(sc.nb) for n in range(sc.nb)]
            lo, hi = (_combine(sc.v, [f(v) for v in raw]) for f in (_lo, _hi))
            for r in range(sc.n):
                one = np.flatnonzero(sc.v[r])
                w[at(r)] = raw[one[0]] if len(one) == 1 else _pack(lo[r], hi[r])

        def rows8(i):
            return pl.ds(pl.multiple_of(i * 8, 8), 8)

        def prep_mlp(which):
            w, w4 = ((wg, wg4), (wu, wu4), (wd, wd4))[which]

            def big(t):
                i, rows = t // 8, rows8(t % 8)
                prep(sa, w, (lambda s: (i, s // 2, s % 2, rows)) if which < 2 else (lambda s: (i, s, rows)))

            def small(t):
                for h in range(2):
                    prep(sb, w4, (lambda s: (s, h, rows8(t))) if which < 2
                         else (lambda s: (s, rows8(t), slice(h * 128, (h + 1) * 128))))
            loop(0, NI * 8, big, "z_prepb")
            loop(0, 8, small, "z_prepb")

        def ordered(v, after):
            if after is None:
                return v
            return jnp.concatenate([jnp.where(after[0] == 0, v[0:8], after[1]), v[8:]], axis=0)

        def run(steps):
            for step, _ in steps:
                step()

        class Background:
            def __init__(self, zero):
                self.zero, self.queue, self.wait, self.period = zero, [], 0, 1

            def add(self, steps, period, delay):
                self.queue += steps
                self.period, self.wait = period, delay

            def __call__(self):
                self.wait -= 1
                if not self.queue or self.wait > 0:
                    return None
                self.wait = self.period
                step, ref = self.queue.pop(0)
                step()
                return self.zero, ref[self.zero, 0:8, 0:128]

        mrows = slice(0, M)

        def tok_head(t, i):
            def norm(w, r):
                if w == 0 and t is not None:
                    v = xs[pl.ds(pl.multiple_of(t * T + r, 8), 8), :].astype(F32)
                else:
                    v = xb[0, pl.ds(pl.multiple_of(i * T + r, 8), 8), :]
                ha[w, M + r:M + r + 8, :] = _ln(v)
            return [(functools.partial(norm, w, r), ha) for w in range(1 if t is None else 2) for r in range(0, T, 8)]

        def a_input(halves):
            return _left(sa, [b for w in range(halves) for b in _cols(ha[w], NA)])

        def attn_masks():
            r = jax.lax.broadcasted_iota(jnp.int32, (2 * L, 128), 0)
            k = jax.lax.broadcasted_iota(jnp.int32, (2 * L, 128), 1)
            rp = jnp.where(r < L, r, r - L)
            kp = k // 2
            same = (kp < L) & (k % 2 == jnp.where(r < L, 0, 1))
            valid = same & ((rp < M) | (rp >= kp))
            return valid, jnp.where(same, -1e9, -jnp.inf).astype(F32)

        def proj(h, g, m, halves, bg=lambda: None):
            c = _block_matmul(sa, halves, lambda s: ordered(h[s][1], bg()), lambda r: _bf(wqkv[g, m, r]))
            n = len(c) // 2
            if m == 0:
                return [jnp.concatenate([c[k], c[k + n]], axis=0) * scale for k in range(n)]
            z = jnp.zeros((64 - L, E), U32)
            return [_bf(jnp.concatenate([_pack(c[k], c[k + n]), z], axis=0)) for k in range(n)]

        def probs(qs, ks, masks):
            res = []
            for q, k in zip(qs, ks):
                s = jnp.where(masks[0], _dot_nt(q, k), masks[1])
                p = jnp.exp(s - jnp.max(s, axis=-1, keepdims=True))
                l = jnp.sum(p, axis=-1, keepdims=True)
                r = pl.reciprocal(l, approx=True)
                res.append(p * (r * (2.0 - l * r)))
            return res

        def mix(ps, vs):
            o = [_dot(p, v) for p, v in zip(ps, vs)]
            return _left(sa, [y[:L] for y in o] + [y[L:] for y in o])

        def out_proj(g0, n, c, halves, lhs, acc=None):
            return _block_matmul(sa, halves, lhs,
                                 lambda r: _bf(wo[r, pl.ds(g0, n), :, c * 128:(c + 1) * 128].reshape(n * E // 2, 128)),
                                 acc, list(range(sa.n))[::cfg["rev"]])

        def finish_cols(c, y, residual):
            for k, b in enumerate(y):
                cols = slice((k % NA) * DA + c * 128, (k % NA) * DA + (c + 1) * 128)
                ha[k // NA, mrows, cols] = b[:M]
                residual(k // NA, cols, b[M:])

        def a_step(halves, zero, mlp_input, next_tokens, residual):
            masks = attn_masks()
            so, po, kc = cfg["so"], cfg["po"], cfg["kc"]
            pr, ps, os_, acc, now = {}, {}, {}, {}, [0]
            span = len(sa.active[halves]) * KA
            side = sorted([((3 * g + 2) * span + so, 1, g) for g in range(G)]
                          + [((3 * g + 2) * span + so + po, 0, g) for g in range(G)])
            bg = Background(zero)

            def tick(tiles):
                while side and side[0][0] <= now[0]:
                    _, scores, g = side.pop(0)
                    if scores:
                        ps[g] = probs(pr[g, 0], pr[g, 1], masks)
                    else:
                        os_[g] = mix(ps[g], pr[g, 2])
                now[0] += tiles
                return bg()

            def out_lhs(g0, n, s):
                after = tick(n)
                assert all(g0 + k in os_ for k in range(n))
                return jnp.concatenate([ordered(os_[g0 + k][s][1], None if k else after) for k in range(n)], axis=1)
            h = a_input(halves)
            bg.add(mlp_input, *cfg["bg_mlp"])
            for g in range(G):
                for m in range(3):
                    pr[g, m] = proj(h, g, m, halves, lambda: tick(KA))
            bg.add(next_tokens, *cfg["bg_tok"])
            for g0, n in zip(np.cumsum([0] + kc[:-1]).tolist(), kc):
                for c in range(KA):
                    acc[c] = out_proj(g0, n, c, halves, functools.partial(out_lhs, g0, n), acc.get(c))
                    if g0 + n == G:
                        finish_cols(c, acc[c], residual)
            run(bg.queue)

        def a_dual(c, i):
            t = c * d + i
            rows = pl.ds(pl.multiple_of(i * T, T), T)
            xrows = pl.ds(pl.multiple_of(t * T, T), T)

            def residual(layer, cols, v):
                xa[layer, rows, cols] = v + (xb[0, rows, cols] if layer else xs[xrows, cols].astype(F32))
            a_step(2, i // d, b_head(0, (i + d - 1) % d) + b_head(1, (i + d - 1) % d),
                   tok_head(jnp.minimum(t + 1, nseg - 1), jnp.minimum(i + 1, d - 1)), residual)

        def single_io(w, i):
            rows = pl.ds(pl.multiple_of(i * T, T), T)

            def residual(layer, cols, v):
                xa[w, rows, cols] = v + xb[0, rows, cols]
            return tok_head(None, jnp.minimum(i + 1, d - 1)), residual

        def a_head(c):
            return tok_head(jnp.minimum(c * d, nseg - 1), 0)

        def b_head(w, i):
            def norm(h, r):
                v = xa[w, pl.ds(pl.multiple_of(i * T + h * T2 + r, 8), 8), :]
                bn[2 * w + h, pl.ds(pl.multiple_of(i * T2 + r, 8), 8), :] = _ln(v)
            return [(functools.partial(norm, h, r), bn) for h in range(2) for r in range(0, T2, 8)]

        def b_step(c, w):
            bg = Background(w // 2)
            bg.add(a_head(c + 1), *cfg["bg_head"])
            o8, o4 = list(range(sa.n))[::cfg["rb"]], _ORDER_MLP

            def gated(sc, lhs, rhs, order):
                g = [_sigmoid(v) for v in _block_matmul(sc, 2, lhs, functools.partial(rhs, 0), order=order)]
                u = _block_matmul(sc, 2, lhs, functools.partial(rhs, 1), order=order)
                return _left(sc, [gg * uu for gg, uu in zip(g, u)])
            a8 = _left(sa, [b for h in range(2) for b in _cols(bn[2 * w + h], NA)])
            hs = [gated(sa, lambda s: ordered(a8[s][1], bg()),
                        lambda m, r: _bf((wg, wu)[m][i, r // 2, r % 2]), o8) for i in range(NI)]
            run(bg.queue)
            a4 = _left(sb, [b for h in range(2) for b in _cols(bn[2 * w + h], NB)])
            h4 = gated(sb, lambda s: a4[s][1], lambda m, r: _bf((wg4, wu4)[m][r].reshape(DB // 2, 128)), o4)
            y = _block_matmul(sa, 2, lambda s: jnp.concatenate([h[s][1] for h in hs], axis=1),
                              lambda r: _bf(wd[:, r].reshape(NI * 64, 128)), order=o8)
            for n in range(2):
                z = _block_matmul(sb, 2, lambda s: h4[s][1], lambda r: _bf(wd4[r, :, n * 128:(n + 1) * 128]),
                                  y[n::2], o4)
                for k, v in enumerate(z):
                    cols = slice((k % NB) * DB + n * 128, (k % NB) * DB + (n + 1) * 128)
                    for i in range(d):
                        rows = slice(i * T + (k // NB) * T2, i * T + (k // NB + 1) * T2)
                        r = v[i * T2:(i + 1) * T2] + xa[w, rows, cols]
                        xb[w, rows, cols] = r
                        yb[rows, cols] = r.astype(BF16)

        def y_copy(c):
            return pltpu.make_async_copy(yb, out_hbm.at[pl.ds(pl.multiple_of(c * C, C), C), :], ysem.at[0])

        with scope("z_head"):
            x_cps[0].start()
            for m in range(3):
                start(qkv_copies(0, m))
            x_cps[0].wait()
            xb[0] = xs[0:C, :].astype(F32)
            ha[0, mrows, :] = mem_ref[...].astype(F32)
            ha[1, mrows, :] = mem_ref[...].astype(F32)
            run(tok_head(None, 0))
            xa[1] = jnp.zeros((C, D), F32)
            bn[...] = jnp.zeros(bn.shape, F32)

        def first_qkv(g):
            for m in range(3):
                @pl.when(g + 1 < G)
                def _():
                    start(qkv_copies(g + 1, m))

                @pl.when((g + 1 == G) & (m == 0))
                def _():
                    for g2 in range(G):
                        start(wo_copies(g2))
                wait(qkv_copies(g, m))
                loop(0, DA // 16, lambda i: prep_qkv(g, m, pl.ds(pl.multiple_of(i * 8, 8), 8)), "y_pq")
            h = a_input(1)
            for s, v in mix(probs(proj(h, g, 0, 1), proj(h, g, 1, 1), attn_masks()), proj(h, g, 2, 1)):
                ba[g * n1 + s] = v
        loop(0, G, first_qkv, "z_first")
        start(b_cps[0] + b_cps[1] + b_cps[2])

        def first_out(g):
            wait(wo_copies(g))

            def rows(i):
                for c in range(KA):
                    prep(sa, wo, lambda s: (s, g, rows8(i), slice(c * 128, (c + 1) * 128)))
            loop(0, E // 16, rows, "y_po")
            for c in range(KA):
                for k, v in enumerate(out_proj(g, 1, c, 1, lambda s: ba[g * n1 + s])):
                    xa[1, 0:L, k * DA + c * 128:k * DA + (c + 1) * 128] += v
        loop(0, G, first_out, "z_first_o")
        nxt, res = single_io(0, 0)
        run(nxt)
        for c in range(KA):
            finish_cols(c, [xa[1, 0:L, k * DA + c * 128:k * DA + (c + 1) * 128] for k in range(NA)], res)

        def chunk(c):
            edge = (c == 0) | (c == nch)
            w0 = jnp.where(c < nch, 0, 1)

            @pl.when(edge)
            def _():
                @pl.when(c == nch)
                def _():
                    ha[0, mrows, :] = ha[1, mrows, :]
                    run(tok_head(None, 0))
                loop(1 - w0, d, lambda i: a_step(1, i // d, b_head(w0, (i + d - 1) % d),
                                                 *single_io(w0, i)), "z_single")
                run(b_head(w0, d - 1))

                @pl.when(c == 0)
                def _():
                    for which, cps in enumerate(b_cps):
                        with scope("z_waitb"):
                            wait(cps)
                        prep_mlp(which)
                    x_cps[1].start()

            @pl.when(jnp.logical_not(edge))
            def _():
                loop(0, d, lambda i: a_dual(c, i), "z_dual")
                with scope("z_bhead"):
                    run(b_head(0, d - 1) + b_head(1, d - 1))

            @pl.when(c >= 2)
            def _():
                y_copy(c - 2).wait()
            loop(w0, jnp.where(c > 0, 2, 1), lambda w: b_step(c, w), "z_b")

            @pl.when(c == 0)
            def _():
                run(a_head(1))
                x_cps[1].wait()

            @pl.when(c >= 1)
            def _():
                y_copy(c - 1).start()
        loop(0, nch + 1, chunk, "z_chunk")
        y_copy(nch - 1).wait()

    any_spec = pl.BlockSpec(memory_space=pl.ANY)
    V = pltpu.VMEM
    return pl.pallas_call(
        kern,
        out_shape=jax.ShapeDtypeStruct((S, D), BF16),
        in_specs=[any_spec, pl.BlockSpec(memory_space=pltpu.VMEM)] + [any_spec] * 7,
        out_specs=any_spec,
        scratch_shapes=[
            V((S, D), BF16), V((G, 3, sa.n, DA // 2, E), U32), V((sa.n, G, E // 2, DA), U32),
            V((NI, sa.n // 2, 2, 64, 128), U32), V((NI, sa.n // 2, 2, 64, 128), U32), V((NI, sa.n, 64, 128), U32),
            V((sb.n, 2, 64, 128), U32), V((sb.n, 2, 64, 128), U32), V((sb.n, 64, DB), U32),
            V((2, L, D), F32), V((G * n1, L, 128), F32), V((4, C2, D), F32),            V((2, C, D), F32), V((2, C, D), F32), V((C, D), BF16),
            pltpu.SemaphoreType.DMA((G, 3)), pltpu.SemaphoreType.DMA((G,)),
            pltpu.SemaphoreType.DMA((5,)), pltpu.SemaphoreType.DMA((1,)),
        ],
        compiler_params=pltpu.CompilerParams(vmem_limit_bytes=126 * 2**20),
    )


@functools.partial(jax.jit, static_argnames=("A_seg_len",))
def pallas_interleave_layers__memory_aug_recurrent_mem_tr__glu_gated_glu__prompt_kernel(
        A_x, A_mem0, A_Wq, A_Wk, A_Wv, A_Wo, A_seg_len, B_x, B_w_gate, B_w_up, B_w_down):
    del B_x
    B, S, D = A_x.shape
    H, E = A_Wq.shape[1:]
    M = A_mem0.shape[1]
    F = B_w_gate.shape[1]
    call = build(S, D, H, E, M, int(A_seg_len), F, CFG)
    NA, NB = _S8.nb, _S4.nb
    qkv = [w.reshape(NA, D // (2 * NA), 2, H, E) for w in (A_Wq, A_Wk, A_Wv)]
    out = call(A_x.reshape(S, D), A_mem0.reshape(M, D), *qkv, A_Wo.reshape(H // NA, NA, E, D),
               B_w_gate.reshape(NB, 2, D // NA, F), B_w_up.reshape(NB, 2, D // NA, F),
               B_w_down.reshape(F // 128, 128, D))
    return out.reshape(B, S, D)
```

```python
import collections
import contextlib
import functools

import jax
import jax.experimental.pallas as pl
import jax.experimental.pallas.tpu as pltpu
import jax.numpy as jnp
import numpy as np

F32, BF16, U32 = jnp.float32, jnp.bfloat16, jnp.uint32
CFG = dict(d=4, so=60, po=150, kc=[3, 1], bg_mlp=(60, 320), bg_tok=(10, 10), bg_head=(30, 220), rb=1, rev=-1)


class _Scheme:
    def __init__(self, nb, rows):
        self.nb, self.n = nb, len(rows)
        self.u, self.v, self.w = (np.zeros((self.n, size), np.int64) for size in (2 * nb, nb * nb, 2 * nb))
        for r, row in enumerate(rows):
            for coef, text in zip((self.u, self.v, self.w), row.split()):
                for k in range(0, len(text), 3):
                    coef[r, int(text[k + 1:k + 3])] = 1 if text[k] == "+" else -1
            if self.v[r][np.flatnonzero(self.v[r])[0]] < 0:
                self.v[r], self.w[r] = -self.v[r], -self.w[r]
        assert (np.einsum("ra,rb,rc->abc", self.u, self.v, self.w).reshape(2, nb, nb, nb, 2, nb)
                == np.einsum("st,jk,il->sjkitl", np.eye(2), np.eye(nb), np.eye(nb))).all()
        self.slot = {}
        for r in range(self.n):
            k, n = divmod(int(np.flatnonzero(self.v[r])[0]), nb)
            if np.count_nonzero(self.v[r]) == 1 and n * nb + k not in self.slot.values():
                self.slot[r] = n * nb + k
        self.mixed = [r for r in range(self.n) if r not in self.slot]
        self.slot.update(zip(self.mixed, [s for s in range(self.n - 1, -1, -1) if s not in self.slot.values()]))
        self.active = {2: list(range(self.n)),
                       1: [r for r in range(self.n) if self.u[r, :nb].any() and self.w[r, :nb].any()]}


_S4 = _Scheme(4, (
    '+00+04 +00+01+08 +04', '+00 +00+02+04 +00-04', '+01+05 +04+05+07+09 +01', '+05 -01-05+06-13 +01-05',
    '+00-01 -04 +00-01', '+04-05 -01 +04-05', '+00+05 -01+04 -01+04', '+01-02+05-06 -09 +05+06',
    '+01-02 +06 +01+02-05-06', '+01-02+05 -06-09 +01-05-06', '+01-03 -07 +01-03', '+05-07 -13 +05-07',
    '+03+05 -07+13 +01-07', '+02 +03+06+08+10+11 +02', '+06 +02-09+10-12-14 +06', '+00-02+04-06 -03-08 +00-02',
    '+04-06 +02+12 +00-02-04+06', '+00+04-06 -02+08 +00-02-04', '+00-02+03 +03 +00-02+03', '+04-06+07 +12 +04-06+07',
    '-03+04-06 +03-12 +00-02+07', '+03+07 -03-11-12+13+15 +07', '+03 -03+07+12+14+15 +03-07',
    '+02+03+06+07 -03-11 +02-03', '+06+07 -12-14 +02-03-06+07', '+03+06+07 +03+11+12+14 +02-03+07',
))
_S8 = _Scheme(8, (
    '+00+08 +00-01-04+06-07+16-33-40+48 +08', '+00 +00-02+05-06-08+12+32-48-56 +00-08', '+00+01 +08-12 +00+01',
    '+08+09 +01+33 +08+09', '+00-09 +01-08+12+33 +01+08', '+00-02+08-10 -16 +00+02', '+08-10 -02 +00+02-08-10',
    '+00+08-10 +02+16 +00+02-08', '+00+03-04+08+11-12 -03 +00-03+04', '+08+11-12 -24 +00-03+04-08+11-12',
    '+03+08+11-12 +03+24 +00-03+04+11', '+00-04 +03+12-32 +00+04', '+08-12 +04-24-33 +08+12', '+00+12 +04+32 +04+08',
    '+00+05+08+13 +40 +00-05', '+08+13 +05 +00-05-08+13', '+00+08+13 -05-40 +00-05-08',
    '-00+06-07-08+14-15 +48 +00+06+07', '-08+14-15 +06 +00+06+07-08-14-15', '-00-08+14-15 -06-48 +00+06+07-08',
    '+00+07 +48+56 +00+07', '+08+15 -06+07 +08+15', '+00-15 -06+07-48-56 +07+08',
    '+01+09 -08+09-11+12-14+15-17-33-41+57 +01', '+09 +01-09-10-12-13+15-25+33-49-57 +01-09',
    '+01+02+09+10 +17 +09-10', '+01+02 -10 +01-02-09+10', '+01+02+09 +10+17 +01-09+10', '+01-03 +11 +01+03',
    '+09-11 -25 +09+11', '+03+09 +11+25 +01+11', '+00-01-04+08-09-12 +33 +08-09+12',
    '+00-01-04 -12 +00-01+04-08+09-12', '+00-01-04-09 -12-33 +01+08-09+12', '+01+05+09+13 +41 +09-13',
    '+01+05 -13 +01-05-09+13', '+01+05+09 +13+41 +01-09+13', '+01-06 +14-15 +01+06', '+09-14 -49-57 +09+14',
    '+06+09 +14-15+49+57 +01+14', '+01+06-07+09+14-15 -57 +09+14+15', '+01+06-07 +15 +01+06+07-09-14-15',
    '+01+06-07+09 +15+57 -01+09+14+15', '+02 -10-16+18+19+22+30+34+58 +02', '+10 +02+17+18+20+23+26+50+51 +10',
    '+02-03+10-11 -19-30-42 +02-03', '+10-11 -21+26+51 +02-03-10+11', '-03+10-11 +19-26 +02-03+11',
    '+02-04+10-12 -20 +10-12', '+02-04 -34 +02-04-10+12', '+02-04-12 +20-34 +04+10-12',
    '+02-03+05+10-11+13 +42 +10-11-13', '+02-03+05 -21 +02-03-05-10+11+13', '+02-03+05+10-11 +21+42 +02-03-10+11+13',
    '+02-06+10-14 -22-30 +02-06', '+10-14 +50+51 +02-06-10+14', '-06+10-14 +22+30-50-51 +02-06+14',
    '+02-07+10-15 -23 +10-15', '+02-07 -58 +02-07-10+15', '+02-07-15 +23-58 +07+10-15',
    '+03+11 -03+19-24-25+27+28-31-42-43 +11', '+03 +03+11+21+24+26+27+29+35-59 +03-11', '+03-04 -03-35 +03-04',
    '+11-12 +24-28 +11-12', '+03+12 +03+24-28+35 -04+11', '+03+05+11+13 +42+43 +03-05', '+11+13 +21+29 +03-05-11+13',
    '+03+11+13 -21-29-42-43 +03-05-11', '+02-03-06 +30 +02-03-06', '+10-11-14 +51 +10-11-14',
    '+06+10-11 +30-51 +02-03-14', '+03+07 +59 +03+07', '+11+15 +31 +11+15', '+03-15 +31-59 +07+11',
    '+04+12 +03+20-32+35+36-38-44 +04', '+12 -04+24-28-34-36-37-52 +04-12', '+04+05+12+13 -39+44 +12-13',
    '+04+05 -37+60 +04-05-12+13', '+04+05+12 +37+44 +04-12+13', '+04-06 +38 +04+06', '+12-14 -52 +12+14',
    '+06+12 +38+52 +04+14', '+04+05-07 -60 +04-05+07', '+12+13-15 +39 +12-13+15', '+04+05+15 +39+60 +07+12-13',
    '+05 -13-21-37+40+42+43+45-46+60+61 +05', '+13 -05-21-29-39+41+42+44+45+47+53 +13', '+05-06+13-14 +46 +05+06',
    '+13-14 +53 +05+06-13-14', '-06+13-14 -46-53 +05+06-14', '+05-07+13-15 +39-47 +13-15',
    '+05-07 -60-61 +05-07-13+15', '+05-07-15 -39+47-60-61 +07+13-15', '+06+14 +22+30+46-49-51-52+54-55-57 +14',
    '+06 +14-15-30+38+50+51-53+54+62 +06-14', '+06-07 -15-48-62 +06+07', '+14-15 +06+55+57 +14+15',
    '+06+15 +55+62 +07+14', '+07+15 +23-39+47-48-56-59-60-62+63 +07', '+15 -06+07+31-39-55-58-60-61-63 +07-15',
))
_ORDER_MLP = [4, 5, 6, 7, 8, 9, 10, 11, 12, 2, 3, 15, 16, 17, 18, 19, 20, 0, 1, 23, 24, 25, 13, 14, 21, 22]


def _combine(coef, xs):
    xs = list(xs)
    rows = [{k: int(c) for k, c in enumerate(row) if c} for row in coef]
    while True:
        count = collections.Counter((a, b, row[a] * row[b]) for row in rows for a in row for b in row if a < b)
        if not count or max(count.values()) < 2:
            break
        a, b, s = max(count, key=count.get)
        xs.append(xs[a] + xs[b] if s > 0 else xs[a] - xs[b])
        for row in rows:
            if a in row and b in row and row[a] * row[b] == s:
                row[len(xs) - 1] = row.pop(a)
                del row[b]
    out = []
    for row in rows:
        terms = sorted(row.items(), key=lambda t: -t[1])
        acc = xs[terms[0][0]] if terms[0][1] > 0 else -xs[terms[0][0]]
        for k, c in terms[1:]:
            acc = acc + xs[k] if c > 0 else acc - xs[k]
        out.append(acc)
    return out


def _left(sc, blocks):
    return list(enumerate(_combine(sc.u[sc.active[len(blocks) // sc.nb], :len(blocks)], blocks)))


def _block_matmul(sc, halves, lhs, rhs, outs=None, order=None):
    outs = [(1, o) for o in outs] if outs else [None] * (halves * sc.nb)
    todo = list(enumerate(sc.active[halves]))
    for pos, r in sorted(todo, key=lambda t: order.index(t[1])) if order else todo:
        m = _dot(lhs(pos), rhs(sc.slot[r]))
        for k, c in enumerate(sc.w[r, :len(outs)]):
            if c and outs[k] is None:
                outs[k] = (c, m)
            elif c:
                s, acc = outs[k]
                outs[k] = (s, acc + m) if s == c else (1, acc - m) if s > 0 else (1, m - acc)
    return [acc if s > 0 else -acc for s, acc in outs]


def _ln(x):
    m = jnp.mean(x, axis=-1, keepdims=True)
    c = x - m
    v = jnp.mean(c * c, axis=-1, keepdims=True)
    return c * jax.lax.rsqrt(v + 1e-5)


def _sigmoid(x):
    return 0.5 * jnp.tanh(0.5 * x) + 0.5


def _dot(a, b):
    return jax.lax.dot_general(a, b, (((1,), (0,)), ((), ())), preferred_element_type=F32)


def _dot_nt(a, b):
    return jax.lax.dot_general(a, b, (((1,), (1,)), ((), ())), preferred_element_type=F32)


def _lo(w):
    return pltpu.bitcast(w << 16, F32)


def _hi(w):
    return pltpu.bitcast(w & np.uint32(0xFFFF0000), F32)


def _pack(lo, hi):
    return pltpu.bitcast(pltpu.pack_elementwise([lo, hi], packed_dtype=BF16), U32)


def _bf(w):
    return pltpu.bitcast(w, BF16)


def _cols(x, nb):
    n = x.shape[1] // nb
    return [x[:, k * n:(k + 1) * n] for k in range(nb)]


def build(S, D, H, E, M, T, F, cfg):
    d = cfg["d"]
    nseg = S // T
    nch = nseg // d
    sa, sb = _S8, _S4
    NA, NB = sa.nb, sb.nb
    NI = F // D
    assert D == NA * 128 and F == NI * D + NB * 128 and E == 128 and 2 * (M + T) <= 128
    C, L, G, DA = d * T, M + T, H // NA, D // NA
    KA, n1 = DA // 128, len(sa.active[1])
    C2, T2, DB = C // 2, T // 2, D // NB
    scale = float(E) ** -0.5
    scope = jax.named_scope if cfg.get("prof") else (lambda n: contextlib.nullcontext())

    def loop(lo, hi, fn, name):
        def body(i, carry):
            with scope(name):
                fn(i)
            return carry
        jax.lax.fori_loop(lo, hi, body, 0)

    def kern(x_hbm, mem_ref, wq, wk, wv, wo_hbm, wg_hbm, wu_hbm, wd_hbm, out_hbm,
             xs, wqkv, wo, wg, wu, wd, wg4, wu4, wd4, ha, ba, bn, xa, xb, yb, qsem, osem, wsem, ysem):
        def qkv_copies(g, m):
            return [pltpu.make_async_copy((wq, wk, wv)[m].bitcast(U32).at[:, :, par, NA // 2 * g + p, :],
                                          wqkv.at[g, m, pl.ds((2 * p + par) * NA, NA)], qsem.at[g, m])
                    for p in range(NA // 2) for par in range(2)]

        def wo_copies(g):
            return [pltpu.make_async_copy(wo_hbm.bitcast(U32).at[g, :, :, pl.ds(n * DA, DA)],
                                          wo.at[pl.ds(n * NA, NA), g], osem.at[g]) for n in range(NA)]

        def in_copies(src, dst, dst4, sem):
            src = src.bitcast(U32)
            return ([pltpu.make_async_copy(src.at[:, :, :, pl.ds(n * NI * 128, NI * 128)],
                                           dst.at[pl.ds(n * NA // 2, NA // 2)], sem) for n in range(NA)]
                    + [pltpu.make_async_copy(src.at[:, :, :, pl.ds((NI * NA + n) * 128, 128)],
                                             dst4.at[pl.ds(n * NB, NB)], sem) for n in range(NB)])
        wd_src = wd_hbm.bitcast(U32)
        b_cps = [in_copies(wg_hbm, wg, wg4, wsem.at[0]), in_copies(wu_hbm, wu, wu4, wsem.at[1]),
                 [pltpu.make_async_copy(wd_src.at[pl.ds(0, NI * NA), :, pl.ds(n * 128, 128)],
                                        wd.at[pl.ds(n * NI * NA, NI * NA)], wsem.at[2]) for n in range(NA)]
                 + [pltpu.make_async_copy(wd_src.at[pl.ds(NI * NA, NB), :, pl.ds(n * DB, DB)],
                                          wd4.at[pl.ds(n * NB, NB)], wsem.at[2]) for n in range(NB)]]
        x_cps = [pltpu.make_async_copy(x_hbm.at[0:2 * C], xs.at[0:2 * C], wsem.at[3]),
                 pltpu.make_async_copy(x_hbm.at[2 * C:S], xs.at[2 * C:S], wsem.at[4])]

        def start(cps):
            for cp in cps:
                cp.start()

        def wait(cps):
            for cp in cps:
                cp.wait()

        def prep_qkv(g, m, rows):
            raw = [wqkv[g, m, s, rows, :] for s in range(NA * NA)]
            ev, od = (_combine(sa.v, [(_hi if n % 2 else _lo)(raw[(n // 2 * 2 + par) * NA + k])
                                      for k in range(NA) for n in range(NA)]) for par in range(2))
            for r in range(sa.n):
                wqkv[g, m, sa.slot[r], rows, :] = _pack(ev[r], od[r])

        def prep(sc, w, at):
            raw = [w[at(n * sc.nb + k)] for k in range(sc.nb) for n in range(sc.nb)]
            lo, hi = (_combine(sc.v[sc.mixed], [f(v) for v in raw]) for f in (_lo, _hi))
            for r, a, b in zip(sc.mixed, lo, hi):
                w[at(sc.slot[r])] = _pack(a, b)

        def rows8(i):
            return pl.ds(pl.multiple_of(i * 8, 8), 8)

        def prep_mlp(which):
            w, w4 = ((wg, wg4), (wu, wu4), (wd, wd4))[which]

            def big(t):
                for i in range(NI):
                    prep(sa, w, (lambda s: (s // 2, s % 2, rows8(t), slice(i * 128, (i + 1) * 128))) if which < 2
                         else (lambda s: (s * NI + i, rows8(t))))
                for h in range(2):
                    prep(sb, w4, (lambda s: (s, h, rows8(t))) if which < 2
                         else (lambda s: (s, rows8(t), slice(h * 128, (h + 1) * 128))))
            loop(0, 8, big, "z_prepb")

        def ordered(v, after):
            if after is None:
                return v
            return jnp.concatenate([jnp.where(after[0] == 0, v[0:8], after[1]), v[8:]], axis=0)

        def run(steps):
            for step, _ in steps:
                step()

        class Background:
            def __init__(self, zero):
                self.zero, self.queue, self.wait, self.period = zero, [], 0, 1

            def add(self, steps, period, delay):
                self.queue += steps
                self.period, self.wait = period, delay

            def __call__(self):
                self.wait -= 1
                if not self.queue or self.wait > 0:
                    return None
                self.wait = self.period
                step, ref = self.queue.pop(0)
                step()
                return self.zero, ref[self.zero, 0:8, 0:128]

        mrows = slice(0, M)

        def tok_head(t, i):
            def norm(w, r):
                if w == 0 and t is not None:
                    v = xs[pl.ds(pl.multiple_of(t * T + r, 8), 8), :].astype(F32)
                else:
                    v = xb[0, pl.ds(pl.multiple_of(i * T + r, 8), 8), :]
                ha[w, M + r:M + r + 8, :] = _ln(v)
            return [(functools.partial(norm, w, r), ha) for w in range(1 if t is None else 2) for r in range(0, T, 8)]

        def a_input(halves):
            return _left(sa, [b for w in range(halves) for b in _cols(ha[w], NA)])

        def attn_masks():
            r = jax.lax.broadcasted_iota(jnp.int32, (2 * L, 128), 0)
            k = jax.lax.broadcasted_iota(jnp.int32, (2 * L, 128), 1)
            rp = jnp.where(r < L, r, r - L)
            kp = k // 2
            same = (kp < L) & (k % 2 == jnp.where(r < L, 0, 1))
            valid = same & ((rp < M) | (rp >= kp))
            return valid, jnp.where(same, -1e9, -jnp.inf).astype(F32)

        def proj(h, g, m, halves, bg=lambda: None):
            c = _block_matmul(sa, halves, lambda s: ordered(h[s][1], bg()), lambda r: _bf(wqkv[g, m, r]))
            n = len(c) // 2
            if m == 0:
                return [jnp.concatenate([c[k], c[k + n]], axis=0) * scale for k in range(n)]
            z = jnp.zeros((64 - L, E), U32)
            return [_bf(jnp.concatenate([_pack(c[k], c[k + n]), z], axis=0)) for k in range(n)]

        def probs(qs, ks, masks):
            res = []
            for q, k in zip(qs, ks):
                s = jnp.where(masks[0], _dot_nt(q, k), masks[1])
                p = jnp.exp(s - jnp.max(s, axis=-1, keepdims=True))
                l = jnp.sum(p, axis=-1, keepdims=True)
                r = pl.reciprocal(l, approx=True)
                res.append(p * (r * (2.0 - l * r)))
            return res

        def mix(ps, vs):
            o = [_dot(p, v) for p, v in zip(ps, vs)]
            return _left(sa, [y[:L] for y in o] + [y[L:] for y in o])

        def out_proj(g0, n, c, halves, lhs, acc=None):
            return _block_matmul(sa, halves, lhs,
                                 lambda r: _bf(wo[r, pl.ds(g0, n), :, c * 128:(c + 1) * 128].reshape(n * E // 2, 128)),
                                 acc, list(range(sa.n))[::cfg["rev"]])

        def finish_cols(c, y, residual):
            for k, b in enumerate(y):
                cols = slice((k % NA) * DA + c * 128, (k % NA) * DA + (c + 1) * 128)
                ha[k // NA, mrows, cols] = b[:M]
                residual(k // NA, cols, b[M:])

        def a_step(halves, zero, mlp_input, next_tokens, residual):
            masks = attn_masks()
            so, po, kc = cfg["so"], cfg["po"], cfg["kc"]
            pr, ps, os_, acc, now = {}, {}, {}, {}, [0]
            span = len(sa.active[halves]) * KA
            side = sorted([((3 * g + 2) * span + so, 1, g) for g in range(G)]
                          + [((3 * g + 2) * span + so + po, 0, g) for g in range(G)])
            bg = Background(zero)

            def tick(tiles):
                while side and side[0][0] <= now[0]:
                    _, scores, g = side.pop(0)
                    if scores:
                        ps[g] = probs(pr[g, 0], pr[g, 1], masks)
                    else:
                        os_[g] = mix(ps[g], pr[g, 2])
                now[0] += tiles
                return bg()

            def out_lhs(g0, n, s):
                after = tick(n)
                assert all(g0 + k in os_ for k in range(n))
                return jnp.concatenate([ordered(os_[g0 + k][s][1], None if k else after) for k in range(n)], axis=1)
            h = a_input(halves)
            bg.add(mlp_input, *cfg["bg_mlp"])
            for g in range(G):
                for m in range(3):
                    pr[g, m] = proj(h, g, m, halves, lambda: tick(KA))
            bg.add(next_tokens, *cfg["bg_tok"])
            for g0, n in zip(np.cumsum([0] + kc[:-1]).tolist(), kc):
                for c in range(KA):
                    acc[c] = out_proj(g0, n, c, halves, functools.partial(out_lhs, g0, n), acc.get(c))
                    if g0 + n == G:
                        finish_cols(c, acc[c], residual)
            run(bg.queue)

        def a_dual(c, i):
            t = c * d + i
            rows = pl.ds(pl.multiple_of(i * T, T), T)
            xrows = pl.ds(pl.multiple_of(t * T, T), T)

            def residual(layer, cols, v):
                xa[layer, rows, cols] = v + (xb[0, rows, cols] if layer else xs[xrows, cols].astype(F32))
            a_step(2, i // d, b_head(0, (i + d - 1) % d) + b_head(1, (i + d - 1) % d),
                   tok_head(jnp.minimum(t + 1, nseg - 1), jnp.minimum(i + 1, d - 1)), residual)

        def single_io(w, i):
            rows = pl.ds(pl.multiple_of(i * T, T), T)

            def residual(layer, cols, v):
                xa[w, rows, cols] = v + xb[0, rows, cols]
            return tok_head(None, jnp.minimum(i + 1, d - 1)), residual

        def a_head(c):
            return tok_head(jnp.minimum(c * d, nseg - 1), 0)

        def b_head(w, i):
            def norm(h, r):
                v = xa[w, pl.ds(pl.multiple_of(i * T + h * T2 + r, 8), 8), :]
                bn[2 * w + h, pl.ds(pl.multiple_of(i * T2 + r, 8), 8), :] = _ln(v)
            return [(functools.partial(norm, h, r), bn) for h in range(2) for r in range(0, T2, 8)]

        def b_step(c, w):
            bg = Background(w // 2)
            bg.add(a_head(c + 1), *cfg["bg_head"])
            o8, o4 = list(range(sa.n))[::cfg["rb"]], _ORDER_MLP

            def gated(sc, lhs, rhs, order):
                g = [_sigmoid(v) for v in _block_matmul(sc, 2, lhs, functools.partial(rhs, 0), order=order)]
                u = _block_matmul(sc, 2, lhs, functools.partial(rhs, 1), order=order)
                return _left(sc, [gg * uu for gg, uu in zip(g, u)])
            a8 = _left(sa, [b for h in range(2) for b in _cols(bn[2 * w + h], NA)])
            hs = [gated(sa, lambda s: ordered(a8[s][1], bg()),
                        lambda m, r: _bf((wg, wu)[m][r // 2, r % 2, :, i * 128:(i + 1) * 128]), o8) for i in range(NI)]
            run(bg.queue)
            a4 = _left(sb, [b for h in range(2) for b in _cols(bn[2 * w + h], NB)])
            h4 = gated(sb, lambda s: a4[s][1], lambda m, r: _bf((wg4, wu4)[m][r].reshape(DB // 2, 128)), o4)
            y = _block_matmul(sa, 2, lambda s: jnp.concatenate([h[s][1] for h in hs], axis=1),
                              lambda r: _bf(wd[r * NI:(r + 1) * NI].reshape(NI * 64, 128)), order=o8)
            for n in range(2):
                z = _block_matmul(sb, 2, lambda s: h4[s][1], lambda r: _bf(wd4[r, :, n * 128:(n + 1) * 128]),
                                  y[n::2], o4)
                for k, v in enumerate(z):
                    cols = slice((k % NB) * DB + n * 128, (k % NB) * DB + (n + 1) * 128)
                    for i in range(d):
                        rows = slice(i * T + (k // NB) * T2, i * T + (k // NB + 1) * T2)
                        r = v[i * T2:(i + 1) * T2] + xa[w, rows, cols]
                        xb[w, rows, cols] = r
                        yb[rows, cols] = r.astype(BF16)

        def y_copy(c):
            return pltpu.make_async_copy(yb, out_hbm.at[pl.ds(pl.multiple_of(c * C, C), C), :], ysem.at[0])

        with scope("z_head"):
            x_cps[0].start()
            for m in range(3):
                start(qkv_copies(0, m))
            x_cps[0].wait()
            xb[0] = xs[0:C, :].astype(F32)
            ha[0, mrows, :] = mem_ref[...].astype(F32)
            ha[1, mrows, :] = mem_ref[...].astype(F32)
            run(tok_head(None, 0))
            xa[1] = jnp.zeros((C, D), F32)
            bn[...] = jnp.zeros(bn.shape, F32)

        def first_qkv(g):
            for m in range(3):
                @pl.when(g + 1 < G)
                def _():
                    start(qkv_copies(g + 1, m))

                @pl.when((g + 1 == G) & (m == 0))
                def _():
                    for g2 in range(G):
                        start(wo_copies(g2))
                wait(qkv_copies(g, m))
                loop(0, DA // 16, lambda i: prep_qkv(g, m, pl.ds(pl.multiple_of(i * 8, 8), 8)), "y_pq")
            h = a_input(1)
            for s, v in mix(probs(proj(h, g, 0, 1), proj(h, g, 1, 1), attn_masks()), proj(h, g, 2, 1)):
                ba[g * n1 + s] = v
        loop(0, G, first_qkv, "z_first")

        def first_out(g):
            wait(wo_copies(g))
            for k, cps in enumerate(b_cps):
                pl.when(g == k)(functools.partial(start, cps))

            def rows(i):
                for c in range(KA):
                    prep(sa, wo, lambda s: (s, g, rows8(i), slice(c * 128, (c + 1) * 128)))
            loop(0, E // 16, rows, "y_po")
            for c in range(KA):
                for k, v in enumerate(out_proj(g, 1, c, 1, lambda s: ba[g * n1 + s])):
                    xa[1, 0:L, k * DA + c * 128:k * DA + (c + 1) * 128] += v
        loop(0, G, first_out, "z_first_o")
        nxt, res = single_io(0, 0)
        run(nxt)
        for c in range(KA):
            finish_cols(c, [xa[1, 0:L, k * DA + c * 128:k * DA + (c + 1) * 128] for k in range(NA)], res)

        def chunk(c):
            edge = (c == 0) | (c == nch)
            w0 = jnp.where(c < nch, 0, 1)

            @pl.when(edge)
            def _():
                @pl.when(c == nch)
                def _():
                    ha[0, mrows, :] = ha[1, mrows, :]
                    run(tok_head(None, 0))
                loop(1 - w0, d, lambda i: a_step(1, i // d, b_head(w0, (i + d - 1) % d),
                                                 *single_io(w0, i)), "z_single")
                run(b_head(w0, d - 1))

                @pl.when(c == 0)
                def _():
                    for which, cps in enumerate(b_cps):
                        with scope("z_waitb"):
                            wait(cps)
                        prep_mlp(which)
                    x_cps[1].start()

            @pl.when(jnp.logical_not(edge))
            def _():
                loop(0, d, lambda i: a_dual(c, i), "z_dual")
                with scope("z_bhead"):
                    run(b_head(0, d - 1) + b_head(1, d - 1))

            @pl.when(c >= 2)
            def _():
                y_copy(c - 2).wait()
            loop(w0, jnp.where(c > 0, 2, 1), lambda w: b_step(c, w), "z_b")

            @pl.when(c == 0)
            def _():
                run(a_head(1))
                x_cps[1].wait()

            @pl.when(c >= 1)
            def _():
                y_copy(c - 1).start()
        loop(0, nch + 1, chunk, "z_chunk")
        y_copy(nch - 1).wait()

    any_spec = pl.BlockSpec(memory_space=pl.ANY)
    V = pltpu.VMEM
    return pl.pallas_call(
        kern,
        out_shape=jax.ShapeDtypeStruct((S, D), BF16),
        in_specs=[any_spec, pl.BlockSpec(memory_space=pltpu.VMEM)] + [any_spec] * 7,
        out_specs=any_spec,
        scratch_shapes=[
            V((S, D), BF16), V((G, 3, sa.n, DA // 2, E), U32), V((sa.n, G, E // 2, DA), U32),
            V((sa.n // 2, 2, 64, NI * 128), U32), V((sa.n // 2, 2, 64, NI * 128), U32), V((sa.n * NI, 64, 128), U32),
            V((sb.n, 2, 64, 128), U32), V((sb.n, 2, 64, 128), U32), V((sb.n, 64, DB), U32),
            V((2, L, D), F32), V((G * n1, L, 128), F32), V((4, C2, D), F32),            V((2, C, D), F32), V((2, C, D), F32), V((C, D), BF16),
            pltpu.SemaphoreType.DMA((G, 3)), pltpu.SemaphoreType.DMA((G,)),
            pltpu.SemaphoreType.DMA((5,)), pltpu.SemaphoreType.DMA((1,)),
        ],
        compiler_params=pltpu.CompilerParams(vmem_limit_bytes=126 * 2**20),
    )


@functools.partial(jax.jit, static_argnames=("A_seg_len",))
def pallas_interleave_layers__memory_aug_recurrent_mem_tr__glu_gated_glu__prompt_kernel(
        A_x, A_mem0, A_Wq, A_Wk, A_Wv, A_Wo, A_seg_len, B_x, B_w_gate, B_w_up, B_w_down):
    del B_x
    B, S, D = A_x.shape
    H, E = A_Wq.shape[1:]
    M = A_mem0.shape[1]
    F = B_w_gate.shape[1]
    call = build(S, D, H, E, M, int(A_seg_len), F, CFG)
    NA, NB = _S8.nb, _S4.nb
    qkv = [w.reshape(NA, D // (2 * NA), 2, H, E) for w in (A_Wq, A_Wk, A_Wv)]
    out = call(A_x.reshape(S, D), A_mem0.reshape(M, D), *qkv, A_Wo.reshape(H // NA, NA, E, D),
               B_w_gate.reshape(NB, 2, D // NA, F), B_w_up.reshape(NB, 2, D // NA, F),
               B_w_down.reshape(F // 128, 128, D))
    return out.reshape(B, S, D)
```

```python
import collections
import functools

import jax
import jax.experimental.pallas as pl
import jax.experimental.pallas.tpu as pltpu
import jax.numpy as jnp
import numpy as np

F32, BF16, U32 = jnp.float32, jnp.bfloat16, jnp.uint32
CFG = dict(d=4, so=100, po=130, kc=[3, 1], bg_mlp=(37, 700), bg_tok=(12, 2), bg_head=(30, 220))


class _Scheme:
    def __init__(self, nb, rows):
        self.nb, self.n = nb, len(rows)
        self.u, self.v, self.w = (np.zeros((self.n, size), np.int64) for size in (2 * nb, nb * nb, 2 * nb))
        for r, row in enumerate(rows):
            for coef, text in zip((self.u, self.v, self.w), row.split()):
                for k in range(0, len(text), 3):
                    coef[r, int(text[k + 1:k + 3])] = 1 if text[k] == "+" else -1
            if self.v[r][np.flatnonzero(self.v[r])[0]] < 0:
                self.v[r], self.w[r] = -self.v[r], -self.w[r]
        assert (np.einsum("ra,rb,rc->abc", self.u, self.v, self.w).reshape(2, nb, nb, nb, 2, nb)
                == np.einsum("st,jk,il->sjkitl", np.eye(2), np.eye(nb), np.eye(nb))).all()
        self.mixed = [r for r in range(self.n) if np.count_nonzero(self.v[r]) > 1]
        cols = [np.flatnonzero(w) % nb for w in self.w]
        self.by_column = sorted(range(self.n), key=lambda r: (-cols[r].max() // 2, -cols[r].min() // 2,
                                                              -cols[r].max(), -cols[r].min()))
        self.active = {2: list(range(self.n)),
                       1: [r for r in range(self.n) if self.u[r, :nb].any() and self.w[r, :nb].any()]}


_S4 = _Scheme(4, (
    '+00+04 +00+01+08 +04', '+00 +00+02+04 +00-04', '+01+05 +04+05+07+09 +01', '+05 -01-05+06-13 +01-05',
    '+00-01 -04 +00-01', '+04-05 -01 +04-05', '+00+05 -01+04 -01+04', '+01-02+05-06 -09 +05+06',
    '+01-02 +06 +01+02-05-06', '+01-02+05 -06-09 +01-05-06', '+01-03 -07 +01-03', '+05-07 -13 +05-07',
    '+03+05 -07+13 +01-07', '+02 +03+06+08+10+11 +02', '+06 +02-09+10-12-14 +06', '+00-02+04-06 -03-08 +00-02',
    '+04-06 +02+12 +00-02-04+06', '+00+04-06 -02+08 +00-02-04', '+00-02+03 +03 +00-02+03', '+04-06+07 +12 +04-06+07',
    '-03+04-06 +03-12 +00-02+07', '+03+07 -03-11-12+13+15 +07', '+03 -03+07+12+14+15 +03-07',
    '+02+03+06+07 -03-11 +02-03', '+06+07 -12-14 +02-03-06+07', '+03+06+07 +03+11+12+14 +02-03+07',
))
_S8 = _Scheme(8, (
    '+00+08 +00-01-04+06-07+16-33-40+48 +08', '+00 +00-02+05-06-08+12+32-48-56 +00-08', '+00+01 +08-12 +00+01',
    '+08+09 +01+33 +08+09', '+00-09 +01-08+12+33 +01+08', '+00-02+08-10 -16 +00+02', '+08-10 -02 +00+02-08-10',
    '+00+08-10 +02+16 +00+02-08', '+00+03-04+08+11-12 -03 +00-03+04', '+08+11-12 -24 +00-03+04-08+11-12',
    '+03+08+11-12 +03+24 +00-03+04+11', '+00-04 +03+12-32 +00+04', '+08-12 +04-24-33 +08+12', '+00+12 +04+32 +04+08',
    '+00+05+08+13 +40 +00-05', '+08+13 +05 +00-05-08+13', '+00+08+13 -05-40 +00-05-08',
    '-00+06-07-08+14-15 +48 +00+06+07', '-08+14-15 +06 +00+06+07-08-14-15', '-00-08+14-15 -06-48 +00+06+07-08',
    '+00+07 +48+56 +00+07', '+08+15 -06+07 +08+15', '+00-15 -06+07-48-56 +07+08',
    '+01+09 -08+09-11+12-14+15-17-33-41+57 +01', '+09 +01-09-10-12-13+15-25+33-49-57 +01-09',
    '+01+02+09+10 +17 +09-10', '+01+02 -10 +01-02-09+10', '+01+02+09 +10+17 +01-09+10', '+01-03 +11 +01+03',
    '+09-11 -25 +09+11', '+03+09 +11+25 +01+11', '+00-01-04+08-09-12 +33 +08-09+12',
    '+00-01-04 -12 +00-01+04-08+09-12', '+00-01-04-09 -12-33 +01+08-09+12', '+01+05+09+13 +41 +09-13',
    '+01+05 -13 +01-05-09+13', '+01+05+09 +13+41 +01-09+13', '+01-06 +14-15 +01+06', '+09-14 -49-57 +09+14',
    '+06+09 +14-15+49+57 +01+14', '+01+06-07+09+14-15 -57 +09+14+15', '+01+06-07 +15 +01+06+07-09-14-15',
    '+01+06-07+09 +15+57 -01+09+14+15', '+02 -10-16+18+19+22+30+34+58 +02', '+10 +02+17+18+20+23+26+50+51 +10',
    '+02-03+10-11 -19-30-42 +02-03', '+10-11 -21+26+51 +02-03-10+11', '-03+10-11 +19-26 +02-03+11',
    '+02-04+10-12 -20 +10-12', '+02-04 -34 +02-04-10+12', '+02-04-12 +20-34 +04+10-12',
    '+02-03+05+10-11+13 +42 +10-11-13', '+02-03+05 -21 +02-03-05-10+11+13', '+02-03+05+10-11 +21+42 +02-03-10+11+13',
    '+02-06+10-14 -22-30 +02-06', '+10-14 +50+51 +02-06-10+14', '-06+10-14 +22+30-50-51 +02-06+14',
    '+02-07+10-15 -23 +10-15', '+02-07 -58 +02-07-10+15', '+02-07-15 +23-58 +07+10-15',
    '+03+11 -03+19-24-25+27+28-31-42-43 +11', '+03 +03+11+21+24+26+27+29+35-59 +03-11', '+03-04 -03-35 +03-04',
    '+11-12 +24-28 +11-12', '+03+12 +03+24-28+35 -04+11', '+03+05+11+13 +42+43 +03-05', '+11+13 +21+29 +03-05-11+13',
    '+03+11+13 -21-29-42-43 +03-05-11', '+02-03-06 +30 +02-03-06', '+10-11-14 +51 +10-11-14',
    '+06+10-11 +30-51 +02-03-14', '+03+07 +59 +03+07', '+11+15 +31 +11+15', '+03-15 +31-59 +07+11',
    '+04+12 +03+20-32+35+36-38-44 +04', '+12 -04+24-28-34-36-37-52 +04-12', '+04+05+12+13 -39+44 +12-13',
    '+04+05 -37+60 +04-05-12+13', '+04+05+12 +37+44 +04-12+13', '+04-06 +38 +04+06', '+12-14 -52 +12+14',
    '+06+12 +38+52 +04+14', '+04+05-07 -60 +04-05+07', '+12+13-15 +39 +12-13+15', '+04+05+15 +39+60 +07+12-13',
    '+05 -13-21-37+40+42+43+45-46+60+61 +05', '+13 -05-21-29-39+41+42+44+45+47+53 +13', '+05-06+13-14 +46 +05+06',
    '+13-14 +53 +05+06-13-14', '-06+13-14 -46-53 +05+06-14', '+05-07+13-15 +39-47 +13-15',
    '+05-07 -60-61 +05-07-13+15', '+05-07-15 -39+47-60-61 +07+13-15', '+06+14 +22+30+46-49-51-52+54-55-57 +14',
    '+06 +14-15-30+38+50+51-53+54+62 +06-14', '+06-07 -15-48-62 +06+07', '+14-15 +06+55+57 +14+15',
    '+06+15 +55+62 +07+14', '+07+15 +23-39+47-48-56-59-60-62+63 +07', '+15 -06+07+31-39-55-58-60-61-63 +07-15',
))
_ORDER_MLP = [4, 5, 6, 7, 8, 9, 10, 11, 12, 2, 3, 15, 16, 17, 18, 19, 20, 0, 1, 23, 24, 25, 13, 14, 21, 22]


def _combine(coef, xs):
    xs = list(xs)
    rows = [{k: int(c) for k, c in enumerate(row) if c} for row in coef]
    while True:
        count = collections.Counter((a, b, row[a] * row[b]) for row in rows for a in row for b in row if a < b)
        if not count or max(count.values()) < 2:
            break
        a, b, s = max(count, key=count.get)
        xs.append(xs[a] + xs[b] if s > 0 else xs[a] - xs[b])
        for row in rows:
            if a in row and b in row and row[a] * row[b] == s:
                row[len(xs) - 1] = row.pop(a)
                del row[b]
    out = []
    for row in rows:
        terms = sorted(row.items(), key=lambda t: -t[1])
        acc = xs[terms[0][0]] if terms[0][1] > 0 else -xs[terms[0][0]]
        for k, c in terms[1:]:
            acc = acc + xs[k] if c > 0 else acc - xs[k]
        out.append(acc)
    return out


def _left(sc, blocks):
    return list(enumerate(_combine(sc.u[sc.active[len(blocks) // sc.nb], :len(blocks)], blocks)))


def _block_matmul(sc, halves, lhs, rhs, outs=None, order=None):
    outs = [(1, o) for o in outs] if outs else [None] * (halves * sc.nb)
    todo = list(enumerate(sc.active[halves]))
    for pos, r in sorted(todo, key=lambda t: order.index(t[1])) if order else todo:
        m = _dot(lhs(pos), rhs(r))
        for k, c in enumerate(sc.w[r, :len(outs)]):
            if c and outs[k] is None:
                outs[k] = (c, m)
            elif c:
                s, acc = outs[k]
                outs[k] = (s, acc + m) if s == c else (1, acc - m) if s > 0 else (1, m - acc)
    return [acc if s > 0 else -acc for s, acc in outs]


def _ln(x):
    m = jnp.mean(x, axis=-1, keepdims=True)
    c = x - m
    v = jnp.mean(c * c, axis=-1, keepdims=True)
    return c * jax.lax.rsqrt(v + 1e-5)


def _sigmoid(x):
    return 0.5 * jnp.tanh(0.5 * x) + 0.5


def _dot(a, b):
    return jax.lax.dot_general(a, b, (((1,), (0,)), ((), ())), preferred_element_type=F32)


def _dot_nt(a, b):
    return jax.lax.dot_general(a, b, (((1,), (1,)), ((), ())), preferred_element_type=F32)


def _lo(w):
    return pltpu.bitcast(w << 16, F32)


def _hi(w):
    return pltpu.bitcast(w & np.uint32(0xFFFF0000), F32)


def _pack(lo, hi):
    lo, hi = (pltpu.bitcast(v, U32) + np.uint32(0x8000) for v in (lo, hi))
    return (lo >> 16) | (hi & np.uint32(0xFFFF0000))


def _bf(w):
    return pltpu.bitcast(w, BF16)


def _cols(x, nb):
    n = x.shape[1] // nb
    return [x[:, k * n:(k + 1) * n] for k in range(nb)]


def build(S, D, H, E, M, T, F, cfg):
    d = cfg["d"]
    nseg = S // T
    nch = nseg // d
    sa, sb = _S8, _S4
    NA, NB = sa.nb, sb.nb
    NI = F // D
    assert D == NA * 128 and F == NI * D + NB * 128 and E == 128 and 2 * (M + T) <= 128
    C, L, G, DA = d * T, M + T, H // NA, D // NA
    n1, na, nb = len(sa.active[1]), len(sa.mixed), len(sb.mixed)
    C2, T2, DB = C // 2, T // 2, D // NB
    scale = float(E) ** -0.5

    def loop(lo, hi, fn):
        def body(i, carry):
            fn(i)
            return carry
        jax.lax.fori_loop(lo, hi, body, 0)

    def kern(x_hbm, mem_ref, wq, wk, wv, wo_hbm, wg_hbm, wu_hbm, wd_hbm, out_hbm,
             xs, wqkv, wo, wg, wu, wd, mo, mg, mu, md, mg4, mu4, md4, ha, ba, bn, xa, xb, yb, qsem, osem, wsem, xsem, ysem):
        def qkv_copies(g, m):
            return [pltpu.make_async_copy((wq, wk, wv)[m].bitcast(U32).at[:, :, par, NA // 2 * g + p, :],
                                          wqkv.at[g, m, pl.ds((2 * p + par) * NA, NA)], qsem.at[g, m])
                    for p in range(NA // 2) for par in range(2)]

        def wo_copy(g):
            return pltpu.make_async_copy(wo_hbm.bitcast(U32).at[g], wo.at[g], osem.at[g])

        def mlp_copies(which, t):
            rows = pl.ds(pl.multiple_of(t * 16, 16), 16)
            return [pltpu.make_async_copy((wg_hbm, wu_hbm, wd_hbm)[which].bitcast(U32).at[:, rows, :],
                                          (wg, wu, wd)[which].at[:, rows, :], wsem.at[which, t])]
        x_cps = [pltpu.make_async_copy(x_hbm.at[0:2 * C], xs.at[0:2 * C], xsem.at[0]),
                 pltpu.make_async_copy(x_hbm.at[2 * C:S], xs.at[2 * C:S], xsem.at[1])]

        def start(cps):
            for cp in cps:
                cp.start()

        def wait(cps):
            for cp in cps:
                cp.wait()

        def prep_qkv(g, m, rows):
            raw = [wqkv[g, m, s, rows, :] for s in range(NA * NA)]
            ev, od = (_combine(sa.v, [(_hi if n % 2 else _lo)(raw[(n // 2 * 2 + par) * NA + k])
                                      for k in range(NA) for n in range(NA)]) for par in range(2))
            for r in range(sa.n):
                wqkv[g, m, r, rows, :] = _pack(ev[r], od[r])

        def tile(k):
            return slice(k * 128, (k + 1) * 128)

        def w_out(g):
            return sa, lambda k, n, rows: wo[g, k, rows, tile(n)], lambda j, rows: (mo, (j, g, rows))

        def w_in(m, i):
            return (sa, lambda k, n, rows: (wg, wu)[m][k, rows, tile(i * NA + n)],
                    lambda j, rows: ((mg, mu)[m], (i, j, rows)))

        def w_in4(m, h):
            return (sb, lambda k, n, rows: (wg, wu)[m][2 * k + h, rows, tile(NI * NA + n)],
                    lambda j, rows: ((mg4, mu4)[m], (h, j, rows)))

        def w_down(i):
            return sa, lambda k, n, rows: wd[i * NA + k, rows, tile(n)], lambda j, rows: (md, (i, j, rows))

        def w_down4(c):
            return sb, lambda k, n, rows: wd[NI * NA + k, rows, tile(2 * n + c)], lambda j, rows: (md4, (c, j, rows))

        def prep(w, t):
            sc, raw, mixed = w
            rows = pl.ds(pl.multiple_of(t * 8, 8), 8)
            blocks = [raw(k, n, rows) for k in range(sc.nb) for n in range(sc.nb)]
            lo, hi = (_combine(sc.v[sc.mixed], [f(v) for v in blocks]) for f in (_lo, _hi))
            for j in range(len(sc.mixed)):
                ref, idx = mixed(j, rows)
                ref[idx] = _pack(lo[j], hi[j])

        def weight(ws, r):
            def one(sc, raw, mixed):
                if r not in sc.mixed:
                    return raw(*divmod(int(np.flatnonzero(sc.v[r])[0]), sc.nb), slice(None))
                ref, idx = mixed(sc.mixed.index(r), slice(None))
                return ref[idx]
            return _bf(jnp.concatenate([one(*w) for w in ws], axis=0))

        def prep_mlp(which):
            ws = ([w_in(which, i) for i in range(NI)] + [w_in4(which, h) for h in range(2)] if which < 2
                  else [w_down(i) for i in range(NI)] + [w_down4(c) for c in range(2)])

            def rows(t):
                pl.when(t % 2 == 0)(lambda: wait(mlp_copies(which, t // 2)))
                for w in ws:
                    prep(w, t)
            loop(0, 8, rows)

        def ordered(v, after):
            if after is None:
                return v
            return jnp.concatenate([jnp.where(after[0] == 0, v[0:8], after[1]), v[8:]], axis=0)

        def run(steps):
            for step, _ in steps:
                step()

        class Background:
            def __init__(self, zero):
                self.zero, self.queue, self.wait, self.period = zero, [], 0, 1

            def add(self, steps, period, delay):
                self.queue += steps
                self.period, self.wait = period, delay

            def __call__(self):
                self.wait -= 1
                if not self.queue or self.wait > 0:
                    return None
                self.wait = self.period
                step, ref = self.queue.pop(0)
                step()
                return self.zero, ref[self.zero, 0:8, 0:128]

        mrows = slice(0, M)

        def tok_head(t, i):
            def norm(w, r):
                if w == 0 and t is not None:
                    v = xs[pl.ds(pl.multiple_of(t * T + r, 8), 8), :].astype(F32)
                else:
                    v = xb[0, pl.ds(pl.multiple_of(i * T + r, 8), 8), :]
                ha[w, M + r:M + r + 8, :] = _ln(v)
            return [(functools.partial(norm, w, r), ha) for w in range(1 if t is None else 2) for r in range(0, T, 8)]

        def a_input(halves):
            return _left(sa, [b for w in range(halves) for b in _cols(ha[w], NA)])

        def attn_masks():
            r = jax.lax.broadcasted_iota(jnp.int32, (2 * L, 128), 0)
            k = jax.lax.broadcasted_iota(jnp.int32, (2 * L, 128), 1)
            rp = jnp.where(r < L, r, r - L)
            kp = k // 2
            same = (kp < L) & (k % 2 == jnp.where(r < L, 0, 1))
            valid = same & ((rp < M) | (rp >= kp))
            return valid, jnp.where(same, -1e9, -jnp.inf).astype(F32)

        def proj(h, g, m, halves, bg=lambda: None):
            c = _block_matmul(sa, halves, lambda s: ordered(h[s][1], bg()), lambda r: _bf(wqkv[g, m, r]))
            n = len(c) // 2
            if m == 0:
                return [jnp.concatenate([c[k], c[k + n]], axis=0) * scale for k in range(n)]
            z = jnp.zeros((64 - L, E), U32)
            return [_bf(jnp.concatenate([_pack(c[k], c[k + n]), z], axis=0)) for k in range(n)]

        def probs(qs, ks, masks):
            res = []
            for q, k in zip(qs, ks):
                s = jnp.where(masks[0], _dot_nt(q, k), masks[1])
                p = jnp.exp(s - jnp.max(s, axis=-1, keepdims=True))
                l = jnp.sum(p, axis=-1, keepdims=True)
                r = pl.reciprocal(l, approx=True)
                res.append(p * (r * (2.0 - l * r)))
            return res

        def mix(ps, vs):
            o = [_dot(p, v) for p, v in zip(ps, vs)]
            return _left(sa, [y[:L] for y in o] + [y[L:] for y in o])

        def out_proj(g0, n, halves, lhs, acc=None):
            return _block_matmul(sa, halves, lhs, functools.partial(weight, [w_out(g0 + k) for k in range(n)]),
                                 acc, sa.by_column)

        def finish(y, residual):
            for k, b in enumerate(y):
                ha[k // NA, mrows, tile(k % NA)] = b[:M]
                residual(k // NA, tile(k % NA), b[M:])

        def a_step(halves, zero, mlp_input, next_tokens, residual):
            masks = attn_masks()
            so, po, kc = cfg["so"], cfg["po"], cfg["kc"]
            pr, ps, os_, acc, now = {}, {}, {}, None, [0]
            span = len(sa.active[halves])
            side = sorted([((3 * g + 2) * span + so, 1, g) for g in range(G)]
                          + [((3 * g + 2) * span + so + po, 0, g) for g in range(G)])
            bg = Background(zero)

            def tick(tiles):
                while side and side[0][0] <= now[0]:
                    _, scores, g = side.pop(0)
                    if scores:
                        ps[g] = probs(pr[g, 0], pr[g, 1], masks)
                    else:
                        os_[g] = mix(ps[g], pr[g, 2])
                now[0] += tiles
                return bg()

            def out_lhs(g0, n, s):
                after = tick(n)
                assert all(g0 + k in os_ for k in range(n))
                return jnp.concatenate([ordered(os_[g0 + k][s][1], None if k else after) for k in range(n)], axis=1)
            h = a_input(halves)
            bg.add(mlp_input, *cfg["bg_mlp"])
            for g in range(G):
                for m in range(3):
                    pr[g, m] = proj(h, g, m, halves, lambda: tick(1))
            bg.add(next_tokens, *cfg["bg_tok"])
            for g0, n in zip(np.cumsum([0] + kc[:-1]).tolist(), kc):
                acc = out_proj(g0, n, halves, functools.partial(out_lhs, g0, n), acc)
            finish(acc, residual)
            run(bg.queue)

        def a_dual(c, i):
            t = c * d + i
            rows = pl.ds(pl.multiple_of(i * T, T), T)
            xrows = pl.ds(pl.multiple_of(t * T, T), T)

            def residual(layer, cols, v):
                xa[layer, rows, cols] = v + (xb[0, rows, cols] if layer else xs[xrows, cols].astype(F32))
            a_step(2, i // d, b_head(0, (i + d - 1) % d) + b_head(1, (i + d - 1) % d),
                   tok_head(jnp.minimum(t + 1, nseg - 1), jnp.minimum(i + 1, d - 1)), residual)

        def single_io(w, i):
            rows = pl.ds(pl.multiple_of(i * T, T), T)

            def residual(layer, cols, v):
                xa[w, rows, cols] = v + xb[0, rows, cols]
            return tok_head(None, jnp.minimum(i + 1, d - 1)), residual

        def a_head(c):
            return tok_head(jnp.minimum(c * d, nseg - 1), 0)

        def b_head(w, i):
            def norm(h, r):
                v = xa[w, pl.ds(pl.multiple_of(i * T + h * T2 + r, 8), 8), :]
                bn[2 * w + h, pl.ds(pl.multiple_of(i * T2 + r, 8), 8), :] = _ln(v)
            return [(functools.partial(norm, h, r), bn) for h in range(2) for r in range(0, T2, 8)]

        def b_step(c, w):
            bg = Background(w // 2)
            bg.add(a_head(c + 1), *cfg["bg_head"])
            o8, o4 = sa.by_column, _ORDER_MLP

            def gated(sc, lhs, ws, order):
                g = [_sigmoid(v) for v in _block_matmul(sc, 2, lhs, functools.partial(weight, ws(0)), order=order)]
                u = _block_matmul(sc, 2, lhs, functools.partial(weight, ws(1)), order=order)
                return _left(sc, [gg * uu for gg, uu in zip(g, u)])
            a8 = _left(sa, [b for h in range(2) for b in _cols(bn[2 * w + h], NA)])
            hs = [gated(sa, lambda s: ordered(a8[s][1], bg()),
                        lambda m: [w_in(m, i)], o8) for i in range(NI)]
            run(bg.queue)
            a4 = _left(sb, [b for h in range(2) for b in _cols(bn[2 * w + h], NB)])
            h4 = gated(sb, lambda s: a4[s][1], lambda m: [w_in4(m, h) for h in range(2)], o4)
            y = _block_matmul(sa, 2, lambda s: jnp.concatenate([h[s][1] for h in hs], axis=1),
                              functools.partial(weight, [w_down(i) for i in range(NI)]), order=o8)
            for n in range(2):
                z = _block_matmul(sb, 2, lambda s: h4[s][1], functools.partial(weight, [w_down4(n)]),
                                  y[n::2], o4)
                for k, v in enumerate(z):
                    cols = slice((k % NB) * DB + n * 128, (k % NB) * DB + (n + 1) * 128)
                    for i in range(d):
                        rows = slice(i * T + (k // NB) * T2, i * T + (k // NB + 1) * T2)
                        r = v[i * T2:(i + 1) * T2] + xa[w, rows, cols]
                        xb[w, rows, cols] = r
                        yb[rows, cols] = r.astype(BF16)

        def y_copy(c):
            return pltpu.make_async_copy(yb, out_hbm.at[pl.ds(pl.multiple_of(c * C, C), C), :], ysem.at[0])

        x_cps[0].start()
        for m in range(3):
            start(qkv_copies(0, m))
        x_cps[0].wait()
        xb[0] = xs[0:C, :].astype(F32)
        ha[0, mrows, :] = mem_ref[...].astype(F32)
        ha[1, mrows, :] = mem_ref[...].astype(F32)
        run(tok_head(None, 0))
        xa[1] = jnp.zeros((C, D), F32)
        bn[...] = jnp.zeros(bn.shape, F32)

        def first_qkv(g):
            for m in range(3):
                @pl.when(g + 1 < G)
                def _():
                    start(qkv_copies(g + 1, m))

                @pl.when((g + 1 == G) & (m == 0))
                def _():
                    start([wo_copy(k) for k in range(G)])
                wait(qkv_copies(g, m))
                loop(0, DA // 16, lambda i: prep_qkv(g, m, pl.ds(pl.multiple_of(i * 8, 8), 8)))
            h = a_input(1)
            for s, v in mix(probs(proj(h, g, 0, 1), proj(h, g, 1, 1), attn_masks()), proj(h, g, 2, 1)):
                ba[g * n1 + s] = v
        loop(0, G, first_qkv)

        start([cp for which in range(3) for t in range(4) for cp in mlp_copies(which, t)])

        def first_out(g):
            wo_copy(g).wait()
            loop(0, 8, functools.partial(prep, w_out(g)))
            for k, v in enumerate(out_proj(g, 1, 1, lambda s: ba[g * n1 + s])):
                xa[1, 0:L, tile(k)] += v
        loop(0, G, first_out)
        nxt, res = single_io(0, 0)
        run(nxt)
        finish(_cols(xa[1, 0:L, :], NA), res)

        def chunk(c):
            edge = (c == 0) | (c == nch)
            w0 = jnp.where(c < nch, 0, 1)

            @pl.when(edge)
            def _():
                @pl.when(c == nch)
                def _():
                    ha[0, mrows, :] = ha[1, mrows, :]
                    run(tok_head(None, 0))
                loop(1 - w0, d, lambda i: a_step(1, i // d, b_head(w0, (i + d - 1) % d),
                                                 *single_io(w0, i)))
                run(b_head(w0, d - 1))

                @pl.when(c == 0)
                def _():
                    for which in range(3):
                        prep_mlp(which)
                    x_cps[1].start()

            @pl.when(jnp.logical_not(edge))
            def _():
                loop(0, d, lambda i: a_dual(c, i))
                run(b_head(0, d - 1) + b_head(1, d - 1))

            @pl.when(c >= 2)
            def _():
                y_copy(c - 2).wait()
            loop(w0, jnp.where(c > 0, 2, 1), lambda w: b_step(c, w))

            @pl.when(c == 0)
            def _():
                run(a_head(1))
                x_cps[1].wait()

            @pl.when(c >= 1)
            def _():
                y_copy(c - 1).start()
        loop(0, nch + 1, chunk)
        y_copy(nch - 1).wait()

    any_spec = pl.BlockSpec(memory_space=pl.ANY)
    V = pltpu.VMEM
    return pl.pallas_call(
        kern,
        out_shape=jax.ShapeDtypeStruct((S, D), BF16),
        in_specs=[any_spec, pl.BlockSpec(memory_space=pltpu.VMEM)] + [any_spec] * 7,
        out_specs=any_spec,
        scratch_shapes=[
            V((S, D), BF16), V((G, 3, sa.n, DA // 2, E), U32),
            V((G, NA, 64, D), U32), V((NA, 64, F), U32), V((NA, 64, F), U32), V((F // 128, 64, D), U32),
            V((na, G, 64, 128), U32)] + [V((NI, na, 64, 128), U32)] * 3 + [V((2, nb, 64, 128), U32)] * 3 + [
            V((2, L, D), F32), V((G * n1, L, 128), F32), V((4, C2, D), F32),            V((2, C, D), F32), V((2, C, D), F32), V((C, D), BF16),
            pltpu.SemaphoreType.DMA((G, 3)), pltpu.SemaphoreType.DMA((G,)),
            pltpu.SemaphoreType.DMA((3, 4)), pltpu.SemaphoreType.DMA((2,)), pltpu.SemaphoreType.DMA((1,)),
        ],
        compiler_params=pltpu.CompilerParams(vmem_limit_bytes=126 * 2**20),
    )


@functools.partial(jax.jit, static_argnames=("A_seg_len",))
def pallas_interleave_layers__memory_aug_recurrent_mem_tr__glu_gated_glu__prompt_kernel(
        A_x, A_mem0, A_Wq, A_Wk, A_Wv, A_Wo, A_seg_len, B_x, B_w_gate, B_w_up, B_w_down):
    del B_x
    B, S, D = A_x.shape
    H, E = A_Wq.shape[1:]
    M = A_mem0.shape[1]
    F = B_w_gate.shape[1]
    call = build(S, D, H, E, M, int(A_seg_len), F, CFG)
    NA = _S8.nb
    qkv = [w.reshape(NA, D // (2 * NA), 2, H, E) for w in (A_Wq, A_Wk, A_Wv)]
    out = call(A_x.reshape(S, D), A_mem0.reshape(M, D), *qkv, A_Wo.reshape(H // NA, NA, E, D),
               B_w_gate.reshape(NA, D // NA, F), B_w_up.reshape(NA, D // NA, F),
               B_w_down.reshape(F // 128, 128, D))
    return out.reshape(B, S, D)
```

```python
import collections
import functools

import jax
import jax.experimental.pallas as pl
import jax.experimental.pallas.tpu as pltpu
import jax.numpy as jnp
import numpy as np

F32, BF16, U32 = jnp.float32, jnp.bfloat16, jnp.uint32
CFG = dict(d=4, so=100, po=130, kc=[3, 1], bg_mlp=(37, 700), bg_tok=(12, 2), bg_head=(30, 220))


class _Scheme:
    def __init__(self, nb, rows):
        self.nb, self.n = nb, len(rows)
        self.u, self.v, self.w = (np.zeros((self.n, size), np.int64) for size in (2 * nb, nb * nb, 2 * nb))
        for r, row in enumerate(rows):
            for coef, text in zip((self.u, self.v, self.w), row.split()):
                for k in range(0, len(text), 3):
                    coef[r, int(text[k + 1:k + 3])] = 1 if text[k] == "+" else -1
            if self.v[r][np.flatnonzero(self.v[r])[0]] < 0:
                self.v[r], self.w[r] = -self.v[r], -self.w[r]
        assert (np.einsum("ra,rb,rc->abc", self.u, self.v, self.w).reshape(2, nb, nb, nb, 2, nb)
                == np.einsum("st,jk,il->sjkitl", np.eye(2), np.eye(nb), np.eye(nb))).all()
        self.mixed = [r for r in range(self.n) if np.count_nonzero(self.v[r]) > 1]
        cols = [np.flatnonzero(w) % nb for w in self.w]
        self.by_column = sorted(range(self.n), key=lambda r: (-cols[r].max() // 2, -cols[r].min() // 2,
                                                              -cols[r].max(), -cols[r].min()))
        self.active = {2: list(range(self.n)),
                       1: [r for r in range(self.n) if self.u[r, :nb].any() and self.w[r, :nb].any()]}


_S4 = _Scheme(4, (
    '+00+04 +00+01+08 +04', '+00 +00+02+04 +00-04', '+01+05 +04+05+07+09 +01', '+05 -01-05+06-13 +01-05',
    '+00-01 -04 +00-01', '+04-05 -01 +04-05', '+00+05 -01+04 -01+04', '+01-02+05-06 -09 +05+06',
    '+01-02 +06 +01+02-05-06', '+01-02+05 -06-09 +01-05-06', '+01-03 -07 +01-03', '+05-07 -13 +05-07',
    '+03+05 -07+13 +01-07', '+02 +03+06+08+10+11 +02', '+06 +02-09+10-12-14 +06', '+00-02+04-06 -03-08 +00-02',
    '+04-06 +02+12 +00-02-04+06', '+00+04-06 -02+08 +00-02-04', '+00-02+03 +03 +00-02+03', '+04-06+07 +12 +04-06+07',
    '-03+04-06 +03-12 +00-02+07', '+03+07 -03-11-12+13+15 +07', '+03 -03+07+12+14+15 +03-07',
    '+02+03+06+07 -03-11 +02-03', '+06+07 -12-14 +02-03-06+07', '+03+06+07 +03+11+12+14 +02-03+07',
))
_S8 = _Scheme(8, (
    '+00+08 +00-01-04+06-07+16-33-40+48 +08', '+00 +00-02+05-06-08+12+32-48-56 +00-08', '+00+01 +08-12 +00+01',
    '+08+09 +01+33 +08+09', '+00-09 +01-08+12+33 +01+08', '+00-02+08-10 -16 +00+02', '+08-10 -02 +00+02-08-10',
    '+00+08-10 +02+16 +00+02-08', '+00+03-04+08+11-12 -03 +00-03+04', '+08+11-12 -24 +00-03+04-08+11-12',
    '+03+08+11-12 +03+24 +00-03+04+11', '+00-04 +03+12-32 +00+04', '+08-12 +04-24-33 +08+12', '+00+12 +04+32 +04+08',
    '+00+05+08+13 +40 +00-05', '+08+13 +05 +00-05-08+13', '+00+08+13 -05-40 +00-05-08',
    '-00+06-07-08+14-15 +48 +00+06+07', '-08+14-15 +06 +00+06+07-08-14-15', '-00-08+14-15 -06-48 +00+06+07-08',
    '+00+07 +48+56 +00+07', '+08+15 -06+07 +08+15', '+00-15 -06+07-48-56 +07+08',
    '+01+09 -08+09-11+12-14+15-17-33-41+57 +01', '+09 +01-09-10-12-13+15-25+33-49-57 +01-09',
    '+01+02+09+10 +17 +09-10', '+01+02 -10 +01-02-09+10', '+01+02+09 +10+17 +01-09+10', '+01-03 +11 +01+03',
    '+09-11 -25 +09+11', '+03+09 +11+25 +01+11', '+00-01-04+08-09-12 +33 +08-09+12',
    '+00-01-04 -12 +00-01+04-08+09-12', '+00-01-04-09 -12-33 +01+08-09+12', '+01+05+09+13 +41 +09-13',
    '+01+05 -13 +01-05-09+13', '+01+05+09 +13+41 +01-09+13', '+01-06 +14-15 +01+06', '+09-14 -49-57 +09+14',
    '+06+09 +14-15+49+57 +01+14', '+01+06-07+09+14-15 -57 +09+14+15', '+01+06-07 +15 +01+06+07-09-14-15',
    '+01+06-07+09 +15+57 -01+09+14+15', '+02 -10-16+18+19+22+30+34+58 +02', '+10 +02+17+18+20+23+26+50+51 +10',
    '+02-03+10-11 -19-30-42 +02-03', '+10-11 -21+26+51 +02-03-10+11', '-03+10-11 +19-26 +02-03+11',
    '+02-04+10-12 -20 +10-12', '+02-04 -34 +02-04-10+12', '+02-04-12 +20-34 +04+10-12',
    '+02-03+05+10-11+13 +42 +10-11-13', '+02-03+05 -21 +02-03-05-10+11+13', '+02-03+05+10-11 +21+42 +02-03-10+11+13',
    '+02-06+10-14 -22-30 +02-06', '+10-14 +50+51 +02-06-10+14', '-06+10-14 +22+30-50-51 +02-06+14',
    '+02-07+10-15 -23 +10-15', '+02-07 -58 +02-07-10+15', '+02-07-15 +23-58 +07+10-15',
    '+03+11 -03+19-24-25+27+28-31-42-43 +11', '+03 +03+11+21+24+26+27+29+35-59 +03-11', '+03-04 -03-35 +03-04',
    '+11-12 +24-28 +11-12', '+03+12 +03+24-28+35 -04+11', '+03+05+11+13 +42+43 +03-05', '+11+13 +21+29 +03-05-11+13',
    '+03+11+13 -21-29-42-43 +03-05-11', '+02-03-06 +30 +02-03-06', '+10-11-14 +51 +10-11-14',
    '+06+10-11 +30-51 +02-03-14', '+03+07 +59 +03+07', '+11+15 +31 +11+15', '+03-15 +31-59 +07+11',
    '+04+12 +03+20-32+35+36-38-44 +04', '+12 -04+24-28-34-36-37-52 +04-12', '+04+05+12+13 -39+44 +12-13',
    '+04+05 -37+60 +04-05-12+13', '+04+05+12 +37+44 +04-12+13', '+04-06 +38 +04+06', '+12-14 -52 +12+14',
    '+06+12 +38+52 +04+14', '+04+05-07 -60 +04-05+07', '+12+13-15 +39 +12-13+15', '+04+05+15 +39+60 +07+12-13',
    '+05 -13-21-37+40+42+43+45-46+60+61 +05', '+13 -05-21-29-39+41+42+44+45+47+53 +13', '+05-06+13-14 +46 +05+06',
    '+13-14 +53 +05+06-13-14', '-06+13-14 -46-53 +05+06-14', '+05-07+13-15 +39-47 +13-15',
    '+05-07 -60-61 +05-07-13+15', '+05-07-15 -39+47-60-61 +07+13-15', '+06+14 +22+30+46-49-51-52+54-55-57 +14',
    '+06 +14-15-30+38+50+51-53+54+62 +06-14', '+06-07 -15-48-62 +06+07', '+14-15 +06+55+57 +14+15',
    '+06+15 +55+62 +07+14', '+07+15 +23-39+47-48-56-59-60-62+63 +07', '+15 -06+07+31-39-55-58-60-61-63 +07-15',
))
_ORDER_MLP = [4, 5, 6, 7, 8, 9, 10, 11, 12, 2, 3, 15, 16, 17, 18, 19, 20, 0, 1, 23, 24, 25, 13, 14, 21, 22]


def _combine(coef, xs):
    xs = list(xs)
    rows = [{k: int(c) for k, c in enumerate(row) if c} for row in coef]
    while True:
        count = collections.Counter((a, b, row[a] * row[b]) for row in rows for a in row for b in row if a < b)
        if not count or max(count.values()) < 2:
            break
        a, b, s = max(count, key=count.get)
        xs.append(xs[a] + xs[b] if s > 0 else xs[a] - xs[b])
        for row in rows:
            if a in row and b in row and row[a] * row[b] == s:
                row[len(xs) - 1] = row.pop(a)
                del row[b]
    out = []
    for row in rows:
        terms = sorted(row.items(), key=lambda t: -t[1])
        acc = xs[terms[0][0]] if terms[0][1] > 0 else -xs[terms[0][0]]
        for k, c in terms[1:]:
            acc = acc + xs[k] if c > 0 else acc - xs[k]
        out.append(acc)
    return out


def _left(sc, blocks):
    return list(enumerate(_combine(sc.u[sc.active[len(blocks) // sc.nb], :len(blocks)], blocks)))


def _block_matmul(sc, halves, lhs, rhs, outs=None, order=None):
    outs = [(1, o) for o in outs] if outs else [None] * (halves * sc.nb)
    todo = list(enumerate(sc.active[halves]))
    for pos, r in sorted(todo, key=lambda t: order.index(t[1])) if order else todo:
        m = _dot(lhs(pos), rhs(r))
        for k, c in enumerate(sc.w[r, :len(outs)]):
            if c and outs[k] is None:
                outs[k] = (c, m)
            elif c:
                s, acc = outs[k]
                outs[k] = (s, acc + m) if s == c else (1, acc - m) if s > 0 else (1, m - acc)
    return [acc if s > 0 else -acc for s, acc in outs]


def _ln(x):
    m = jnp.mean(x, axis=-1, keepdims=True)
    c = x - m
    v = jnp.mean(c * c, axis=-1, keepdims=True)
    return c * jax.lax.rsqrt(v + 1e-5)


def _sigmoid(x):
    return 0.5 * jnp.tanh(0.5 * x) + 0.5


def _dot(a, b):
    return jax.lax.dot_general(a, b, (((1,), (0,)), ((), ())), preferred_element_type=F32)


def _dot_nt(a, b):
    return jax.lax.dot_general(a, b, (((1,), (1,)), ((), ())), preferred_element_type=F32)


def _lo(w):
    return pltpu.bitcast(w << 16, F32)


def _hi(w):
    return pltpu.bitcast(w & np.uint32(0xFFFF0000), F32)


def _pack(lo, hi):
    lo, hi = (pltpu.bitcast(v, U32) + np.uint32(0x8000) for v in (lo, hi))
    return (lo >> 16) | (hi & np.uint32(0xFFFF0000))


def _bf(w):
    return pltpu.bitcast(w, BF16)


def _cols(x, nb):
    n = x.shape[1] // nb
    return [x[:, k * n:(k + 1) * n] for k in range(nb)]


def build(S, D, H, E, M, T, F, cfg):
    d = cfg["d"]
    nseg = S // T
    nch = nseg // d
    sa, sb = _S8, _S4
    NA, NB = sa.nb, sb.nb
    NI = F // D
    assert D == NA * 128 and F == NI * D + NB * 128 and E == 128 and 2 * (M + T) <= 128
    C, L, G, DA = d * T, M + T, H // NA, D // NA
    n1, na, nb = len(sa.active[1]), len(sa.mixed), len(sb.mixed)
    C2, T2, DB = C // 2, T // 2, D // NB
    scale = float(E) ** -0.5

    def loop(lo, hi, fn):
        def body(i, carry):
            fn(i)
            return carry
        jax.lax.fori_loop(lo, hi, body, 0)

    def kern(x_hbm, mem_ref, wq, wk, wv, wo_hbm, wg_hbm, wu_hbm, wd_hbm, out_hbm,
             xs, wqkv, wo, wg, wu, wd, mo, mg, mu, md, mg4, mu4, md4, ha, ba, bn, xa, xb, yb, qsem, osem, wsem, xsem, ysem):
        def qkv_copies(g, m):
            return [pltpu.make_async_copy((wq, wk, wv)[m].bitcast(U32).at[:, :, par, NA // 2 * g + p, :],
                                          wqkv.at[g, m, pl.ds((2 * p + par) * NA, NA)], qsem.at[g, m])
                    for p in range(NA // 2) for par in range(2)]

        def wo_copy(g, t):
            rows = pl.ds(pl.multiple_of(t * 16, 16), 16)
            return pltpu.make_async_copy(wo_hbm.bitcast(U32).at[g, :, rows, :], wo.at[g, :, rows, :], osem.at[g, t])

        def mlp_copies(which, t):
            rows = pl.ds(pl.multiple_of(t * 16, 16), 16)
            return [pltpu.make_async_copy((wg_hbm, wu_hbm, wd_hbm)[which].bitcast(U32).at[:, rows, :],
                                          (wg, wu, wd)[which].at[:, rows, :], wsem.at[which, t])]
        x_cps = [pltpu.make_async_copy(x_hbm.at[a:b], xs.at[a:b], xsem.at[k])
                 for k, (a, b) in enumerate(((0, T), (T, C + T), (C + T, S)))]

        def start(cps):
            for cp in cps:
                cp.start()

        def wait(cps):
            for cp in cps:
                cp.wait()

        def prep_qkv(g, m, rows):
            raw = [wqkv[g, m, s, rows, :] for s in range(NA * NA)]
            ev, od = (_combine(sa.v, [(_hi if n % 2 else _lo)(raw[(n // 2 * 2 + par) * NA + k])
                                      for k in range(NA) for n in range(NA)]) for par in range(2))
            for r in range(sa.n):
                wqkv[g, m, r, rows, :] = _pack(ev[r], od[r])

        def tile(k):
            return slice(k * 128, (k + 1) * 128)

        def w_out(g):
            return sa, lambda k, n, rows: wo[g, k, rows, tile(n)], lambda j, rows: (mo, (j, g, rows))

        def w_in(m, i):
            return (sa, lambda k, n, rows: (wg, wu)[m][k, rows, tile(i * NA + n)],
                    lambda j, rows: ((mg, mu)[m], (i, j, rows)))

        def w_in4(m, h):
            return (sb, lambda k, n, rows: (wg, wu)[m][2 * k + h, rows, tile(NI * NA + n)],
                    lambda j, rows: ((mg4, mu4)[m], (h, j, rows)))

        def w_down(i):
            return sa, lambda k, n, rows: wd[i * NA + k, rows, tile(n)], lambda j, rows: (md, (i, j, rows))

        def w_down4(c):
            return sb, lambda k, n, rows: wd[NI * NA + k, rows, tile(2 * n + c)], lambda j, rows: (md4, (c, j, rows))

        def prep(w, t):
            sc, raw, mixed = w
            rows = pl.ds(pl.multiple_of(t * 8, 8), 8)
            blocks = [raw(k, n, rows) for k in range(sc.nb) for n in range(sc.nb)]
            lo, hi = (_combine(sc.v[sc.mixed], [f(v) for v in blocks]) for f in (_lo, _hi))
            for j in range(len(sc.mixed)):
                ref, idx = mixed(j, rows)
                ref[idx] = _pack(lo[j], hi[j])

        def weight(ws, r):
            def one(sc, raw, mixed):
                if r not in sc.mixed:
                    return raw(*divmod(int(np.flatnonzero(sc.v[r])[0]), sc.nb), slice(None))
                ref, idx = mixed(sc.mixed.index(r), slice(None))
                return ref[idx]
            return _bf(jnp.concatenate([one(*w) for w in ws], axis=0))

        def prep_mlp(which):
            ws = ([w_in(which, i) for i in range(NI)] + [w_in4(which, h) for h in range(2)] if which < 2
                  else [w_down(i) for i in range(NI)] + [w_down4(c) for c in range(2)])

            def rows(t):
                pl.when(t % 2 == 0)(lambda: wait(mlp_copies(which, t // 2)))
                for w in ws:
                    prep(w, t)
            loop(0, 8, rows)

        def ordered(v, after):
            if after is None:
                return v
            return jnp.concatenate([jnp.where(after[0] == 0, v[0:8], after[1]), v[8:]], axis=0)

        def run(steps):
            for step, _ in steps:
                step()

        class Background:
            def __init__(self, zero):
                self.zero, self.queue, self.wait, self.period = zero, [], 0, 1

            def add(self, steps, period, delay):
                self.queue += steps
                self.period, self.wait = period, delay

            def __call__(self):
                self.wait -= 1
                if not self.queue or self.wait > 0:
                    return None
                self.wait = self.period
                step, ref = self.queue.pop(0)
                step()
                return self.zero, ref[self.zero, 0:8, 0:128]

        mrows = slice(0, M)

        def tok_head(t, i):
            def norm(w, r):
                if w == 0 and t is not None:
                    v = xs[pl.ds(pl.multiple_of(t * T + r, 8), 8), :].astype(F32)
                else:
                    v = xb[0, pl.ds(pl.multiple_of(i * T + r, 8), 8), :]
                ha[w, M + r:M + r + 8, :] = _ln(v)
            return [(functools.partial(norm, w, r), ha) for w in range(1 if t is None else 2) for r in range(0, T, 8)]

        def a_input(halves):
            return _left(sa, [b for w in range(halves) for b in _cols(ha[w], NA)])

        def attn_masks():
            r = jax.lax.broadcasted_iota(jnp.int32, (2 * L, 128), 0)
            k = jax.lax.broadcasted_iota(jnp.int32, (2 * L, 128), 1)
            rp = jnp.where(r < L, r, r - L)
            kp = k // 2
            same = (kp < L) & (k % 2 == jnp.where(r < L, 0, 1))
            valid = same & ((rp < M) | (rp >= kp))
            return valid, jnp.where(same, -1e9, -jnp.inf).astype(F32)

        def proj(h, g, m, halves, bg=lambda: None):
            c = _block_matmul(sa, halves, lambda s: ordered(h[s][1], bg()), lambda r: _bf(wqkv[g, m, r]))
            n = len(c) // 2
            if m == 0:
                return [jnp.concatenate([c[k], c[k + n]], axis=0) * scale for k in range(n)]
            z = jnp.zeros((64 - L, E), U32)
            return [_bf(jnp.concatenate([_pack(c[k], c[k + n]), z], axis=0)) for k in range(n)]

        def probs(qs, ks, masks):
            res = []
            for q, k in zip(qs, ks):
                s = jnp.where(masks[0], _dot_nt(q, k), masks[1])
                p = jnp.exp(s - jnp.max(s, axis=-1, keepdims=True))
                l = jnp.sum(p, axis=-1, keepdims=True)
                r = pl.reciprocal(l, approx=True)
                res.append(p * (r * (2.0 - l * r)))
            return res

        def mix(ps, vs):
            o = [_dot(p, v) for p, v in zip(ps, vs)]
            return _left(sa, [y[:L] for y in o] + [y[L:] for y in o])

        def out_proj(g0, n, halves, lhs, acc=None):
            return _block_matmul(sa, halves, lhs, functools.partial(weight, [w_out(g0 + k) for k in range(n)]),
                                 acc, sa.by_column)

        def finish(y, residual):
            for k, b in enumerate(y):
                ha[k // NA, mrows, tile(k % NA)] = b[:M]
                residual(k // NA, tile(k % NA), b[M:])

        def a_step(halves, zero, mlp_input, next_tokens, residual):
            masks = attn_masks()
            so, po, kc = cfg["so"], cfg["po"], cfg["kc"]
            pr, ps, os_, acc, now = {}, {}, {}, None, [0]
            span = len(sa.active[halves])
            side = sorted([((3 * g + 2) * span + so, 1, g) for g in range(G)]
                          + [((3 * g + 2) * span + so + po, 0, g) for g in range(G)])
            bg = Background(zero)

            def tick(tiles):
                while side and side[0][0] <= now[0]:
                    _, scores, g = side.pop(0)
                    if scores:
                        ps[g] = probs(pr[g, 0], pr[g, 1], masks)
                    else:
                        os_[g] = mix(ps[g], pr[g, 2])
                now[0] += tiles
                return bg()

            def out_lhs(g0, n, s):
                after = tick(n)
                assert all(g0 + k in os_ for k in range(n))
                return jnp.concatenate([ordered(os_[g0 + k][s][1], None if k else after) for k in range(n)], axis=1)
            h = a_input(halves)
            bg.add(mlp_input, *cfg["bg_mlp"])
            for g in range(G):
                for m in range(3):
                    pr[g, m] = proj(h, g, m, halves, lambda: tick(1))
            bg.add(next_tokens, *cfg["bg_tok"])
            for g0, n in zip(np.cumsum([0] + kc[:-1]).tolist(), kc):
                acc = out_proj(g0, n, halves, functools.partial(out_lhs, g0, n), acc)
            finish(acc, residual)
            run(bg.queue)

        def a_dual(c, i):
            t = c * d + i
            rows = pl.ds(pl.multiple_of(i * T, T), T)
            xrows = pl.ds(pl.multiple_of(t * T, T), T)

            def residual(layer, cols, v):
                xa[layer, rows, cols] = v + (xb[0, rows, cols] if layer else xs[xrows, cols].astype(F32))
            a_step(2, i // d, b_head(0, (i + d - 1) % d) + b_head(1, (i + d - 1) % d),
                   tok_head(jnp.minimum(t + 1, nseg - 1), jnp.minimum(i + 1, d - 1)), residual)

        def single_io(w, i):
            rows = pl.ds(pl.multiple_of(i * T, T), T)

            def residual(layer, cols, v):
                xa[w, rows, cols] = v + xb[0, rows, cols]
            return tok_head(None, jnp.minimum(i + 1, d - 1)), residual

        def a_head(c):
            return tok_head(jnp.minimum(c * d, nseg - 1), 0)

        def b_head(w, i):
            def norm(h, r):
                v = xa[w, pl.ds(pl.multiple_of(i * T + h * T2 + r, 8), 8), :]
                bn[2 * w + h, pl.ds(pl.multiple_of(i * T2 + r, 8), 8), :] = _ln(v)
            return [(functools.partial(norm, h, r), bn) for h in range(2) for r in range(0, T2, 8)]

        def b_step(c, w):
            bg = Background(w // 2)
            bg.add(a_head(c + 1), *cfg["bg_head"])
            o8, o4 = sa.by_column, _ORDER_MLP

            def gated(sc, lhs, ws, order):
                g = [_sigmoid(v) for v in _block_matmul(sc, 2, lhs, functools.partial(weight, ws(0)), order=order)]
                u = _block_matmul(sc, 2, lhs, functools.partial(weight, ws(1)), order=order)
                return _left(sc, [gg * uu for gg, uu in zip(g, u)])
            a8 = _left(sa, [b for h in range(2) for b in _cols(bn[2 * w + h], NA)])
            hs = [gated(sa, lambda s: ordered(a8[s][1], bg()),
                        lambda m: [w_in(m, i)], o8) for i in range(NI)]
            run(bg.queue)
            a4 = _left(sb, [b for h in range(2) for b in _cols(bn[2 * w + h], NB)])
            h4 = gated(sb, lambda s: a4[s][1], lambda m: [w_in4(m, h) for h in range(2)], o4)
            y = _block_matmul(sa, 2, lambda s: jnp.concatenate([h[s][1] for h in hs], axis=1),
                              functools.partial(weight, [w_down(i) for i in range(NI)]), order=o8)
            for n in range(2):
                z = _block_matmul(sb, 2, lambda s: h4[s][1], functools.partial(weight, [w_down4(n)]),
                                  y[n::2], o4)
                for k, v in enumerate(z):
                    cols = slice((k % NB) * DB + n * 128, (k % NB) * DB + (n + 1) * 128)
                    for i in range(d):
                        rows = slice(i * T + (k // NB) * T2, i * T + (k // NB + 1) * T2)
                        r = v[i * T2:(i + 1) * T2] + xa[w, rows, cols]
                        xb[w, rows, cols] = r
                        yb[rows, cols] = r.astype(BF16)

        def y_copy(c):
            return pltpu.make_async_copy(yb, out_hbm.at[pl.ds(pl.multiple_of(c * C, C), C), :], ysem.at[0])

        x_cps[0].start()
        for m in range(3):
            start(qkv_copies(0, m))
        x_cps[0].wait()
        xb[0, 0:T, :] = xs[0:T, :].astype(F32)
        ha[0, mrows, :] = mem_ref[...].astype(F32)
        ha[1, mrows, :] = mem_ref[...].astype(F32)
        run(tok_head(None, 0))
        xa[1] = jnp.zeros((C, D), F32)
        bn[...] = jnp.zeros(bn.shape, F32)

        def first_qkv(g):
            for m in range(3):
                @pl.when(g + 1 < G)
                def _():
                    start(qkv_copies(g + 1, m))

                @pl.when((g + 1 == G) & (m == 0))
                def _():
                    start(x_cps[1:2] + [wo_copy(k, t) for k in range(G) for t in range(4)])
                wait(qkv_copies(g, m))
                loop(0, DA // 16, lambda i: prep_qkv(g, m, pl.ds(pl.multiple_of(i * 8, 8), 8)))
            h = a_input(1)
            for s, v in mix(probs(proj(h, g, 0, 1), proj(h, g, 1, 1), attn_masks()), proj(h, g, 2, 1)):
                ba[g * n1 + s] = v
        loop(0, G, first_qkv)

        start([cp for which in range(3) for t in range(4) for cp in mlp_copies(which, t)])

        x_cps[1].wait()
        xb[0, T:C, :] = xs[T:C, :].astype(F32)

        def first_out(g):
            def rows(t):
                wo_copy(g, t).wait()
                prep(w_out(g), 2 * t)
                prep(w_out(g), 2 * t + 1)
            loop(0, 4, rows)
            for k, v in enumerate(out_proj(g, 1, 1, lambda s: ba[g * n1 + s])):
                xa[1, 0:L, tile(k)] += v
        loop(0, G, first_out)
        nxt, res = single_io(0, 0)
        run(nxt)
        finish(_cols(xa[1, 0:L, :], NA), res)

        def chunk(c):
            edge = (c == 0) | (c == nch)
            w0 = jnp.where(c < nch, 0, 1)

            @pl.when(edge)
            def _():
                @pl.when(c == nch)
                def _():
                    ha[0, mrows, :] = ha[1, mrows, :]
                    run(tok_head(None, 0))
                loop(1 - w0, d, lambda i: a_step(1, i // d, b_head(w0, (i + d - 1) % d),
                                                 *single_io(w0, i)))
                run(b_head(w0, d - 1))

                @pl.when(c == 0)
                def _():
                    for which in range(3):
                        prep_mlp(which)
                    x_cps[2].start()

            @pl.when(jnp.logical_not(edge))
            def _():
                loop(0, d, lambda i: a_dual(c, i))
                run(b_head(0, d - 1) + b_head(1, d - 1))

            @pl.when(c >= 2)
            def _():
                y_copy(c - 2).wait()
            loop(w0, jnp.where(c > 0, 2, 1), lambda w: b_step(c, w))

            @pl.when(c == 0)
            def _():
                run(a_head(1))
                x_cps[2].wait()

            @pl.when(c >= 1)
            def _():
                y_copy(c - 1).start()
        loop(0, nch + 1, chunk)
        y_copy(nch - 1).wait()

    any_spec = pl.BlockSpec(memory_space=pl.ANY)
    V = pltpu.VMEM
    return pl.pallas_call(
        kern,
        out_shape=jax.ShapeDtypeStruct((S, D), BF16),
        in_specs=[any_spec, pl.BlockSpec(memory_space=pltpu.VMEM)] + [any_spec] * 7,
        out_specs=any_spec,
        scratch_shapes=[
            V((S, D), BF16), V((G, 3, sa.n, DA // 2, E), U32),
            V((G, NA, 64, D), U32), V((NA, 64, F), U32), V((NA, 64, F), U32), V((F // 128, 64, D), U32),
            V((na, G, 64, 128), U32)] + [V((NI, na, 64, 128), U32)] * 3 + [V((2, nb, 64, 128), U32)] * 3 + [
            V((2, L, D), F32), V((G * n1, L, 128), F32), V((4, C2, D), F32),            V((2, C, D), F32), V((2, C, D), F32), V((C, D), BF16),
            pltpu.SemaphoreType.DMA((G, 3)), pltpu.SemaphoreType.DMA((G, 4)),
            pltpu.SemaphoreType.DMA((3, 4)), pltpu.SemaphoreType.DMA((3,)), pltpu.SemaphoreType.DMA((1,)),
        ],
        compiler_params=pltpu.CompilerParams(vmem_limit_bytes=126 * 2**20),
    )


@functools.partial(jax.jit, static_argnames=("A_seg_len",))
def pallas_interleave_layers__memory_aug_recurrent_mem_tr__glu_gated_glu__prompt_kernel(
        A_x, A_mem0, A_Wq, A_Wk, A_Wv, A_Wo, A_seg_len, B_x, B_w_gate, B_w_up, B_w_down):
    del B_x
    B, S, D = A_x.shape
    H, E = A_Wq.shape[1:]
    M = A_mem0.shape[1]
    F = B_w_gate.shape[1]
    call = build(S, D, H, E, M, int(A_seg_len), F, CFG)
    NA = _S8.nb
    qkv = [w.reshape(NA, D // (2 * NA), 2, H, E) for w in (A_Wq, A_Wk, A_Wv)]
    out = call(A_x.reshape(S, D), A_mem0.reshape(M, D), *qkv, A_Wo.reshape(H // NA, NA, E, D),
               B_w_gate.reshape(NA, D // NA, F), B_w_up.reshape(NA, D // NA, F),
               B_w_down.reshape(F // 128, 128, D))
    return out.reshape(B, S, D)
```
